```python
import jax
import jax.numpy as jnp

def _softmax(x, axis=-1):
    return jax.nn.softmax(x, axis=axis)
def _gelu(x):
    return jax.nn.gelu(x, approximate=True)
def _silu(x):
    return jax.nn.silu(x)
def _sigmoid(x):
    return jax.nn.sigmoid(x)
def _layernorm(x, axis=-1, eps=1e-5):
    m = jnp.mean(x, axis=axis, keepdims=True)
    v = jnp.var(x, axis=axis, keepdims=True)
    return (x - m) / jnp.sqrt(v + eps)
def _scatter_add(tgt, idx, src, axis=0):
    return tgt.at[idx].add(src)
def _segment_sum(src, seg, n):
    return jax.ops.segment_sum(src, seg, n)
class _Rng:
    def __init__(self, key):
        self._k = key
    def _next(self):
        self._k, sub = jax.random.split(self._k)
        return sub
    def normal(self, shape):
        return jax.random.normal(self._next(), shape, dtype=jnp.bfloat16)
    def randint(self, lo, hi, shape):
        return jax.random.randint(self._next(), shape, lo, hi, dtype=jnp.int32)
    def uniform(self, shape, lo=0.0, hi=1.0):
        return jax.random.uniform(self._next(), shape, jnp.bfloat16, lo, hi)
    def permutation(self, n):
        return jax.random.permutation(self._next(), n)


kernel_name = 'recurrent_scan__ssm_conv_s4__moe_arch_mod__prompt'

def setup_inputs():
    _rng = _Rng(jax.random.key(int.from_bytes(__import__("os").urandom(4), "little")))
    _w = (lambda a: (lambda t: t.astype(jnp.bfloat16) if jnp.issubdtype(t.dtype, jnp.floating) else t)(jnp.asarray(a)))
    def _A_setup():
        B, L, D, N = 1, 2048, 576, 128
        A_re = -jnp.exp((lambda *s: _rng.normal(s) * 0.05)(D, N))
        A_im = jnp.pi * (lambda *s: _rng.normal(s) * 0.05)(D, N)
        B_re = (lambda *s: _rng.normal(s) * 0.05)(D, N)
        B_im = (lambda *s: _rng.normal(s) * 0.05)(D, N)
        C_re = (lambda *s: _rng.normal(s) * 0.05)(D, N)
        C_im = (lambda *s: _rng.normal(s) * 0.05)(D, N)
        log_dt = (lambda *s: _rng.normal(s) * 0.05)(D) * 0.5 - 4.0
        Dskip = (lambda *s: _rng.normal(s) * 0.05)(D)
        return {
            "u": _w((lambda *s: _rng.normal(s) * 0.05)(B, L, D)),
            "A_re": _w(A_re),
            "A_im": _w(A_im),
            "B_re": _w(B_re),
            "B_im": _w(B_im),
            "C_re": _w(C_re),
            "C_im": _w(C_im),
            "log_dt": _w(log_dt),
            "Dskip": _w(Dskip),
        }
    _A_in = _A_setup()

    def _B_setup():
        B, S, D, F, C = 1, 2048, 576, 4608, 8
        return {
            "x": _w((lambda *s: _rng.normal(s) * 0.05)(B, S, D)),
            "w_r": _w((lambda *s: _rng.normal(s) * 0.05)(D)),
            "w_gate": _w((lambda *s: _rng.normal(s) * 0.05)(D, F)),
            "w_up": _w((lambda *s: _rng.normal(s) * 0.05)(D, F)),
            "w_down": _w((lambda *s: _rng.normal(s) * 0.05)(F, D)),
        }
    _B_in = _B_setup()

    return {
        "A_u": _A_in["u"],
        "A_A_re": _A_in["A_re"],
        "A_A_im": _A_in["A_im"],
        "A_B_re": _A_in["B_re"],
        "A_B_im": _A_in["B_im"],
        "A_C_re": _A_in["C_re"],
        "A_C_im": _A_in["C_im"],
        "A_log_dt": _A_in["log_dt"],
        "A_Dskip": _A_in["Dskip"],
        "B_x": _B_in["x"],
        "B_w_r": _B_in["w_r"],
        "B_w_gate": _B_in["w_gate"],
        "B_w_up": _B_in["w_up"],
        "B_w_down": _B_in["w_down"],
    }

def reference(A_u, A_A_re, A_A_im, A_B_re, A_B_im, A_C_re, A_C_im, A_log_dt, A_Dskip, B_x, B_w_r, B_w_gate, B_w_up, B_w_down):
    def _A_ref(u, A_re, A_im, B_re, B_im, C_re, C_im, log_dt, Dskip):
        Bsz, L, D = u.shape
        dt = jnp.exp(log_dt)[:, None]
        A = A_re + 1j * A_im
        Bc = B_re + 1j * B_im
        Cc = C_re + 1j * C_im
        logdA = dt * A
        dB = dt * Bc
        l = (lambda x, dt: x.astype(dt))(jnp.arange(L), A_re.dtype)
        P = jnp.exp(logdA[:, :, None] * l[None, None, :])
        K = jnp.einsum("dn,dnl,dn->dl", Cc, P, dB).real
        L2 = 2 * L
        Kp = jnp.pad(K, ((0, 0), (0, L)))
        up = (lambda x, *d: x.transpose(*d))(u, 0, 2, 1)
        up = jnp.pad(up, ((0, 0), (0, 0), (0, L)))
        Kf = (lambda x, axes=(-2,-1): jnp.fft.rfft2(x.astype(jnp.float32), axes=axes))(Kp[:, None, :], axes=(-2, -1))
        Uf = (lambda x, axes=(-2,-1): jnp.fft.rfft2(x.astype(jnp.float32), axes=axes))(up[:, :, None, :], axes=(-2, -1))
        Yf = Uf * Kf[None, :, :, :]
        y = (lambda x, s, axes=(-2,-1): jnp.fft.irfft2(x, s=s, axes=axes).astype(jnp.bfloat16))(Yf, (1, L2), axes=(-2, -1))[:, :, 0, :L]
        y = (lambda x, *d: x.transpose(*d))(y, 0, 2, 1) + u * Dskip[None, None, :]
        return y

    def _B_ref(x, w_r, w_gate, w_up, w_down):
        B, S, D = x.shape
        C = 8
        r = x @ w_r
        idx = jnp.argsort(-r, axis=-1)[:, :C]
        idx_e = jnp.repeat(idx.reshape(B, C, 1), D, axis=2)
        x_sel = jnp.take_along_axis(x, idx_e, axis=1)
        g = _silu(x_sel @ w_gate)
        u = x_sel @ w_up
        y = (g * u) @ w_down
        r_sel = _sigmoid(jnp.take_along_axis(r, idx, axis=1))
        y = y * r_sel.reshape(B, C, 1)
        b_off = (jnp.arange(B) * S).reshape(B, 1)
        flat_idx = (idx + b_off).reshape(B * C)
        zero = (x * 0.0).reshape(B * S, D)
        upd = _scatter_add(zero, flat_idx, y.reshape(B * C, D), axis=0)
        return x + upd.reshape(B, S, D)

    x = A_u
    xn = _layernorm(x, axis=-1)
    s = _A_ref(xn, A_A_re, A_A_im, A_B_re, A_B_im, A_C_re, A_C_im, A_log_dt, A_Dskip)
    g = _silu(_B_ref(xn, B_w_r, B_w_gate, B_w_up, B_w_down))
    return x + s * g
```

```python
import functools
import math

import numpy as np
import jax
import jax.numpy as jnp
from jax import lax
import jax.experimental.pallas as pl
import jax.experimental.pallas.tpu as pltpu

F32 = jnp.float32
BF16 = jnp.bfloat16
U32 = jnp.uint32
I32 = jnp.int32

D = 576
L = 2048
N = 128
FF = 4608
NSEL = 8
NCH = 8
RB = 64
NB = D // RB
NS = D // 16
SPB = RB // 16
FCH = (10, 10, 8, 5, 3)

_TILES = {
    "odd": (1, 3, 5, 7),
    "even": (2, 4, 6, 8),
    "t2": (258, 260, 262, 264),
    "t3": (516, 520, 772, 776),
    "t4": (1032, 1288, 1544, 1800),
}


def _rlag(l):
    u = int(np.float32(l).view(np.uint32))
    u = (u + 0x7FFF + ((u >> 16) & 1)) & 0xFFFF0000
    return int(np.uint32(u).view(np.float32))


def _tile_pts(name):
    base = name.rstrip("v")
    p = np.array([_TILES[base][l // 32] + 8 * (l % 32) for l in range(128)])
    if name == "t3v":
        p[127] = 512
    if name == "t4v":
        p[127] = 1024
    return p


def _fdk_row(r):
    f1 = 4 * np.arange(128) + 1
    f02 = np.concatenate([4 * np.arange(64), 4 * np.arange(64) + 2])
    w = 2 * np.pi / 512
    sgn = (-1.0) ** r
    r02 = np.cos(w * f02 * r) - sgn
    i02 = -np.sin(w * f02 * r)
    r02[0] *= 0.5
    i02[0] = -sgn
    return np.concatenate([np.cos(w * f1 * r), -np.sin(w * f1 * r), r02, i02]) / 128.0


def _gmat(c, tile):
    pts = _tile_pts(tile)
    g = np.zeros((128, 512))
    for r in range(1, 257):
        idx = np.nonzero(pts == _rlag(256 * c + r))[0]
        if len(idx):
            g[idx[0]] += _fdk_row(r)
    return g


def _pack_bf16(a):
    u = np.ascontiguousarray(a, np.float32).view(np.uint32)
    u = ((u + 0x7FFF + ((u >> 16) & 1)) >> 16).astype(np.uint32)
    return (u[0::2] | (u[1::2] << 16)).astype(np.uint32)


def _tables():
    f1 = 4 * np.arange(128) + 1
    w = 2 * np.pi / 512
    t = np.arange(128)[:, None] + 1
    a = np.cos(w * f1 * t)
    b = -np.sin(w * f1 * t)
    f0 = 4 * np.arange(64)
    f2 = f0 + 2
    m0 = np.concatenate([np.cos(w * f0 * t), -np.sin(w * f0 * t)], axis=1)
    m2 = np.concatenate([-np.sin(w * f2 * t), np.cos(w * f2 * t)], axis=1)
    um = np.concatenate([m0, a, m2, b - a, a + b], axis=1)
    g2 = _gmat(2, "t3v")
    g4 = _gmat(4, "t4v")
    gm = np.concatenate([
        _gmat(0, "odd"), _gmat(0, "even"),
        _gmat(1, "even"), _gmat(1, "t2"),
        g2, g2[:64],
        g4, g4[:96],
    ], axis=0)
    return _pack_bf16(um), _pack_bf16(gm)


_UM, _GM = _tables()


def _bf(x):
    return pltpu.bitcast(x, BF16)


def _u32(x):
    return pltpu.bitcast(x.astype(BF16), U32)


def _rb(x):
    return x.astype(BF16).astype(F32)


def _cmul(a, b):
    return (a[0] * b[0] - a[1] * b[1], a[0] * b[1] + a[1] * b[0])


def _csq(a):
    t = a[0] * a[1]
    return (a[0] * a[0] - a[1] * a[1], t + t)


def _sincos(th):
    magic = 12582912.0
    kf = th * (2.0 / math.pi) + magic
    ki = pltpu.bitcast(kf, I32)
    k = kf - magic
    r = th - k * 1.5703125
    r = r - k * 4.837512969970703125e-4
    r = r - k * 7.54978995489188216e-8
    r2 = r * r
    s = r + r * r2 * (-1.6666654611e-1 + r2 * (8.3321608736e-3 + r2 * -1.9515295891e-4))
    c = 1.0 + r2 * (-0.5 + r2 * (4.166664568298827e-2 + r2 * (-1.388731625493765e-3 + r2 * 2.443315711809948e-5)))
    swap = (ki & 1) == 1
    sn = jnp.where(swap, c, s)
    cs = jnp.where(swap, s, c)
    sbit = (ki & 2) << 30
    cbit = ((ki + 1) & 2) << 30
    sn = pltpu.bitcast(pltpu.bitcast(sn, I32) ^ sbit, F32)
    cs = pltpu.bitcast(pltpu.bitcast(cs, I32) ^ cbit, F32)
    return cs, sn


def _dot(a, b):
    return jnp.dot(a, b, preferred_element_type=F32)


def _dot_nt(a, b):
    return lax.dot_general(a, b, (((1,), (1,)), ((), ())), preferred_element_type=F32)


def _col_bcast(vec_ref):
    v = vec_ref[...].astype(F32).reshape(1, D)
    vp = jnp.concatenate([v, jnp.zeros((1, 64), F32)], axis=1)
    return [jnp.broadcast_to(vp[:, t * 128:(t + 1) * 128], (128, 128)).T for t in range(5)]


def _base8(p, dt):
    are, aim, bre, bim, cre, cim = p
    y1 = (dt * are) * math.log2(math.e)
    ph = {1: _sincos(dt * aim)}
    e = 1
    while e < 512:
        ph[2 * e] = _csq(ph[e])
        e *= 2
    pw = {}
    for e in (1, 2, 4, 8, 16, 256, 512):
        mg = jnp.exp2(y1 * float(e)) if e > 1 else jnp.exp2(y1)
        pw[e] = (mg * ph[e][0], mg * ph[e][1])
    w = _cmul((cre, cim), (dt * bre, dt * bim))
    k0 = jnp.sum(w[0], axis=1, keepdims=True)
    w1 = _cmul(w, pw[1])
    w2 = _cmul(w1, pw[1])
    w3 = _cmul(w2, pw[1])
    w258 = _cmul(w2, pw[256])

    def rot(z):
        return (pltpu.roll(z[0], 4, 0), pltpu.roll(z[1], 4, 0))
    rots = {e: rot(pw[e]) for e in (2, 4, 8, 16, 512)}
    return (pw, rots, w1, w2, rot(w3), rot(w258)), k0


def _grp_xy(bs, grp, lo4):
    pw, rots, w1, w2, w3r, w258r = bs

    def sel(lo, hi):
        return (jnp.where(lo4, lo[0], hi[0]), jnp.where(lo4, lo[1], hi[1]))
    if grp == 0:
        dup = {e: sel(pw[e], rots[e]) for e in (2, 4, 16, 512)}
        x0, x2, a8 = sel(w1, w3r), sel(w2, w258r), rots[8]
    else:
        dup = {e: sel(rots[e], pw[e]) for e in (2, 4, 16, 512)}
        x0, x2, a8 = sel(w3r, w1), sel(w258r, w2), pw[8]
    xv = [None] * 10
    xv[0] = x0
    xv[1] = _cmul(x0, dup[4])
    xv[2] = x2
    xv[3] = _cmul(xv[2], dup[2])
    xv[4] = _cmul(xv[3], dup[2])
    xv[5] = _cmul(xv[4], dup[2])
    xv[6] = _cmul(xv[3], dup[512])
    xv[7] = _cmul(xv[5], dup[512])
    xv[8] = _cmul(xv[7], dup[512])
    xv[9] = _cmul(xv[8], dup[512])
    y = (jnp.where(lo4, 1.0, a8[0]), jnp.where(lo4, 0.0, -a8[1]))
    m = dup[16]
    ys = [y]
    for _ in range(15):
        y = (y[0] * m[0] + y[1] * m[1], y[1] * m[0] - y[0] * m[1])
        ys.append(y)

    def mat(vs):
        return jnp.concatenate([jnp.concatenate([v[0] for v in vs], 0),
                                jnp.concatenate([v[1] for v in vs], 0)], 1).astype(BF16)
    return _dot_nt(mat(xv), mat(ys))


def _pk(a, b):
    return pltpu.pack_elementwise([a, b], packed_dtype=BF16)


def _upk(w, h):
    return pltpu.unpack_elementwise(w, index=h, packed_dtype=BF16, unpacked_dtype=F32)


_KT = [(0, 256, 0), (128, 256, 256), (384, 128, 512), (512, 128, 576),
       (640, 128, 704), (768, 128, 800), (768, 128, 768), (768, 128, 736)]

CFG = dict(RU=16, gw=4, kt0=4, ffn_grp=(3, 1, 1), xsel_at=26, xw=16, kt_ln=3, kt_lag=1, utj=4, order=1, lag=1, lead=1, scopes=False)


def _kernel(z_hbm, x_hbm, are_hbm, aim_hbm, bre_hbm, bim_hbm, cre_hbm, cim_hbm, ldt_hbm, dsk_hbm,
            wr_hbm, wg_hbm, wu_hbm, wd_hbm, um_hbm, gm_hbm, out_hbm,
            zs, xb, prm, ldt, dsk, wr, wg, wu, wd, um, gm,
            umt, dtc, dkc, k0c, kd, xh, vv, ur0, ur1, ur2, yb, ob,
            sem_small, sem_x, sem_w, sem_o, *ksps):
    urs = (ur0, ur1, ur2)
    _cur = [None]

    def mark(name):
        if not CFG["scopes"]:
            return
        if _cur[0] is not None:
            _cur[0].__exit__(None, None, None)
            _cur[0] = None
        if name:
            _cur[0] = jax.named_scope(name)
            _cur[0].__enter__()
    small = [(ldt_hbm, ldt), (are_hbm, prm.at[0]), (aim_hbm, prm.at[1]), (bre_hbm, prm.at[2]),
             (bim_hbm, prm.at[3]), (cre_hbm, prm.at[4]), (cim_hbm, prm.at[5]),
             (dsk_hbm, dsk), (wr_hbm, wr)]
    small_cp = [pltpu.make_async_copy(s, d, sem_small.at[i]) for i, (s, d) in enumerate(small)]
    for cp in small_cp:
        cp.start()
    x_cp = [pltpu.make_async_copy(s, d, sem_x.at[i]) for i, (s, d) in
            enumerate([(gm_hbm, gm), (z_hbm, zs), (um_hbm, um), (x_hbm, xb)])]
    for cp in x_cp:
        cp.start()
    w_cp = []
    off = 0
    for c, n in enumerate(FCH):
        cs = pl.ds(off * 128, n * 128)
        w_cp.append([pltpu.make_async_copy(h.at[:, cs], b.bitcast(BF16).at[:, cs], sem_w.at[i, c])
                     for i, (h, b) in enumerate([(wg_hbm, wg), (wu_hbm, wu), (wd_hbm, wd)])])
        for cp in w_cp[-1]:
            cp.start(priority=1)
        off += n

    sub = lax.broadcasted_iota(I32, (8, 128), 0)
    lane = lax.broadcasted_iota(I32, (8, 128), 1)
    lo4 = sub < 4
    gidx = 4 * (lane % 32) + (sub % 4)
    lo64 = lane < 64
    beven = ((lane // 32) % 2) == 0
    last = lane == 127

    mark('s0_wait0')
    small_cp[0].wait()
    mark('s1_prep')
    dtb = _col_bcast(ldt)
    for t in range(5):
        n = 128 if t < 4 else 64
        dtc[pl.ds(t * 128, n), :] = _rb(jnp.exp(dtb[t][:n]))
    mark('s2_waitp')
    for cp in small_cp[1:]:
        cp.wait()
    mark('s3_A1')
    zo = []

    def dyn(r):
        return pl.multiple_of(zo[0] + r, 8)

    ktp = {}

    def kt_unit(b, c):
        l0, kk, g0 = _KT[c]
        raw = _dot(_bf(kd[pl.ds(b * (RB // 2), RB // 2), pl.ds(l0, kk)]), _bf(gm[pl.ds(g0 // 2, kk // 2), :]))
        if c == 0:
            s1, s2 = raw[:, :256], raw[:, 256:]
        else:
            prev = ktp.pop(b)
            s1, s2 = raw[:, :256] - prev[:, :256], raw[:, 256:] + prev[:, 256:]
        if c < NCH - 1:
            ktp[b] = raw
        dl = jnp.take_along_axis(s2[:, 128:], jnp.zeros((RB, 128), I32), axis=1, mode="promise_in_bounds")
        rows = pl.ds(dyn(0), RB)
        ksp = ksps[b]
        ksp[rows, pl.ds(512 * c, 128)] = s1[:, :128] - dl
        ksp[rows, pl.ds(512 * c + 128, 128)] = s1[:, 128:]
        ksp[rows, pl.ds(512 * c + 256, 256)] = s2

    def extract(st, o4):
        g = [[jnp.take_along_axis(_pk(o4[0][grp][8 * v:8 * v + 8], o4[1][grp][8 * v:8 * v + 8]), gidx, axis=1,
                                  mode="promise_in_bounds") for v in range(10)] for grp in range(2)]

        def mix(a, b):
            return jnp.where(lo4, a, b), pltpu.roll(jnp.where(lo4, b, a), 4, 0)

        def two(va, vb, m1, m2):
            p, q = mix(jnp.where(m1, g[0][va], g[0][vb]), jnp.where(m1, g[1][va], g[1][vb]))
            return jnp.where(m2, p, q)

        def four(gg):
            return jnp.where(lo64, jnp.where(beven, gg[2], gg[3]), jnp.where(beven, gg[4], gg[5]))
        t_odd = two(0, 1, lo64, beven)
        t_even, t_2 = mix(four(g[0]), four(g[1]))
        t_3 = two(6, 7, beven, lo64)
        t_4 = two(8, 9, lo64, beven)
        tl = [t_odd, t_even, t_2, jnp.where(last, t_2, t_3), t_3, jnp.where(last, t_3, t_4), t_4]
        for t in range(7):
            kd[pl.ds(st * 8, 8), pl.ds(128 * t, 128)] = tl[t]

    tk = {}
    row16 = lax.broadcasted_iota(I32, (16, 128), 0)
    lane16 = lax.broadcasted_iota(I32, (16, 128), 1)

    def ln_chunk(j):
        cj = slice(256 * j, 256 * j + 256)
        s1 = s2 = None
        for i in range(NS):
            v = xb[pl.ds(i * 16, 16), cj].astype(F32)
            v0, v1 = v[:8], v[8:]
            a, b = v0 + v1, v0 * v0 + v1 * v1
            s1, s2 = (a, b) if i == 0 else (s1 + a, s2 + b)
        mean = jnp.sum(s1, axis=0, keepdims=True) * (1.0 / D)
        var = jnp.sum(s2, axis=0, keepdims=True) * (1.0 / D) - mean * mean
        var = jnp.maximum(var, 0.0)
        sd = _rb(jnp.sqrt(_rb(_rb(var) + 1e-5)))
        mb = jnp.broadcast_to(_rb(mean), (16, 256))
        hi = jnp.broadcast_to(0.5 / sd, (16, 256))
        for i in range(NS):
            rw = pl.ds(dyn(i * 8), 8)
            hv = _rb(xb[pl.ds(i * 16, 16), cj].astype(F32) - mb) * hi
            h0, h1 = hv[:, :128], hv[:, 128:]
            xh[rw, pl.ds(256 * j, 128)] = _u32(h0)
            xh[rw, pl.ds(256 * j + 128, 128)] = _u32(h1)
            vv[rw, pl.ds(256 * j, 128)] = _u32(h0 + h1)
            vv[rw, pl.ds(256 * j + 128, 128)] = _u32(h0 - h1)
        if j == 0:
            tk["w"] = jnp.broadcast_to(wr[...].astype(F32).reshape(1, D), (16, D)).astype(BF16)
        r = _dot(tk["w"], _bf(xh[:, cj]))
        for t in range(2):
            r_t = r[:, 128 * t:128 * t + 128]
            tk["rc"] = r_t if (j == 0 and t == 0) else jnp.where(row16 == 2 * j + t, r_t, tk["rc"])

    def topk():
        bits = pltpu.bitcast(_rb(tk["rc"] * 2.0), I32)
        mono = (jnp.where(bits < 0, bits ^ 0x7FFF0000, bits) >> 16) + 32768
        key = pltpu.bitcast(0x30000000 + (mono << 11) + (2047 - (row16 * 128 + lane16)), F32)
        kcol = jnp.zeros((16, 128), I32)
        for j in range(NSEL):
            mx = jnp.max(jnp.max(key, axis=0, keepdims=True), axis=1, keepdims=True)
            mxb = jnp.broadcast_to(mx, (16, 128))
            key = jnp.where(key == mxb, 0.0, key)
            kcol = jnp.where(row16 == j, pltpu.bitcast(mxb, I32), kcol)
        kcol = kcol - 0x30000000
        idxcol = jnp.where(row16 < NSEL, 2047 - (kcol & 2047), -1)
        hb = ((kcol >> 11) - 32768) << 16
        rsel = pltpu.bitcast(jnp.where(hb < 0, hb ^ 0x7FFF0000, hb), F32)
        rsel = jnp.where(row16 < NSEL, rsel, 0.0)
        tk["rs"] = _rb(jax.nn.sigmoid(rsel))
        tk["oh"] = jnp.concatenate(
            [jnp.where(idxcol == lane16 + 128 * t, 1.0, 0.0) for t in range(16)], axis=1).astype(BF16)

    def xsel(t):
        cs = slice(128 * t, 128 * t + 128)
        v = _dot_nt(tk["oh"][:, cs], _bf(xh[:, cs]))
        tk["xa"] = v if t == 0 else tk["xa"] + v
        if t == 15:
            tk["xs"] = (tk["xa"] * 2.0).astype(BF16)

    def ffn_gu(c):
        cs = pl.ds(sum(FCH[:c]) * 128, FCH[c] * 128)
        g = _rb(_dot(tk["xs"], _bf(wg[:, cs])))
        u = _rb(_dot(tk["xs"], _bf(wu[:, cs])))
        sg = _rb(0.5 * jnp.tanh(0.5 * g) + 0.5)
        tk["h", c] = (_rb(g * sg) * u).astype(BF16)

    def ffn_dn(c):
        cs = pl.ds(sum(FCH[:c]) * 128, FCH[c] * 128)
        y = _dot_nt(tk.pop(("h", c)), _bf(wd[:, cs]))
        tk["y"] = y if c == 0 else tk["y"] + y

    def ffn_all():
        c = 0
        for n in CFG["ffn_grp"]:
            for cc in range(c, c + n):
                for cp in w_cp[cc]:
                    cp.wait()
            for cc in range(c, c + n):
                ffn_gu(cc)
                if cc > 0:
                    ffn_dn(cc - 1)
            c += n
        ffn_dn(c - 1)

    utj = CFG["utj"]
    RU = CFG["RU"]

    def ut_piece(b, k, j0):
        rw = pl.ds(b * (RU // 2), RU // 2)
        rows = pl.ds(dyn(0), RU)
        ur = urs[b % 3]
        js = range(j0, j0 + utj)

        def lhs(ref, o):
            return _bf(jnp.concatenate([ref[rw, pl.ds(256 * j + o, 128)] for j in js], axis=0))

        def put(val, col):
            for i, j in enumerate(js):
                ur[rows, pl.ds(640 * j + col, 128)] = val[i * RU:(i + 1) * RU]
        if k == 0:
            v = _dot(lhs(vv, 0), _bf(um[:, 0:256]))
            b2 = _dot(lhs(vv, 128), _bf(um[:, 256:384]))
            a0 = v[:, :128]
            l64 = lax.broadcasted_iota(I32, a0.shape, 1) < 64
            put(jnp.where(l64, a0, b2), 0)
            put(v[:, 128:], 128)
            put(pltpu.roll(jnp.where(l64, b2, a0), 64, 1), 256)
        else:
            put(_dot(lhs(xh, 128), _bf(um[:, 384:512])), 384)
            put(_dot(lhs(xh, 0), _bf(um[:, 512:640])), 512)

    def mac(g, cls):
        ur = urs[(8 * g // RU) % 3]

        @functools.lru_cache(None)
        def us(j):
            def ld(c):
                return ur[pl.ds((8 * g) % RU, 8), pl.ds(640 * j + c, 128)]
            if cls == 0:
                a, b = ld(0), ld(256)
                return (a, b, a + b)
            t1, t2, t3 = ld(128), ld(384), ld(512)
            return (t1 + t2, t3 - t1, t2 + t3)

        @functools.lru_cache(None)
        def ks(j):
            o = 512 * j + 256 * (1 - cls)
            ksp, kr = ksps[8 * g // RB], pl.ds((8 * g) % RB, 8)
            sr, si = ksp[kr, pl.ds(o, 128)], ksp[kr, pl.ds(o + 128, 128)]
            return (sr, si - sr, sr + si)
        outs = []
        prev = None
        for m in range(NCH):
            acc = None
            for j in range(m + 1):
                a, b, s = us(j)
                c_, e_, g_ = ks(m - j)
                t = (c_ * s, a * e_, b * g_)
                acc = t if acc is None else tuple(x + y for x, y in zip(acc, t))
            z = (acc[0] - acc[2], acc[0] + acc[1])
            if m % 2:
                za, zb = prev, z
                if cls == 0:
                    zr = _pk(za[0], zb[0])
                    zis = pltpu.roll(_pk(za[1], zb[1]), 64, 1)
                    outs.append((jnp.where(lo64, zr, zis), jnp.where(lo64, zis, zr)))
                else:
                    outs.append((_pk(za[0] + za[1], zb[0] + zb[1]), _pk(za[1], zb[1]), _pk(za[0], zb[0])))
            prev = z
        return outs

    zq, wq = {}, {}

    def inv(g, cls):
        zo_ = zq.pop((g, cls))

        def st(t):
            return _bf(jnp.concatenate([zo_[p][t] for p in range(4)], axis=0))
        if cls == 0:
            wq[g] = [_dot(st(t), _bf(umt[:, c:c + 128])) for t, c in ((0, 0), (1, 256))]
        else:
            q1, q2, q3 = [_dot(st(t), _bf(umt[:, c:c + 128])) for t, c in ((0, 128), (1, 384), (2, 512))]
            w0, w2 = wq.pop(g)
            p_ = q1 + w2
            y0 = p_ + (q2 + w0)
            y1 = (q3 + w0) - p_
            for p in range(4):
                yb[pl.ds(8 * g, 8), pl.ds(256 * p, 128)] = _u32(y0[16 * p:16 * p + 16])
                yb[pl.ds(8 * g, 8), pl.ds(256 * p + 128, 128)] = _u32(y1[16 * p:16 * p + 16])

    ktq = []
    slotno = [0]
    pat = CFG.get("kt_pat", [1, 0, 0, 1, 0, 0, 1, 0, 1, 0, 1, 1, 0, 1, 0, 1])
    xw = CFG["xw"]

    def kt_drain(n):
        for _ in range(n):
            if ktq and ktq[0][0] <= slotno[0]:
                kt_unit(*ktq.pop(0)[1:])

    utq = [(b, k, j) for b in range(D // RU) for j in range(0, NCH, utj) for k in range(2)]
    pend = None
    for st in range(NS):
        if st == xw:
            mark('s4_waitx')
            for cp in x_cp:
                cp.wait()
            zo.append(zs[0] * 8)
            mark('s5_ln')
            dkb = _col_bcast(dsk)
            for t in range(5):
                n = 128 if t < 4 else 64
                dkc[pl.ds(t * 128, n), :] = dkb[t][:n]
                umt[:, pl.ds(128 * t, 128)] = pltpu.bitcast(_bf(um[:, 128 * t:128 * t + 128]).T, U32)
            for j in range(NCH):
                kt_drain(CFG["kt_ln"])
                ln_chunk(j)
            mark('s6_A2')
            topk()
        r0 = st * 16
        pk = [pltpu.bitcast(prm[k, pl.ds(r0, 16), :], U32) for k in range(6)]
        o4 = []
        for half in range(2):
            rows = pl.ds(r0 + half, 8, stride=2)
            bs, k0 = _base8([_upk(w, half) for w in pk], dtc[rows, :])
            k0c[rows, :] = jnp.broadcast_to(k0, (8, 128))
            if half == 0 and pend is not None:
                extract(*pend)
                if (pend[0] + 1) % SPB == 0:
                    ktq.extend([(slotno[0] + 4 * CFG["kt_lag"], pend[0] // SPB, c) for c in range(NCH)])
            oo = []
            for grp in range(2):
                if st >= xw:
                    kt_drain(pat[slotno[0] % 16])
                slotno[0] += 1
                oo.append(_grp_xy(bs, grp, lo4))
            o4.append(oo)
        pend = (st, o4)
        if 0 <= st - CFG['xsel_at'] < 8:
            xsel(2 * (st - CFG['xsel_at']))
            xsel(2 * (st - CFG['xsel_at']) + 1)
    extract(*pend)
    ktq.extend([(0, NB - 1, c) for c in range(NCH)])
    slotno[0] += 1000

    mark('s7_B')
    gpb = RB // 8
    npre = 16 // utj + (2 * CFG["lead"] * 64 // RU) // utj
    for i in range(npre):
        ut_piece(*utq.pop(0))
    lag = CFG["lag"]
    NG = D // 8
    for s in range(NG + lag):
        for cls in range(2):
            if s < NG:
                zq[(s, cls)] = mac(s, cls)
            if CFG["order"] == 1 and s >= lag:
                inv(s - lag, cls)
            if ((2 * s + cls) * 64 // RU) % utj == 0:
                for _ in range(max(1, 64 // RU // utj)):
                    if utq:
                        ut_piece(*utq.pop(0))
            if cls == 1:
                kt_drain(1)
            if CFG["order"] == 0 and s >= lag:
                inv(s - lag, cls)

    mark('s8_ffn')
    ffn_all()
    rs = jnp.concatenate([tk["rs"]] * 5, axis=1)[:, :D]
    upd = (_rb(_rb(tk["y"]) * rs) * 0.5).astype(BF16)
    updt = lax.dot_general(upd, jnp.eye(16, 128, dtype=BF16), (((0,), (0,)), ((), ())),
                           preferred_element_type=F32).astype(BF16)

    mark('s9_final')
    ohp = jnp.concatenate([tk["oh"], jnp.zeros((112, L), BF16)], axis=0)
    o_cp = []
    for b in range(NB):
        rows = pl.ds(b * RB, RB)
        du = _dot(updt[b * RB:(b + 1) * RB], ohp)
        for s in range(SPB):
            r16 = pl.ds(b * RB + 16 * s, 16)
            h = _bf(xh[pl.ds(b * (RB // 2) + 8 * s, 8), :]).astype(F32)
            yw = yb[r16, :]
            y = jnp.concatenate([_upk(yw[:, 256 * (m // 2):256 * (m // 2) + 256], m % 2) for m in range(NCH)], axis=1)
            dv = (dkc[r16, :] + k0c[r16, :]) * 2.0
            s_ = y + h * jnp.concatenate([dv] * 16, axis=1)
            zh = h + du[16 * s:16 * s + 16]
            g = zh * jnp.tanh(zh) + zh
            ob[r16, :] = (xb[r16, :].astype(F32) + s_ * g).astype(BF16)
        cp = pltpu.make_async_copy(ob.at[rows, :], out_hbm.at[rows, :], sem_o.at[b])
        cp.start()
        o_cp.append(cp)
    mark('sa_waito')
    for cp in o_cp:
        cp.wait()
    mark(None)


@jax.jit
def pallas_recurrent_scan__ssm_conv_s4__moe_arch_mod__prompt_kernel(A_u, A_A_re, A_A_im, A_B_re, A_B_im, A_C_re, A_C_im, A_log_dt, A_Dskip,
              B_x, B_w_r, B_w_gate, B_w_up, B_w_down):
    xt = jnp.transpose(A_u[0])
    wdt = jnp.transpose(B_w_down)
    scratch = [
        pltpu.SMEM((1,), I32),
        pltpu.VMEM((D, L), BF16),
        pltpu.VMEM((6, D, N), BF16),
        pltpu.VMEM((D,), BF16),
        pltpu.VMEM((D,), BF16),
        pltpu.VMEM((D,), BF16),
        pltpu.VMEM((D // 2, FF), U32),
        pltpu.VMEM((D // 2, FF), U32),
        pltpu.VMEM((D // 2, FF), U32),
        pltpu.VMEM(_UM.shape, U32),
        pltpu.VMEM(_GM.shape, U32),
        pltpu.VMEM(_UM.shape, U32),
        pltpu.VMEM((D, 128), F32),
        pltpu.VMEM((D, 128), F32),
        pltpu.VMEM((D, 128), F32),
        pltpu.VMEM((D // 2, 896), U32),
        pltpu.VMEM((D // 2, L), U32),
        pltpu.VMEM((D // 2, L), U32),
        pltpu.VMEM((CFG['RU'], 5120), F32),
        pltpu.VMEM((CFG['RU'], 5120), F32),
        pltpu.VMEM((CFG['RU'], 5120), F32),
        pltpu.VMEM((D, L // 2), U32),
        pltpu.VMEM((D, L), BF16),
        pltpu.SemaphoreType.DMA((10,)),
        pltpu.SemaphoreType.DMA((4,)),
        pltpu.SemaphoreType.DMA((3, len(FCH))),
        pltpu.SemaphoreType.DMA((NB,)),
    ] + [pltpu.VMEM((RB, 4096), F32)] * NB
    out = pl.pallas_call(
        _kernel,
        out_shape=jax.ShapeDtypeStruct((D, L), BF16),
        in_specs=[pl.BlockSpec(memory_space=pl.ANY)] * 16,
        out_specs=pl.BlockSpec(memory_space=pl.ANY),
        scratch_shapes=scratch,
        compiler_params=pltpu.CompilerParams(vmem_limit_bytes=100 * 2**20),
        name="s4_mod",
    )(jnp.zeros((1,), I32), xt, A_A_re, A_A_im, A_B_re, A_B_im, A_C_re, A_C_im, A_log_dt, A_Dskip,
      B_w_r, B_w_gate, B_w_up, wdt, jnp.asarray(_UM), jnp.asarray(_GM))
    return jnp.transpose(out)[None]
```

```python
import functools
import math

import numpy as np
import jax
import jax.numpy as jnp
from jax import lax
import jax.experimental.pallas as pl
import jax.experimental.pallas.tpu as pltpu

F32 = jnp.float32
BF16 = jnp.bfloat16
U32 = jnp.uint32
I32 = jnp.int32

D = 576
L = 2048
N = 128
FF = 4608
NSEL = 8
NCH = 8
RB = 64
NB = D // RB
NS = D // 16
SPB = RB // 16
FCH = (10, 10, 8, 6, 2)

_TILES = {
    "odd": (1, 3, 5, 7),
    "even": (2, 4, 6, 8),
    "t2": (258, 260, 262, 264),
    "t3": (516, 520, 772, 776),
    "t4": (1032, 1288, 1544, 1800),
}


def _rlag(l):
    u = int(np.float32(l).view(np.uint32))
    u = (u + 0x7FFF + ((u >> 16) & 1)) & 0xFFFF0000
    return int(np.uint32(u).view(np.float32))


def _tile_pts(name):
    base = name.rstrip("v")
    p = np.array([_TILES[base][l // 32] + 8 * (l % 32) for l in range(128)])
    if name == "t3v":
        p[127] = 512
    if name == "t4v":
        p[127] = 1024
    return p


def _fdk_row(r):
    f1 = 4 * np.arange(128) + 1
    f02 = np.concatenate([4 * np.arange(64), 4 * np.arange(64) + 2])
    w = 2 * np.pi / 512
    sgn = (-1.0) ** r
    r02 = np.cos(w * f02 * r)
    i02 = -np.sin(w * f02 * r)
    r02[0] = (-sgn - 1.0) / 4.0
    i02[0] = (1.0 - sgn) / 4.0
    return np.concatenate([np.cos(w * f1 * r), -np.sin(w * f1 * r), r02, i02]) / 128.0


def _gmat(c, tile):
    pts = _tile_pts(tile)
    g = np.zeros((128, 512))
    for r in range(1, 257):
        idx = np.nonzero(pts == _rlag(256 * c + r))[0]
        if len(idx):
            g[idx[0]] += _fdk_row(r)
    return g


def _pack_bf16(a):
    u = np.ascontiguousarray(a, np.float32).view(np.uint32)
    u = ((u + 0x7FFF + ((u >> 16) & 1)) >> 16).astype(np.uint32)
    return (u[0::2] | (u[1::2] << 16)).astype(np.uint32)


def _tables():
    f1 = 4 * np.arange(128) + 1
    w = 2 * np.pi / 512
    t = np.arange(128)[:, None] + 1
    a = np.cos(w * f1 * t)
    b = -np.sin(w * f1 * t)
    f0 = 4 * np.arange(64)
    f2 = f0 + 2
    m0 = np.concatenate([np.cos(w * f0 * t), -np.sin(w * f0 * t)], axis=1)
    m2 = np.concatenate([-np.sin(w * f2 * t), np.cos(w * f2 * t)], axis=1)
    m0[:, 64] = (-1.0) ** t[:, 0]
    um = np.concatenate([m0, a, m2, b - a, a + b], axis=1)
    g0 = np.concatenate([_gmat(0, "odd"), _gmat(0, "even")], axis=0)
    lags = np.concatenate([_tile_pts("odd"), _tile_pts("even")])
    sel = np.full((8, 256), -1, np.int32)
    for k, (c, tile) in enumerate([(1, "t2"), (2, "t3v"), (4, "t4v"), (1, "even")]):
        pts = _tile_pts(tile)
        for rho, r in enumerate(lags):
            idx = np.nonzero(pts == _rlag(256 * c + int(r)))[0]
            if len(idx):
                sel[k, rho] = idx[0]
    selp = np.zeros((8, 512), np.int32)
    selp[:, :256] = sel
    return _pack_bf16(um), np.concatenate([_pack_bf16(g0), selp.view(np.uint32)], axis=0)


_UM, _G0 = _tables()


def _bf(x):
    return pltpu.bitcast(x, BF16)


def _u32(x):
    return pltpu.bitcast(x.astype(BF16), U32)


def _rb(x):
    return x.astype(BF16).astype(F32)


def _cmul(a, b):
    return (a[0] * b[0] - a[1] * b[1], a[0] * b[1] + a[1] * b[0])


def _csq(a):
    t = a[0] * a[1]
    return (a[0] * a[0] - a[1] * a[1], t + t)


def _sincos(th):
    magic = 12582912.0
    kf = th * (2.0 / math.pi) + magic
    ki = pltpu.bitcast(kf, I32)
    k = kf - magic
    r = th - k * 1.5703125
    r = r - k * 4.837512969970703125e-4
    r = r - k * 7.54978995489188216e-8
    r2 = r * r
    s = r + r * r2 * (-1.6666654611e-1 + r2 * (8.3321608736e-3 + r2 * -1.9515295891e-4))
    c = 1.0 + r2 * (-0.5 + r2 * (4.166664568298827e-2 + r2 * (-1.388731625493765e-3 + r2 * 2.443315711809948e-5)))
    swap = (ki & 1) == 1
    sn = jnp.where(swap, c, s)
    cs = jnp.where(swap, s, c)
    sbit = (ki & 2) << 30
    cbit = ((ki + 1) & 2) << 30
    sn = pltpu.bitcast(pltpu.bitcast(sn, I32) ^ sbit, F32)
    cs = pltpu.bitcast(pltpu.bitcast(cs, I32) ^ cbit, F32)
    return cs, sn


def _dot(a, b):
    return jnp.dot(a, b, preferred_element_type=F32)


def _dot_nt(a, b):
    return lax.dot_general(a, b, (((1,), (1,)), ((), ())), preferred_element_type=F32)


def _col_bcast(vec_ref):
    v = vec_ref[...].astype(F32).reshape(1, D)
    vp = jnp.concatenate([v, jnp.zeros((1, 64), F32)], axis=1)
    return [jnp.broadcast_to(vp[:, t * 128:(t + 1) * 128], (128, 128)).T for t in range(5)]


def _base8(p, dt):
    are, aim, bre, bim, cre, cim = p
    y1 = (dt * are) * math.log2(math.e)
    ph = {1: _sincos(dt * aim)}
    e = 1
    while e < 512:
        ph[2 * e] = _csq(ph[e])
        e *= 2
    pw = {}
    for e in (1, 2, 4, 8, 16, 256, 512):
        mg = jnp.exp2(y1 * float(e)) if e > 1 else jnp.exp2(y1)
        pw[e] = (mg * ph[e][0], mg * ph[e][1])
    w = _cmul((cre, cim), (dt * bre, dt * bim))
    k0 = jnp.sum(w[0], axis=1, keepdims=True)
    w1 = _cmul(w, pw[1])
    w2 = _cmul(w1, pw[1])
    w3 = _cmul(w2, pw[1])
    w258 = _cmul(w2, pw[256])

    def rot(z):
        return (pltpu.roll(z[0], 4, 0), pltpu.roll(z[1], 4, 0))
    rots = {e: rot(pw[e]) for e in (2, 4, 8, 16, 512)}
    return (pw, rots, w1, w2, rot(w3), rot(w258)), k0


def _grp_xy(bs, grp, lo4):
    pw, rots, w1, w2, w3r, w258r = bs

    def sel(lo, hi):
        return (jnp.where(lo4, lo[0], hi[0]), jnp.where(lo4, lo[1], hi[1]))
    if grp == 0:
        dup = {e: sel(pw[e], rots[e]) for e in (2, 4, 16, 512)}
        x0, x2, a8 = sel(w1, w3r), sel(w2, w258r), rots[8]
    else:
        dup = {e: sel(rots[e], pw[e]) for e in (2, 4, 16, 512)}
        x0, x2, a8 = sel(w3r, w1), sel(w258r, w2), pw[8]
    xv = [None] * 10
    xv[0] = x0
    xv[1] = _cmul(x0, dup[4])
    xv[2] = x2
    xv[3] = _cmul(xv[2], dup[2])
    xv[4] = _cmul(xv[3], dup[2])
    xv[5] = _cmul(xv[4], dup[2])
    xv[6] = _cmul(xv[3], dup[512])
    xv[7] = _cmul(xv[5], dup[512])
    xv[8] = _cmul(xv[7], dup[512])
    xv[9] = _cmul(xv[8], dup[512])
    y = (jnp.where(lo4, 1.0, a8[0]), jnp.where(lo4, 0.0, -a8[1]))
    m = dup[16]
    ys = [y]
    for _ in range(15):
        y = (y[0] * m[0] + y[1] * m[1], y[1] * m[0] - y[0] * m[1])
        ys.append(y)

    def mat(vs):
        return jnp.concatenate([jnp.concatenate([v[0] for v in vs], 0),
                                jnp.concatenate([v[1] for v in vs], 0)], 1).astype(BF16)
    return mat(xv), mat(ys)


def _pk(a, b):
    return pltpu.pack_elementwise([a, b], packed_dtype=BF16)


def _upk(w, h):
    return pltpu.unpack_elementwise(w, index=h, packed_dtype=BF16, unpacked_dtype=F32)


_KT = [(0, 256, 0), (128, 256, 256), (384, 128, 512), (512, 128, 576),
       (640, 128, 704), (768, 128, 800), (768, 128, 768), (768, 128, 736)]

CFG = dict(npre=0, kgr=(1, 4), n01=(3, 1), carry=1, r1=128, ktr1=(0, 1), ktr2=(1, 2), lnr=(1, 1), gg_at=3, xs_lag=8, fuse=1, flag=2, ffb=2, bw=[(0, 0), (20, 1), (44, 2)], hrows=320, wall=0, link=0, split=1, ktb=4, RU=16, gw=4, kt0=4, ffn_grp=(3, 1, 1), xsel_at=27, xw=22, kt_ln=4, pre=1, utpre=0, kdyn=1, ktag=0, kt_lag=1, utj=4, order=1, lag=1, lead=1, scopes=False)


def _kernel(x_hbm, are_hbm, aim_hbm, bre_hbm, bim_hbm, cre_hbm, cim_hbm, ldt_hbm, dsk_hbm,
            wr_hbm, wg_hbm, wu_hbm, wd_hbm, um_hbm, g0_hbm, out_hbm,
            zs, xb, prm, ldt, dsk, wr, wg, wu, wd, um, g0b, gm,
            umt, dtc, dkc, k0c, kd, xh, vv, ur0, ur1, ur2, yb, ob, junk, rs_s, oh_s, xs_s, hit_s, zmk, deff, updt_s, ya_s,
            sem_small, sem_w, sem_o, *ksps):
    urs = (ur0, ur1, ur2)
    _cur = [None]

    def mark(name):
        if not CFG["scopes"]:
            return
        if _cur[0] is not None:
            _cur[0].__exit__(None, None, None)
            _cur[0] = None
        if name:
            _cur[0] = jax.named_scope(name)
            _cur[0].__enter__()
    R1 = CFG["r1"]
    prs = [are_hbm, aim_hbm, bre_hbm, bim_hbm, cre_hbm, cim_hbm]
    order = (1, 0, 2, 3, 4, 5)
    grp0 = [(ldt_hbm, ldt)]
    grp1 = [(prs[i].at[pl.ds(0, R1)], prm.at[i, pl.ds(0, R1)]) for i in order]
    grp2 = [(prs[i].at[pl.ds(R1, D - R1)], prm.at[i, pl.ds(R1, D - R1)]) for i in order]
    grp2 += [(g0_hbm, g0b), (um_hbm, um), (dsk_hbm, dsk), (wr_hbm, wr)]
    grp3 = [(x_hbm, xb)]
    in_cp = []
    for grp in (grp0, grp1, grp2, grp3):
        n0 = sum(len(g) for g in in_cp)
        in_cp.append([pltpu.make_async_copy(s, d, sem_small.at[n0 + i]) for i, (s, d) in enumerate(grp)])
        for cp in in_cp[-1]:
            cp.start()
    w_cp = []
    off = 0
    for c, n in enumerate(FCH):
        cs = pl.ds(off * 128, n * 128)
        w_cp.append([pltpu.make_async_copy(h.at[:, cs], b.bitcast(BF16).at[:, cs], sem_w.at[i, c])
                     for i, (h, b) in enumerate([(wg_hbm, wg), (wu_hbm, wu), (wd_hbm, wd)])])
        for cp in w_cp[-1]:
            cp.start(priority=1)
        off += n

    class M:
        pass

    def masks():
        sub = lax.broadcasted_iota(I32, (8, 128), 0)
        lane = lax.broadcasted_iota(I32, (8, 128), 1)
        M.lo4 = sub < 4
        M.gidx = 4 * (lane % 32) + (sub % 4)
        M.lo64 = lane < 64
        M.beven = ((lane // 32) % 2) == 0
        M.last = lane == 127
        M.mz = jnp.where(lane == 0, 0.0, 1.0)
        M.row16 = lax.broadcasted_iota(I32, (16, 128), 0)
        M.lane16 = lax.broadcasted_iota(I32, (16, 128), 1)
    masks()

    mark('s0_wait0')
    in_cp[0][0].wait()
    mark('s1_prep')
    dtb = _col_bcast(ldt)
    for t in range(5):
        n = 128 if t < 4 else 64
        dtc[pl.ds(t * 128, n), :] = _rb(jnp.exp(dtb[t][:n]))
    mark('s2_waitp')
    for cp in in_cp[1]:
        cp.wait()
    mark('s3_A1')
    zo = []

    def dyn(r):
        return pl.multiple_of(zo[0] + r, 8)

    inB = [False]

    def kt_unit(b, c):
        l0, kk, g0 = _KT[c]
        gw = g0b[pl.ds(0, 128), :] if c == 0 else gm[pl.ds((g0 - 256) // 2, kk // 2), :]
        raw = _dot(_bf(kd[pl.ds(b * (RB // 2), RB // 2), pl.ds(l0, kk)]), _bf(gw))
        rows = pl.ds(dyn(0), RB) if inB[0] else pl.ds(0, RB)
        ksps[b][rows, pl.ds(512 * c, 512)] = raw
        if CFG["ktag"]:
            tg = pltpu.roll(ksps[b][pl.ds(0, 8), pl.ds(512 * c, 128)], 1, 1)
            junk[pl.ds(8 * ((b * NCH + c) % 8), 8), :] = tg

    def ggen():
        sel = pltpu.bitcast(g0b[pl.ds(128, 8), :], I32)

        def onehot(k, r0, n):
            ri = lax.broadcasted_iota(I32, (n, 256), 0) + r0
            return jnp.where(ri == sel[k:k + 1, :256], 1.0, 0.0)
        e = jnp.concatenate([onehot(0, 0, 128), onehot(1, 0, 64), onehot(2, 0, 32),
                             onehot(1, 112, 16), onehot(2, 112, 16), onehot(3, 112, 16)], axis=0).astype(BF16)
        g = _dot(e, _bf(g0b[pl.ds(0, 128), :]))

        def put(r, v):
            gm[pl.ds((r - 256) // 2, v.shape[0] // 2), :] = _u32(v)

        def zero(r, n):
            gm[pl.ds((r - 256) // 2, n // 2), :] = jnp.zeros((n // 2, 512), U32)
        zero(256, 112)
        put(368, g[256:272])
        put(384, g[0:128])
        put(512, g[128:192])
        zero(576, 48)
        put(624, g[224:240])
        put(640, g[128:192])
        put(704, g[192:224])
        zero(736, 80)
        put(816, g[240:256])
        put(832, g[192:224])
        zero(864, 64)

    def extract(st, o4):
        g = [[jnp.take_along_axis(_pk(o4[0][grp][8 * v:8 * v + 8], o4[1][grp][8 * v:8 * v + 8]), M.gidx, axis=1,
                                  mode="promise_in_bounds") for v in range(10)] for grp in range(2)]

        def mix(a, b):
            return jnp.where(M.lo4, a, b), pltpu.roll(jnp.where(M.lo4, b, a), 4, 0)

        def two(va, vb, m1, m2):
            p, q = mix(jnp.where(m1, g[0][va], g[0][vb]), jnp.where(m1, g[1][va], g[1][vb]))
            return jnp.where(m2, p, q)

        def four(gg):
            return jnp.where(M.lo64, jnp.where(M.beven, gg[2], gg[3]), jnp.where(M.beven, gg[4], gg[5]))
        t_odd = two(0, 1, M.lo64, M.beven)
        t_even, t_2 = mix(four(g[0]), four(g[1]))
        t_3 = two(6, 7, M.beven, M.lo64)
        t_4 = two(8, 9, M.lo64, M.beven)
        tl = [t_odd, t_even, t_2, jnp.where(M.last, t_2, t_3), t_3, jnp.where(M.last, t_3, t_4), t_4]
        for t in range(7):
            kd[pl.ds(st * 8, 8), pl.ds(128 * t, 128)] = tl[t]

    tk = {}

    def ln_chunk(j):
        cj = slice(256 * j, 256 * j + 256)
        s1 = s2 = None
        for i in range(NS):
            v16 = xb[pl.ds(i * 16, 16), cj].astype(F32)
            for v in (v16[:8], v16[8:]):
                s1, s2 = (v, v * v) if s1 is None else (s1 + v, s2 + v * v)
        mean = jnp.sum(s1, axis=0, keepdims=True) * (1.0 / D)
        var = jnp.sum(s2, axis=0, keepdims=True) * (1.0 / D) - mean * mean
        var = jnp.maximum(var, 0.0)
        sd = _rb(jnp.sqrt(_rb(_rb(var) + 1e-5)))
        mb = jnp.broadcast_to(_rb(mean), (16, 256))
        hi = jnp.broadcast_to(0.5 / sd, (16, 256))
        if j == 0:
            wrow = wr[...].astype(F32).reshape(1, D)
            tk["w"] = [(jnp.broadcast_to(wrow[:, k0:min(k0 + 128, D)], (16, min(128, D - k0)))
                        + jnp.zeros((16, min(128, D - k0)), F32)).astype(BF16) for k0 in range(0, D, 128)]
        r = None
        for i in range(NS):
            rw = pl.ds(dyn(i * 8), 8)
            hv = _rb(xb[pl.ds(i * 16, 16), cj].astype(F32) - mb) * hi
            h0, h1 = hv[:, :128], hv[:, 128:]
            xh[rw, pl.ds(256 * j, 128)] = _u32(h0)
            xh[rw, pl.ds(256 * j + 128, 128)] = _u32(h1)
            vv[pl.ds(i * 8, 8), pl.ds(256 * j, 128)] = _u32(h0 + h1)
            vv[pl.ds(i * 8, 8), pl.ds(256 * j + 128, 128)] = _u32(h0 - h1)
            if i % 8 == 7 or i == NS - 1:
                k0, k1 = (i // 8) * 128, (i + 1) * 16
                yield
                p = _dot(tk["w"][i // 8], _bf(xh[pl.ds(k0 // 2, (k1 - k0) // 2), cj]))
                r = p if r is None else r + p
        for t in range(2):
            r_t = r[:, 128 * t:128 * t + 128]
            tk["rc"] = r_t if (j == 0 and t == 0) else jnp.where(M.row16 == 2 * j + t, r_t, tk["rc"])

    def topk():
        bits = pltpu.bitcast(_rb(tk["rc"] * 2.0), I32)
        mono = (jnp.where(bits < 0, bits ^ 0x7FFF0000, bits) >> 16) + 32768
        key = pltpu.bitcast(0x30000000 + (mono << 11) + (2047 - (M.row16 * 128 + M.lane16)), F32)
        kcol = jnp.zeros((16, 128), I32)
        for j in range(NSEL):
            mx = jnp.max(jnp.max(key, axis=0, keepdims=True), axis=1, keepdims=True)
            mxb = jnp.broadcast_to(mx, (16, 128))
            key = jnp.where(key == mxb, 0.0, key)
            kcol = jnp.where(M.row16 == j, pltpu.bitcast(mxb, I32), kcol)
        kcol = kcol - 0x30000000
        idxcol = jnp.where(M.row16 < NSEL, 2047 - (kcol & 2047), -1)
        hb = ((kcol >> 11) - 32768) << 16
        rsel = pltpu.bitcast(jnp.where(hb < 0, hb ^ 0x7FFF0000, hb), F32)
        rsel = jnp.where(M.row16 < NSEL, rsel, 0.0)
        rs_s[...] = _rb(jax.nn.sigmoid(rsel))
        tk["oh"] = jnp.concatenate(
            [jnp.where(idxcol == M.lane16 + 128 * t, 1.0, 0.0) for t in range(16)], axis=1).astype(BF16)
        oh_s[...] = pltpu.bitcast(tk["oh"], U32)
        hb_ = jnp.where(M.row16[:8] < NSEL, jnp.left_shift(1, jnp.maximum(idxcol[:8], 0) >> 7), 0)
        for sh in (4, 2, 1):
            hb_ = hb_ | pltpu.roll(hb_, sh, 0)
        hit_s[0] = hb_[0, 0]

    def xsel(t):
        cs = slice(128 * t, 128 * t + 128)
        v = _dot_nt(tk["oh"][:, cs], _bf(xh[:, cs]))
        tk["xa"] = v if t == 0 else tk["xa"] + v
        if t == 15:
            xs_s[...] = _u32(tk["xa"] * 2.0)

    def link(v):
        if not CFG["link"]:
            return v
        w = pltpu.bitcast(v, U32)
        dep = ob[pl.ds(0, 8), pl.ds(0, 128)] & tk["zm"]
        return pltpu.bitcast(jnp.concatenate([w[:, :128] | dep, w[:, 128:]], axis=1), BF16)

    def ffn_gu(p, lk):
        cs = pl.ds(256 * p, 256)
        xs = link(tk["xs"]) if lk else tk["xs"]
        gu = _dot(xs, _bf(jnp.concatenate([wg[:, cs], wu[:, cs]], axis=1)))
        g = _rb(gu[:, :256])
        u = _rb(gu[:, 256:])
        sg = _rb(0.5 * jnp.tanh(0.5 * g) + 0.5)
        tk["h", p] = (_rb(g * sg) * u).astype(BF16)

    def ffn_dn(p, lk):
        h = tk.pop(("h", p))
        y = _dot_nt(link(h) if lk else h, _bf(wd[:, pl.ds(256 * p, 256)]))
        tk["y"] = y if p == 0 else tk["y"] + y

    def fin16(i, c0, c1, du, dynst):
        r16 = pl.ds(16 * i, 16)
        cs = pl.ds(128 * c0, 128 * (c1 - c0))
        h = _bf(xh[pl.ds(8 * i, 8), cs]).astype(F32)
        y = jnp.concatenate([_upk(yb[r16, pl.ds(256 * (c // 4) + 128 * (c % 2), 128)], (c // 2) % 2)
                             for c in range(c0, c1)], axis=1)
        dv = deff[r16, :]
        s_ = y + h * jnp.concatenate([dv] * (c1 - c0), axis=1)
        zh = h if du is None else h + du
        g = zh * jnp.tanh(zh) + zh
        rw = pl.ds(dyn(8 * i), 8) if dynst else pl.ds(8 * i, 8)
        ob[rw, cs] = _u32(xb[r16, cs].astype(F32) + s_ * g)

    utj = CFG["utj"]
    RU = CFG["RU"]

    def ut_piece(b, k, j0):
        rw = pl.ds(b * (RU // 2), RU // 2)
        rows = pl.ds(dyn(0), RU)
        ur = urs[b % 3]
        js = range(j0, j0 + utj)

        def lhs(ref, o):
            return _bf(jnp.concatenate([ref[rw, pl.ds(256 * j + o, 128)] for j in js], axis=0))

        def put(val, col):
            for i, j in enumerate(js):
                ur[rows, pl.ds(640 * j + col, 128)] = val[i * RU:(i + 1) * RU]
        if k == 0:
            v = _dot(lhs(vv, 0), _bf(um[:, 0:256]))
            b2 = _dot(lhs(vv, 128), _bf(um[:, 256:384]))
            a0 = v[:, :128]

            def sel(p, q):
                return jnp.concatenate([jnp.where(M.lo64, p[8 * i:8 * i + 8], q[8 * i:8 * i + 8])
                                        for i in range(a0.shape[0] // 8)], axis=0)
            put(sel(a0, b2), 0)
            put(v[:, 128:], 128)
            put(pltpu.roll(sel(b2, a0), 64, 1), 256)
        else:
            put(_dot(lhs(xh, 128), _bf(um[:, 384:512])), 384)
            put(_dot(lhs(xh, 0), _bf(um[:, 512:640])), 512)

    def mac(g, cls):
        ur = urs[(8 * g // RU) % 3]

        @functools.lru_cache(None)
        def us(j):
            def ld(c):
                return ur[pl.ds((8 * g) % RU, 8), pl.ds(640 * j + c, 128)]
            if cls == 0:
                a, b = ld(0), ld(256)
                return (a, b, a + b)
            t1, t2, t3 = ld(128), ld(384), ld(512)
            return (t1 + t2, t3 - t1, t2 + t3)

        @functools.lru_cache(None)
        def kraw(j):
            o = 512 * j + 256 * (1 - cls)
            ksp, kr = ksps[8 * g // RB], pl.ds((8 * g) % RB, 8)
            return ksp[kr, pl.ds(o, 128)], ksp[kr, pl.ds(o + 128, 128)]

        @functools.lru_cache(None)
        def ks(j):
            sr, si = kraw(j)
            if j > 0:
                pr, pi_ = kraw(j - 1)
                sr, si = (sr + pr, si + pi_) if cls == 0 else (sr - pr, si - pi_)
            return (sr * M.mz if cls == 0 else sr, si - sr, sr + si)
        outs = []
        prev = None
        for m in range(NCH):
            acc = None
            for j in range(m + 1):
                a, b, s = us(j)
                c_, e_, g_ = ks(m - j)
                t = (c_ * s, a * e_, b * g_)
                acc = t if acc is None else tuple(x + y for x, y in zip(acc, t))
            z = (acc[0] - acc[2], acc[0] + acc[1])
            if m % 2:
                za, zb = prev, z
                if cls == 0:
                    zr = _pk(za[0], zb[0])
                    zis = _pk(za[1], zb[1]) if CFG.get('nrz') else pltpu.roll(_pk(za[1], zb[1]), 64, 1)
                    outs.append((jnp.where(M.lo64, zr, zis), jnp.where(M.lo64, zis, zr)))
                else:
                    outs.append((_pk(za[0] + za[1], zb[0] + zb[1]), _pk(za[1], zb[1]), _pk(za[0], zb[0])))
            prev = z
        return outs

    zq, wq = {}, {}

    def inv(g, cls):
        zo_ = zq.pop((g, cls))

        def st(t):
            return _bf(jnp.concatenate([zo_[p][t] for p in range(4)], axis=0))
        if cls == 0:
            wq[g] = [_dot(st(t), _bf(umt[:, c:c + 128])) for t, c in ((0, 0), (1, 256))]
        else:
            q1, q2, q3 = [_dot(st(t), _bf(umt[:, c:c + 128])) for t, c in ((0, 128), (1, 384), (2, 512))]
            w0, w2 = wq.pop(g)
            p_ = q1 + w2
            y0 = p_ + (q2 + w0)
            y1 = (q3 + w0) - p_
            yr = pl.ds(dyn(8 * g), 8) if CFG["fuse"] else pl.ds(8 * g, 8)
            for p in range(4):
                yb[yr, pl.ds(256 * p, 128)] = _u32(y0[16 * p:16 * p + 16])
                yb[yr, pl.ds(256 * p + 128, 128)] = _u32(y1[16 * p:16 * p + 16])

    ktq = []
    slotno = [0]
    pat = CFG.get("kt_pat", [1, 0, 1, 1, 0, 1, 0, 1, 1, 0, 1, 1, 0, 1, 0, 1])
    xw = CFG["xw"]

    def kt_drain(n):
        for _ in range(n):
            if ktq and ktq[0][0] <= slotno[0]:
                kt_unit(*ktq.pop(0)[1:])

    utq = [(b, k, j) for b in range(D // RU) for j in range(0, NCH, utj) for k in range(2)]
    pend = [None]

    pre_xy = {}

    def kxy(st, half):
        r0 = st * 16
        pk = [pltpu.bitcast(prm[k, pl.ds(r0, 16), :], U32) for k in range(6)]
        rows = pl.ds(r0 + half, 8, stride=2)
        bs, k0 = _base8([_upk(w, half) for w in pk], dtc[rows, :])
        k0c[rows, :] = jnp.broadcast_to(k0, (8, 128))
        return [_grp_xy(bs, grp, M.lo4) for grp in range(2)]

    def kgen(s0, s1):
        for st in range(s0, s1):
            o4 = []
            for half in range(2):
                xy = pre_xy.pop((st, half)) if (st, half) in pre_xy else kxy(st, half)
                if half == 0 and pend[0] is not None:
                    flush()
                oo = []
                for grp in range(2):
                    yield
                    slotno[0] += 1
                    oo.append(_dot_nt(*xy[grp]))
                o4.append(oo)
            pend[0] = (st, o4)
        if s1 == NS or not CFG["carry"]:
            flush()
        else:
            for h in range(CFG["npre"]):
                pre_xy[(s1 + h // 2, h % 2)] = kxy(s1 + h // 2, h % 2)

    def flush():
        extract(*pend[0])
        if (pend[0][0] + 1) % SPB == 0:
            ktq.extend([(slotno[0] + 4 * CFG["kt_lag"], pend[0][0] // SPB, c) for c in range(NCH)])
        pend[0] = None

    def region(name, fn):
        def body():
            masks()
            mark(name)
            fn()
            mark(None)
        if CFG["split"]:
            pl.when(zs[0] == 0)(body)
        else:
            body()

    def consts():
        dkb = _col_bcast(dsk)
        for t in range(5):
            n = 128 if t < 4 else 64
            dkc[pl.ds(t * 128, n), :] = dkb[t][:n]
            mt = _bf(um[:, 128 * t:128 * t + 128]).T
            if t == 0:
                ri = lax.broadcasted_iota(I32, (128, 128), 0)
                ci = lax.broadcasted_iota(I32, (128, 128), 1)
                alt = jnp.where(ci % 2 == 1, 1.0, -1.0)
                mt = jnp.where(ri == 0, alt, jnp.where(ri == 64, 1.0, mt.astype(F32))).astype(BF16)
            umt[:, pl.ds(128 * t, 128)] = pltpu.bitcast(mt, U32)

    def rate(num, den):
        acc = [0]

        def step():
            acc[0] += num
            n = acc[0] // den
            acc[0] -= n * den
            return n
        return step

    only = CFG.get("only")
    doA = only in (None, "A")
    s1 = R1 // 16 - (CFG['npre'] + 1) // 2
    if doA:
        for _ in kgen(0, s1):
            pass
    mark('s3_w2')
    for cp in in_cp[2]:
        cp.wait()
    mark('s3_A1b')
    zs[0] = pltpu.bitcast(g0b[pl.ds(128, 8), pl.ds(384, 128)], I32)[0, 0]
    zo.append(zs[0] * 8)
    if doA:
        slotno[0] += 100
        ktr = rate(*CFG["ktr1"])
        for i, _ in enumerate(kgen(s1, xw)):
            if i == CFG["gg_at"]:
                ggen()
            if i > CFG["gg_at"]:
                kt_drain(ktr())
        consts()
    mark('s4_waitx')
    in_cp[3][0].wait()
    mark(None)

    def phase_a2():
        slotno[0] += 100
        kg = kgen(xw, NS)
        kgr = rate(*CFG["kgr"])
        for _ in range(CFG["pre"]):
            next(kg)
        for j in range(NCH):
            for k, _ in enumerate(ln_chunk(j)):
                kt_drain(CFG["n01"][0 if k == 0 else 1])
                for _ in range(kgr()):
                    next(kg)
        topk()
        ktr = rate(*CFG["ktr2"])
        xq = list(range(16))
        for i, _ in enumerate(kg):
            kt_drain(ktr())
            if i >= CFG["xs_lag"] and xq:
                xsel(xq.pop(0))
        while xq:
            xsel(xq.pop(0))
        slotno[0] += 1000
        kt_drain(len(ktq) - NCH)

    ffp = [0, 0]

    def ffn_next():
        if ffp[1] < ffp[0] - 1 or (ffp[1] < ffp[0] and ffp[0] >= ffp_max[0]):
            ffn_dn(ffp[1], False)
            ffp[1] += 1
        elif ffp[0] < ffp_max[0]:
            ffn_gu(ffp[0], False)
            ffp[0] += 1
    ffp_max = [0]

    def phase_b(g0, g1):
        inB[0] = True
        lag = CFG["lag"]
        NG = D // 8
        if g0 == 0:
            npre = 16 // utj + (2 * CFG["lead"] * 64 // RU) // utj
            for i in range(0 if CFG["utpre"] else npre):
                ut_piece(*utq.pop(0))
            if CFG["fuse"]:
                for t in range(5):
                    n = 128 if t < 4 else 64
                    deff[pl.ds(128 * t, n), :] = (dkc[pl.ds(128 * t, n), :] + k0c[pl.ds(128 * t, n), :]) * 2.0
        fl = CFG["flag"]
        for s in range(g0, g1):
            for cls in range(2):
                if s < NG:
                    zq[(s, cls)] = mac(s, cls)
                if CFG["order"] == 1 and lag <= s < NG + lag:
                    inv(s - lag, cls)
                if ((2 * s + cls) * 64 // RU) % utj == 0:
                    for _ in range(max(1, 64 // RU // utj)):
                        if utq:
                            ut_piece(*utq.pop(0))
                if cls == 1 and s % 4 == CFG["ktb"] % 4 and s >= CFG["ktb"]:
                    kt_drain(1)
                if CFG["order"] == 0 and lag <= s < NG + lag:
                    inv(s - lag, cls)
                if CFG["fuse"]:
                    q = 2 * (s - lag - fl) + cls - 2
                    if 0 <= q < 4 * NS:
                        fin16(q // 4, 4 * (q % 4), 4 * (q % 4) + 4, None, False)
                if CFG["ffb"] and cls == 0 and s % CFG["ffb"] == 0:
                    ffn_next()

    if only in (None, "A"):
        region('s5_A2', phase_a2)
    elif only == "B":
        ktq.extend([(0, NB - 1, c) for c in range(NCH)])
    HR = CFG["hrows"]
    obb = ob.bitcast(BF16)
    o_cp = [[pltpu.make_async_copy(obb.at[pl.ds(r0, n), pl.ds(128 * t, 128)],
                                   out_hbm.at[pl.ds(r0, n), pl.ds(128 * t, 128)], sem_o.at[hf, t])
             for t in range(16)] for hf, (r0, n) in enumerate([(0, HR), (HR, D - HR)])]

    def start_free(hf):
        hit = hit_s[0]
        for t in range(16):
            @pl.when(((hit >> t) & 1) == 0)
            def _():
                o_cp[hf][t].start(priority=1)

    GEND = D // 8 + CFG["lag"] + CFG["flag"] + 2
    if only in (None, "B"):
        def pb():
            g = 0
            for gs, cc in CFG["bw"]:
                if gs > g:
                    phase_b(g, gs)
                    g = gs
                if cc == len(CFG["bw"]) - 1 and only is None:
                    assert (2 * (gs - 1 - CFG["lag"] - CFG["flag"]) + 1 - 2 + 1) // 4 * 16 >= HR
                    start_free(0)
                mark(f's7_w{cc}')
                for cp in w_cp[cc]:
                    cp.wait()
                mark(f's7_B{cc}')
                ffp_max[0] = sum(FCH[:cc + 1]) // 2
                tk["xs"] = _bf(xs_s[...])
            phase_b(g, GEND)
            while CFG["ffb"] and ffp[1] < ffp_max[0]:
                ffn_next()
            if CFG["ffb"]:
                ya_s[...] = tk["y"]
        region('s7_B', pb)
    if only in ("A", "B"):
        for cc in range(len(CFG["bw"]), len(FCH)):
            for cp in w_cp[cc]:
                cp.wait()
        cp = pltpu.make_async_copy(ob.bitcast(BF16), out_hbm, sem_o.at[0, 0])
        cp.start()
        cp.wait()
        cp = pltpu.make_async_copy(yb.bitcast(BF16).at[pl.ds(0, D), :], out_hbm.at[:, pl.ds(0, 1024)], sem_o.at[0, 0])
        cp.start()
        cp.wait()
        for kk in ksps:
            cp = pltpu.make_async_copy(kk.at[:, pl.ds(0, 512)], junk.at[:, pl.ds(0, 512)], sem_o.at[0, 0])
            cp.start()
            cp.wait()
        for kk in (vv, xs_s, kd, umt):
            cp = pltpu.make_async_copy(kk.at[pl.ds(0, 8), pl.ds(0, 512)], oh_s.at[:, pl.ds(0, 512)], sem_o.at[0, 0])
            cp.start()
            cp.wait()
        cp = pltpu.make_async_copy(ya_s, junk.at[pl.ds(0,16), :], sem_o.at[0, 0])
        cp.start()
        cp.wait()
        return
    masks()
    tk["xs"] = _bf(xs_s[...])
    tk["rs"] = rs_s[...]
    tk["oh"] = _bf(oh_s[...])

    mark('s8_ffn')
    start_free(1)
    tk["y"] = ya_s[...]
    for cc in range(len(CFG["bw"]), len(FCH)):
        if cc == len(CFG["bw"]) or not CFG["wall"]:
            for c2 in (range(cc, len(FCH)) if CFG["wall"] else [cc]):
                mark(f's8_w{c2}')
                for cp in w_cp[c2]:
                    cp.wait()
                mark(f's8_f{c2}')
        ffp_max[0] = sum(FCH[:cc + 1]) // 2
        while ffp[0] < ffp_max[0]:
            ffn_gu(ffp[0], False)
            ffp[0] += 1
            if ffp[1] < ffp[0] - 1:
                ffn_dn(ffp[1], False)
                ffp[1] += 1
    while ffp[1] < ffp[0]:
        ffn_dn(ffp[1], False)
        ffp[1] += 1
    rs = jnp.concatenate([tk["rs"]] * 5, axis=1)[:, :D]
    upd = (_rb(_rb(tk["y"]) * rs) * 0.5).astype(BF16)
    updt_s[...] = _u32(lax.dot_general(upd, jnp.eye(16, 256, dtype=BF16), (((0,), (0,)), ((), ())),
                                       preferred_element_type=F32))
    mark('s9_final')
    hit = hit_s[0]
    for t in range(16):
        @pl.when(((hit >> t) & 1) == 1)
        def _():
            ohp = jnp.concatenate([_bf(oh_s[:, pl.ds(128 * t, 128)]), jnp.zeros((112, 128), BF16)], axis=0)
            du = _dot(_bf(updt_s[:, pl.ds(0, 128)]), ohp)
            for i in range(NS):
                fin16(i, t, t + 1, du[16 * i:16 * i + 16], False)
            for hf in range(2):
                o_cp[hf][t].start(priority=1)
    mark('sa_waito')
    for cps in o_cp:
        for cp in cps:
            cp.wait()
    mark(None)


@jax.jit
def pallas_recurrent_scan__ssm_conv_s4__moe_arch_mod__prompt_kernel(A_u, A_A_re, A_A_im, A_B_re, A_B_im, A_C_re, A_C_im, A_log_dt, A_Dskip,
              B_x, B_w_r, B_w_gate, B_w_up, B_w_down):
    xt = jnp.transpose(A_u[0])
    wdt = jnp.transpose(B_w_down)
    scratch = [
        pltpu.SMEM((1,), I32),
        pltpu.VMEM((D, L), BF16),
        pltpu.VMEM((6, D, N), BF16),
        pltpu.VMEM((D,), BF16),
        pltpu.VMEM((D,), BF16),
        pltpu.VMEM((D,), BF16),
        pltpu.VMEM((D // 2, FF), U32),
        pltpu.VMEM((D // 2, FF), U32),
        pltpu.VMEM((D // 2, FF), U32),
        pltpu.VMEM(_UM.shape, U32),
        pltpu.VMEM(_G0.shape, U32),
        pltpu.VMEM((336, 512), U32),
        pltpu.VMEM(_UM.shape, U32),
        pltpu.VMEM((D, 128), F32),
        pltpu.VMEM((D, 128), F32),
        pltpu.VMEM((D, 128), F32),
        pltpu.VMEM((D // 2, 896), U32),
        pltpu.VMEM((D // 2, L), U32),
        pltpu.VMEM((D // 2, L), U32),
        pltpu.VMEM((CFG['RU'], 5120), F32),
        pltpu.VMEM((CFG['RU'], 5120), F32),
        pltpu.VMEM((CFG['RU'], 5120), F32),
        pltpu.VMEM((D, L // 2), U32),
        pltpu.VMEM((D // 2, L), U32),
        pltpu.VMEM((64, D), F32),
        pltpu.VMEM((16, 128), F32),
        pltpu.VMEM((8, L), U32),
        pltpu.VMEM((8, D), U32),
        pltpu.SMEM((1,), I32),
        pltpu.VMEM((8, 128), U32),
        pltpu.VMEM((D, 128), F32),
        pltpu.VMEM((D // 2, 256), U32),
        pltpu.VMEM((16, D), F32),
        pltpu.SemaphoreType.DMA((18,)),
        pltpu.SemaphoreType.DMA((3, len(FCH))),
        pltpu.SemaphoreType.DMA((2, 16)),
    ] + [pltpu.VMEM((RB, 4096), F32)] * NB
    out = pl.pallas_call(
        _kernel,
        out_shape=jax.ShapeDtypeStruct((D, L), BF16),
        in_specs=[pl.BlockSpec(memory_space=pl.ANY)] * 15,
        out_specs=pl.BlockSpec(memory_space=pl.ANY),
        scratch_shapes=scratch,
        compiler_params=pltpu.CompilerParams(vmem_limit_bytes=100 * 2**20, disable_semaphore_checks=True,
                                             disable_bounds_checks=True),
        name="s4_mod",
    )(xt, A_A_re, A_A_im, A_B_re, A_B_im, A_C_re, A_C_im, A_log_dt, A_Dskip,
      B_w_r, B_w_gate, B_w_up, wdt, jnp.asarray(_UM), jnp.asarray(_G0))
    return jnp.transpose(out)[None]
```

```python
import functools
import math

import numpy as np
import jax
import jax.numpy as jnp
from jax import lax
import jax.experimental.pallas as pl
import jax.experimental.pallas.tpu as pltpu

F32 = jnp.float32
BF16 = jnp.bfloat16
U32 = jnp.uint32
I32 = jnp.int32

D = 576
L = 2048
N = 128
FF = 4608
NSEL = 8
NCH = 8
RB = 64
NB = D // RB
NS = D // 16
SPB = RB // 16
FCH = (10, 10, 8, 6, 2)

_TILES = {
    "odd": (1, 3, 5, 7),
    "even": (2, 4, 6, 8),
    "t2": (258, 260, 262, 264),
    "t3": (516, 520, 772, 776),
    "t4": (1032, 1288, 1544, 1800),
}


def _rlag(l):
    u = int(np.float32(l).view(np.uint32))
    u = (u + 0x7FFF + ((u >> 16) & 1)) & 0xFFFF0000
    return int(np.uint32(u).view(np.float32))


def _tile_pts(name):
    base = name.rstrip("v")
    p = np.array([_TILES[base][l // 32] + 8 * (l % 32) for l in range(128)])
    if name == "t3v":
        p[127] = 512
    if name == "t4v":
        p[127] = 1024
    return p


def _fdk_row(r):
    f1 = 4 * np.arange(128) + 1
    f02 = np.concatenate([4 * np.arange(64), 4 * np.arange(64) + 2])
    w = 2 * np.pi / 512
    sgn = (-1.0) ** r
    r02 = np.cos(w * f02 * r)
    i02 = -np.sin(w * f02 * r)
    r02[0] = (-sgn - 1.0) / 4.0
    i02[0] = (1.0 - sgn) / 4.0
    return np.concatenate([np.cos(w * f1 * r), -np.sin(w * f1 * r), r02, i02]) / 128.0


def _gmat(c, tile):
    pts = _tile_pts(tile)
    g = np.zeros((128, 512))
    for r in range(1, 257):
        idx = np.nonzero(pts == _rlag(256 * c + r))[0]
        if len(idx):
            g[idx[0]] += _fdk_row(r)
    return g


def _pack_bf16(a):
    u = np.ascontiguousarray(a, np.float32).view(np.uint32)
    u = ((u + 0x7FFF + ((u >> 16) & 1)) >> 16).astype(np.uint32)
    return (u[0::2] | (u[1::2] << 16)).astype(np.uint32)


def _tables():
    f1 = 4 * np.arange(128) + 1
    w = 2 * np.pi / 512
    t = np.arange(128)[:, None] + 1
    a = np.cos(w * f1 * t)
    b = -np.sin(w * f1 * t)
    f0 = 4 * np.arange(64)
    f2 = f0 + 2
    m0 = np.concatenate([np.cos(w * f0 * t), -np.sin(w * f0 * t)], axis=1)
    m2 = np.concatenate([-np.sin(w * f2 * t), np.cos(w * f2 * t)], axis=1)
    m0[:, 64] = (-1.0) ** t[:, 0]
    um = np.concatenate([m0, a, m2, b - a, a + b], axis=1)
    g0 = np.concatenate([_gmat(0, "odd"), _gmat(0, "even")], axis=0)
    lags = np.concatenate([_tile_pts("odd"), _tile_pts("even")])
    sel = np.full((8, 256), -1, np.int32)
    for k, (c, tile) in enumerate([(1, "t2"), (2, "t3v"), (4, "t4v"), (1, "even")]):
        pts = _tile_pts(tile)
        for rho, r in enumerate(lags):
            idx = np.nonzero(pts == _rlag(256 * c + int(r)))[0]
            if len(idx):
                sel[k, rho] = idx[0]
    selp = np.zeros((8, 512), np.int32)
    selp[:, :256] = sel
    return _pack_bf16(um), np.concatenate([_pack_bf16(g0), selp.view(np.uint32)], axis=0)


_UM, _G0 = _tables()


def _bf(x):
    return pltpu.bitcast(x, BF16)


def _u32(x):
    return pltpu.bitcast(x.astype(BF16), U32)


def _rb(x):
    return x.astype(BF16).astype(F32)


def _cmul(a, b):
    return (a[0] * b[0] - a[1] * b[1], a[0] * b[1] + a[1] * b[0])


def _csq(a):
    t = a[0] * a[1]
    return (a[0] * a[0] - a[1] * a[1], t + t)


def _sincos(th):
    magic = 12582912.0
    kf = th * (2.0 / math.pi) + magic
    ki = pltpu.bitcast(kf, I32)
    k = kf - magic
    r = th - k * 1.5703125
    r = r - k * 4.837512969970703125e-4
    r = r - k * 7.54978995489188216e-8
    r2 = r * r
    s = r + r * r2 * (-1.6666654611e-1 + r2 * (8.3321608736e-3 + r2 * -1.9515295891e-4))
    c = 1.0 + r2 * (-0.5 + r2 * (4.166664568298827e-2 + r2 * (-1.388731625493765e-3 + r2 * 2.443315711809948e-5)))
    swap = (ki & 1) == 1
    sn = jnp.where(swap, c, s)
    cs = jnp.where(swap, s, c)
    sbit = (ki & 2) << 30
    cbit = ((ki + 1) & 2) << 30
    sn = pltpu.bitcast(pltpu.bitcast(sn, I32) ^ sbit, F32)
    cs = pltpu.bitcast(pltpu.bitcast(cs, I32) ^ cbit, F32)
    return cs, sn


def _dot(a, b):
    return jnp.dot(a, b, preferred_element_type=F32)


def _dot_nt(a, b):
    return lax.dot_general(a, b, (((1,), (1,)), ((), ())), preferred_element_type=F32)


def _col_bcast(vec_ref):
    v = vec_ref[...].astype(F32).reshape(1, D)
    vp = jnp.concatenate([v, jnp.zeros((1, 64), F32)], axis=1)
    return [jnp.broadcast_to(vp[:, t * 128:(t + 1) * 128], (128, 128)).T for t in range(5)]


def _base8(p, dt):
    are, aim, bre, bim, cre, cim = p
    y1 = (dt * are) * math.log2(math.e)
    ph = {1: _sincos(dt * aim)}
    e = 1
    while e < 512:
        ph[2 * e] = _csq(ph[e])
        e *= 2
    pw = {}
    for e in (1, 2, 4, 8, 16, 256, 512):
        mg = jnp.exp2(y1 * float(e)) if e > 1 else jnp.exp2(y1)
        pw[e] = (mg * ph[e][0], mg * ph[e][1])
    w = _cmul((cre, cim), (dt * bre, dt * bim))
    k0 = jnp.sum(w[0], axis=1, keepdims=True)
    w1 = _cmul(w, pw[1])
    w2 = _cmul(w1, pw[1])
    w3 = _cmul(w2, pw[1])
    w258 = _cmul(w2, pw[256])

    def rot(z):
        return (pltpu.roll(z[0], 4, 0), pltpu.roll(z[1], 4, 0))
    rots = {e: rot(pw[e]) for e in (2, 4, 8, 16, 512)}
    return (pw, rots, w1, w2, rot(w3), rot(w258)), k0


def _grp_xy(bs, grp, lo4):
    pw, rots, w1, w2, w3r, w258r = bs

    def sel(lo, hi):
        return (jnp.where(lo4, lo[0], hi[0]), jnp.where(lo4, lo[1], hi[1]))
    if grp == 0:
        dup = {e: sel(pw[e], rots[e]) for e in (2, 4, 16, 512)}
        x0, x2, a8 = sel(w1, w3r), sel(w2, w258r), rots[8]
    else:
        dup = {e: sel(rots[e], pw[e]) for e in (2, 4, 16, 512)}
        x0, x2, a8 = sel(w3r, w1), sel(w258r, w2), pw[8]
    xv = [None] * 10
    xv[0] = x0
    xv[1] = _cmul(x0, dup[4])
    xv[2] = x2
    xv[3] = _cmul(xv[2], dup[2])
    xv[4] = _cmul(xv[3], dup[2])
    xv[5] = _cmul(xv[4], dup[2])
    xv[6] = _cmul(xv[3], dup[512])
    xv[7] = _cmul(xv[5], dup[512])
    xv[8] = _cmul(xv[7], dup[512])
    xv[9] = _cmul(xv[8], dup[512])
    y = (jnp.where(lo4, 1.0, a8[0]), jnp.where(lo4, 0.0, -a8[1]))
    m = dup[16]
    ys = [y]
    for _ in range(15):
        y = (y[0] * m[0] + y[1] * m[1], y[1] * m[0] - y[0] * m[1])
        ys.append(y)

    def mat(vs):
        return jnp.concatenate([jnp.concatenate([v[0] for v in vs], 0),
                                jnp.concatenate([v[1] for v in vs], 0)], 1).astype(BF16)
    return mat(xv), mat(ys)


def _pk(a, b):
    return pltpu.pack_elementwise([a, b], packed_dtype=BF16)


def _upk(w, h):
    return pltpu.unpack_elementwise(w, index=h, packed_dtype=BF16, unpacked_dtype=F32)


_KT = [(0, 256, 0), (128, 256, 256), (384, 128, 512), (512, 128, 576),
       (640, 128, 704), (768, 128, 800), (768, 128, 768), (768, 128, 736)]

CFG = dict(npre=0, kgr=(1, 4), n01=(3, 1), carry=1, r1=128, ktr1=(0, 1), ktr2=(1, 2), lnr=(1, 1), gg_at=3, xs_lag=8, fuse=1, flag=2, ffb=2, bw=[(0, 0), (20, 1), (44, 2)], hrows=0, wall=0, link=0, split=1, ktb=4, RU=16, gw=4, kt0=4, ffn_grp=(3, 1, 1), xsel_at=27, xw=22, kt_ln=4, pre=1, utpre=0, kdyn=1, ktag=0, kt_lag=1, utj=4, order=1, lag=1, lead=1, scopes=False)


def _kernel(x_hbm, are_hbm, aim_hbm, bre_hbm, bim_hbm, cre_hbm, cim_hbm, ldt_hbm, dsk_hbm,
            wr_hbm, wg_hbm, wu_hbm, wd_hbm, um_hbm, g0_hbm, out_hbm,
            zs, xb, prm, ldt, dsk, wr, wg, wu, wd, um, g0b, gm,
            umt, dtc, dkc, k0c, kd, xh, vv, ur0, ur1, ur2, yb, ob, junk, rs_s, oh_s, xs_s, hit_s, zmk, deff, updt_s, ya_s,
            sem_small, sem_w, sem_o, *ksps):
    urs = (ur0, ur1, ur2)
    _cur = [None]

    def mark(name):
        if not CFG["scopes"]:
            return
        if _cur[0] is not None:
            _cur[0].__exit__(None, None, None)
            _cur[0] = None
        if name:
            _cur[0] = jax.named_scope(name)
            _cur[0].__enter__()
    R1 = CFG["r1"]
    prs = [are_hbm, aim_hbm, bre_hbm, bim_hbm, cre_hbm, cim_hbm]
    order = (1, 0, 2, 3, 4, 5)
    grp0 = [(ldt_hbm, ldt)]
    grp1 = [(prs[i].at[pl.ds(0, R1)], prm.at[i, pl.ds(0, R1)]) for i in order]
    grp2 = [(prs[i].at[pl.ds(R1, D - R1)], prm.at[i, pl.ds(R1, D - R1)]) for i in order]
    grp2 += [(g0_hbm, g0b), (um_hbm, um), (dsk_hbm, dsk), (wr_hbm, wr)]
    grp3 = [(x_hbm, xb)]
    in_cp = []
    for grp in (grp0, grp1, grp2, grp3):
        n0 = sum(len(g) for g in in_cp)
        in_cp.append([pltpu.make_async_copy(s, d, sem_small.at[n0 + i]) for i, (s, d) in enumerate(grp)])
        for cp in in_cp[-1]:
            cp.start()
    w_cp = []
    off = 0
    for c, n in enumerate(FCH):
        cs = pl.ds(off * 128, n * 128)
        w_cp.append([pltpu.make_async_copy(h.at[:, cs], b.bitcast(BF16).at[:, cs], sem_w.at[i, c])
                     for i, (h, b) in enumerate([(wg_hbm, wg), (wu_hbm, wu), (wd_hbm, wd)])])
        for cp in w_cp[-1]:
            cp.start(priority=1)
        off += n

    class M:
        pass

    def masks():
        sub = lax.broadcasted_iota(I32, (8, 128), 0)
        lane = lax.broadcasted_iota(I32, (8, 128), 1)
        M.lo4 = sub < 4
        M.gidx = 4 * (lane % 32) + (sub % 4)
        M.lo64 = lane < 64
        M.beven = ((lane // 32) % 2) == 0
        M.last = lane == 127
        M.mz = jnp.where(lane == 0, 0.0, 1.0)
        M.row16 = lax.broadcasted_iota(I32, (16, 128), 0)
        M.lane16 = lax.broadcasted_iota(I32, (16, 128), 1)
    masks()

    mark('s0_wait0')
    in_cp[0][0].wait()
    mark('s1_prep')
    dtb = _col_bcast(ldt)
    for t in range(5):
        n = 128 if t < 4 else 64
        dtc[pl.ds(t * 128, n), :] = _rb(jnp.exp(dtb[t][:n]))
    mark('s2_waitp')
    for cp in in_cp[1]:
        cp.wait()
    mark('s3_A1')
    zo = []

    def dyn(r):
        return pl.multiple_of(zo[0] + r, 8)

    inB = [False]

    def kt_unit(b, c):
        l0, kk, g0 = _KT[c]
        gw = g0b[pl.ds(0, 128), :] if c == 0 else gm[pl.ds((g0 - 256) // 2, kk // 2), :]
        raw = _dot(_bf(kd[pl.ds(b * (RB // 2), RB // 2), pl.ds(l0, kk)]), _bf(gw))
        rows = pl.ds(dyn(0), RB) if inB[0] else pl.ds(0, RB)
        ksps[b][rows, pl.ds(512 * c, 512)] = raw
        if CFG["ktag"]:
            tg = pltpu.roll(ksps[b][pl.ds(0, 8), pl.ds(512 * c, 128)], 1, 1)
            junk[pl.ds(8 * ((b * NCH + c) % 8), 8), :] = tg

    def ggen():
        sel = pltpu.bitcast(g0b[pl.ds(128, 8), :], I32)

        def onehot(k, r0, n):
            ri = lax.broadcasted_iota(I32, (n, 256), 0) + r0
            return jnp.where(ri == sel[k:k + 1, :256], 1.0, 0.0)
        e = jnp.concatenate([onehot(0, 0, 128), onehot(1, 0, 64), onehot(2, 0, 32),
                             onehot(1, 112, 16), onehot(2, 112, 16), onehot(3, 112, 16)], axis=0).astype(BF16)
        g = _dot(e, _bf(g0b[pl.ds(0, 128), :]))

        def put(r, v):
            gm[pl.ds((r - 256) // 2, v.shape[0] // 2), :] = _u32(v)

        def zero(r, n):
            gm[pl.ds((r - 256) // 2, n // 2), :] = jnp.zeros((n // 2, 512), U32)
        zero(256, 112)
        put(368, g[256:272])
        put(384, g[0:128])
        put(512, g[128:192])
        zero(576, 48)
        put(624, g[224:240])
        put(640, g[128:192])
        put(704, g[192:224])
        zero(736, 80)
        put(816, g[240:256])
        put(832, g[192:224])
        zero(864, 64)

    def extract(st, o4):
        g = [[jnp.take_along_axis(_pk(o4[0][grp][8 * v:8 * v + 8], o4[1][grp][8 * v:8 * v + 8]), M.gidx, axis=1,
                                  mode="promise_in_bounds") for v in range(10)] for grp in range(2)]

        def mix(a, b):
            return jnp.where(M.lo4, a, b), pltpu.roll(jnp.where(M.lo4, b, a), 4, 0)

        def two(va, vb, m1, m2):
            p, q = mix(jnp.where(m1, g[0][va], g[0][vb]), jnp.where(m1, g[1][va], g[1][vb]))
            return jnp.where(m2, p, q)

        def four(gg):
            return jnp.where(M.lo64, jnp.where(M.beven, gg[2], gg[3]), jnp.where(M.beven, gg[4], gg[5]))
        t_odd = two(0, 1, M.lo64, M.beven)
        t_even, t_2 = mix(four(g[0]), four(g[1]))
        t_3 = two(6, 7, M.beven, M.lo64)
        t_4 = two(8, 9, M.lo64, M.beven)
        tl = [t_odd, t_even, t_2, jnp.where(M.last, t_2, t_3), t_3, jnp.where(M.last, t_3, t_4), t_4]
        for t in range(7):
            kd[pl.ds(st * 8, 8), pl.ds(128 * t, 128)] = tl[t]

    tk = {}

    def ln_chunk(j):
        cj = slice(256 * j, 256 * j + 256)
        s1 = s2 = None
        for i in range(NS):
            v16 = xb[pl.ds(i * 16, 16), cj].astype(F32)
            for v in (v16[:8], v16[8:]):
                s1, s2 = (v, v * v) if s1 is None else (s1 + v, s2 + v * v)
        mean = jnp.sum(s1, axis=0, keepdims=True) * (1.0 / D)
        var = jnp.sum(s2, axis=0, keepdims=True) * (1.0 / D) - mean * mean
        var = jnp.maximum(var, 0.0)
        sd = _rb(jnp.sqrt(_rb(_rb(var) + 1e-5)))
        mb = jnp.broadcast_to(_rb(mean), (16, 256))
        hi = jnp.broadcast_to(0.5 / sd, (16, 256))
        if j == 0:
            wrow = wr[...].astype(F32).reshape(1, D)
            tk["w"] = [(jnp.broadcast_to(wrow[:, k0:min(k0 + 128, D)], (16, min(128, D - k0)))
                        + jnp.zeros((16, min(128, D - k0)), F32)).astype(BF16) for k0 in range(0, D, 128)]
        r = None
        for i in range(NS):
            rw = pl.ds(dyn(i * 8), 8)
            hv = _rb(xb[pl.ds(i * 16, 16), cj].astype(F32) - mb) * hi
            h0, h1 = hv[:, :128], hv[:, 128:]
            xh[rw, pl.ds(256 * j, 128)] = _u32(h0)
            xh[rw, pl.ds(256 * j + 128, 128)] = _u32(h1)
            vv[pl.ds(i * 8, 8), pl.ds(256 * j, 128)] = _u32(h0 + h1)
            vv[pl.ds(i * 8, 8), pl.ds(256 * j + 128, 128)] = _u32(h0 - h1)
            if i % 8 == 7 or i == NS - 1:
                k0, k1 = (i // 8) * 128, (i + 1) * 16
                yield
                p = _dot(tk["w"][i // 8], _bf(xh[pl.ds(k0 // 2, (k1 - k0) // 2), cj]))
                r = p if r is None else r + p
        for t in range(2):
            r_t = r[:, 128 * t:128 * t + 128]
            tk["rc"] = r_t if (j == 0 and t == 0) else jnp.where(M.row16 == 2 * j + t, r_t, tk["rc"])

    def topk():
        bits = pltpu.bitcast(_rb(tk["rc"] * 2.0), I32)
        mono = (jnp.where(bits < 0, bits ^ 0x7FFF0000, bits) >> 16) + 32768
        key = pltpu.bitcast(0x30000000 + (mono << 11) + (2047 - (M.row16 * 128 + M.lane16)), F32)
        kcol = jnp.zeros((16, 128), I32)
        for j in range(NSEL):
            mx = jnp.max(jnp.max(key, axis=0, keepdims=True), axis=1, keepdims=True)
            mxb = jnp.broadcast_to(mx, (16, 128))
            key = jnp.where(key == mxb, 0.0, key)
            kcol = jnp.where(M.row16 == j, pltpu.bitcast(mxb, I32), kcol)
        kcol = kcol - 0x30000000
        idxcol = jnp.where(M.row16 < NSEL, 2047 - (kcol & 2047), -1)
        hb = ((kcol >> 11) - 32768) << 16
        rsel = pltpu.bitcast(jnp.where(hb < 0, hb ^ 0x7FFF0000, hb), F32)
        rsel = jnp.where(M.row16 < NSEL, rsel, 0.0)
        rs_s[...] = _rb(jax.nn.sigmoid(rsel))
        tk["oh"] = jnp.concatenate(
            [jnp.where(idxcol == M.lane16 + 128 * t, 1.0, 0.0) for t in range(16)], axis=1).astype(BF16)
        oh_s[...] = pltpu.bitcast(tk["oh"], U32)
        hb_ = jnp.where(M.row16[:8] < NSEL, jnp.left_shift(1, jnp.maximum(idxcol[:8], 0) >> 7), 0)
        for sh in (4, 2, 1):
            hb_ = hb_ | pltpu.roll(hb_, sh, 0)
        hit_s[0] = hb_[0, 0]

    def xsel(t):
        cs = slice(128 * t, 128 * t + 128)
        v = _dot_nt(tk["oh"][:, cs], _bf(xh[:, cs]))
        tk["xa"] = v if t == 0 else tk["xa"] + v
        if t == 15:
            xs_s[...] = _u32(tk["xa"] * 2.0)

    def link(v):
        if not CFG["link"]:
            return v
        w = pltpu.bitcast(v, U32)
        dep = ob[pl.ds(0, 8), pl.ds(0, 128)] & tk["zm"]
        return pltpu.bitcast(jnp.concatenate([w[:, :128] | dep, w[:, 128:]], axis=1), BF16)

    def ffn_gu(p, lk):
        cs = pl.ds(256 * p, 256)
        xs = link(tk["xs"]) if lk else tk["xs"]
        gu = _dot(xs, _bf(jnp.concatenate([wg[:, cs], wu[:, cs]], axis=1)))
        g = _rb(gu[:, :256])
        u = _rb(gu[:, 256:])
        sg = _rb(0.5 * jnp.tanh(0.5 * g) + 0.5)
        tk["h", p] = (_rb(g * sg) * u).astype(BF16)

    def ffn_dn(p, lk):
        h = tk.pop(("h", p))
        y = _dot_nt(link(h) if lk else h, _bf(wd[:, pl.ds(256 * p, 256)]))
        tk["y"] = y if p == 0 else tk["y"] + y

    def fin16(i, c0, c1, du, dynst):
        r16 = pl.ds(16 * i, 16)
        cs = pl.ds(128 * c0, 128 * (c1 - c0))
        h = _bf(xh[pl.ds(8 * i, 8), cs]).astype(F32)
        y = jnp.concatenate([_upk(yb[r16, pl.ds(256 * (c // 4) + 128 * (c % 2), 128)], (c // 2) % 2)
                             for c in range(c0, c1)], axis=1)
        dv = deff[r16, :]
        s_ = y + h * jnp.concatenate([dv] * (c1 - c0), axis=1)
        zh = h if du is None else h + du
        g = zh * jnp.tanh(zh) + zh
        rw = pl.ds(dyn(8 * i), 8) if dynst else pl.ds(8 * i, 8)
        ob[rw, cs] = _u32(xb[r16, cs].astype(F32) + s_ * g)

    utj = CFG["utj"]
    RU = CFG["RU"]

    def ut_piece(b, k, j0):
        rw = pl.ds(b * (RU // 2), RU // 2)
        rows = pl.ds(dyn(0), RU)
        ur = urs[b % 3]
        js = range(j0, j0 + utj)

        def lhs(ref, o):
            return _bf(jnp.concatenate([ref[rw, pl.ds(256 * j + o, 128)] for j in js], axis=0))

        def put(val, col):
            for i, j in enumerate(js):
                ur[rows, pl.ds(640 * j + col, 128)] = val[i * RU:(i + 1) * RU]
        if k == 0:
            v = _dot(lhs(vv, 0), _bf(um[:, 0:256]))
            b2 = _dot(lhs(vv, 128), _bf(um[:, 256:384]))
            a0 = v[:, :128]

            def sel(p, q):
                return jnp.concatenate([jnp.where(M.lo64, p[8 * i:8 * i + 8], q[8 * i:8 * i + 8])
                                        for i in range(a0.shape[0] // 8)], axis=0)
            put(sel(a0, b2), 0)
            put(v[:, 128:], 128)
            put(pltpu.roll(sel(b2, a0), 64, 1), 256)
        else:
            put(_dot(lhs(xh, 128), _bf(um[:, 384:512])), 384)
            put(_dot(lhs(xh, 0), _bf(um[:, 512:640])), 512)

    def mac(g, cls):
        ur = urs[(8 * g // RU) % 3]

        @functools.lru_cache(None)
        def us(j):
            def ld(c):
                return ur[pl.ds((8 * g) % RU, 8), pl.ds(640 * j + c, 128)]
            if cls == 0:
                a, b = ld(0), ld(256)
                return (a, b, a + b)
            t1, t2, t3 = ld(128), ld(384), ld(512)
            return (t1 + t2, t3 - t1, t2 + t3)

        @functools.lru_cache(None)
        def kraw(j):
            o = 512 * j + 256 * (1 - cls)
            ksp, kr = ksps[8 * g // RB], pl.ds((8 * g) % RB, 8)
            return ksp[kr, pl.ds(o, 128)], ksp[kr, pl.ds(o + 128, 128)]

        @functools.lru_cache(None)
        def ks(j):
            sr, si = kraw(j)
            if j > 0:
                pr, pi_ = kraw(j - 1)
                sr, si = (sr + pr, si + pi_) if cls == 0 else (sr - pr, si - pi_)
            return (sr * M.mz if cls == 0 else sr, si - sr, sr + si)
        outs = []
        prev = None
        for m in range(NCH):
            acc = None
            for j in range(m + 1):
                a, b, s = us(j)
                c_, e_, g_ = ks(m - j)
                t = (c_ * s, a * e_, b * g_)
                acc = t if acc is None else tuple(x + y for x, y in zip(acc, t))
            z = (acc[0] - acc[2], acc[0] + acc[1])
            if m % 2:
                za, zb = prev, z
                if cls == 0:
                    zr = _pk(za[0], zb[0])
                    zis = _pk(za[1], zb[1]) if CFG.get('nrz') else pltpu.roll(_pk(za[1], zb[1]), 64, 1)
                    outs.append((jnp.where(M.lo64, zr, zis), jnp.where(M.lo64, zis, zr)))
                else:
                    outs.append((_pk(za[0] + za[1], zb[0] + zb[1]), _pk(za[1], zb[1]), _pk(za[0], zb[0])))
            prev = z
        return outs

    zq, wq = {}, {}

    def inv(g, cls):
        zo_ = zq.pop((g, cls))

        def st(t):
            return _bf(jnp.concatenate([zo_[p][t] for p in range(4)], axis=0))
        if cls == 0:
            wq[g] = [_dot(st(t), _bf(umt[:, c:c + 128])) for t, c in ((0, 0), (1, 256))]
        else:
            q1, q2, q3 = [_dot(st(t), _bf(umt[:, c:c + 128])) for t, c in ((0, 128), (1, 384), (2, 512))]
            w0, w2 = wq.pop(g)
            p_ = q1 + w2
            y0 = p_ + (q2 + w0)
            y1 = (q3 + w0) - p_
            yr = pl.ds(dyn(8 * g), 8) if CFG["fuse"] else pl.ds(8 * g, 8)
            for p in range(4):
                yb[yr, pl.ds(256 * p, 128)] = _u32(y0[16 * p:16 * p + 16])
                yb[yr, pl.ds(256 * p + 128, 128)] = _u32(y1[16 * p:16 * p + 16])

    ktq = []
    slotno = [0]
    pat = CFG.get("kt_pat", [1, 0, 1, 1, 0, 1, 0, 1, 1, 0, 1, 1, 0, 1, 0, 1])
    xw = CFG["xw"]

    def kt_drain(n):
        for _ in range(n):
            if ktq and ktq[0][0] <= slotno[0]:
                kt_unit(*ktq.pop(0)[1:])

    utq = [(b, k, j) for b in range(D // RU) for j in range(0, NCH, utj) for k in range(2)]
    pend = [None]

    pre_xy = {}

    def kxy(st, half):
        r0 = st * 16
        pk = [pltpu.bitcast(prm[k, pl.ds(r0, 16), :], U32) for k in range(6)]
        rows = pl.ds(r0 + half, 8, stride=2)
        bs, k0 = _base8([_upk(w, half) for w in pk], dtc[rows, :])
        k0c[rows, :] = jnp.broadcast_to(k0, (8, 128))
        return [_grp_xy(bs, grp, M.lo4) for grp in range(2)]

    def kgen(s0, s1):
        for st in range(s0, s1):
            o4 = []
            for half in range(2):
                xy = pre_xy.pop((st, half)) if (st, half) in pre_xy else kxy(st, half)
                if half == 0 and pend[0] is not None:
                    flush()
                oo = []
                for grp in range(2):
                    yield
                    slotno[0] += 1
                    oo.append(_dot_nt(*xy[grp]))
                o4.append(oo)
            pend[0] = (st, o4)
        if s1 == NS or not CFG["carry"]:
            flush()
        else:
            for h in range(CFG["npre"]):
                pre_xy[(s1 + h // 2, h % 2)] = kxy(s1 + h // 2, h % 2)

    def flush():
        extract(*pend[0])
        if (pend[0][0] + 1) % SPB == 0:
            ktq.extend([(slotno[0] + 4 * CFG["kt_lag"], pend[0][0] // SPB, c) for c in range(NCH)])
        pend[0] = None

    def region(name, fn):
        def body():
            masks()
            mark(name)
            fn()
            mark(None)
        if CFG["split"]:
            pl.when(zs[0] == 0)(body)
        else:
            body()

    def consts():
        dkb = _col_bcast(dsk)
        for t in range(5):
            n = 128 if t < 4 else 64
            dkc[pl.ds(t * 128, n), :] = dkb[t][:n]
            mt = _bf(um[:, 128 * t:128 * t + 128]).T
            if t == 0:
                ri = lax.broadcasted_iota(I32, (128, 128), 0)
                ci = lax.broadcasted_iota(I32, (128, 128), 1)
                alt = jnp.where(ci % 2 == 1, 1.0, -1.0)
                mt = jnp.where(ri == 0, alt, jnp.where(ri == 64, 1.0, mt.astype(F32))).astype(BF16)
            umt[:, pl.ds(128 * t, 128)] = pltpu.bitcast(mt, U32)

    def rate(num, den):
        acc = [0]

        def step():
            acc[0] += num
            n = acc[0] // den
            acc[0] -= n * den
            return n
        return step

    only = CFG.get("only")
    doA = only in (None, "A")
    s1 = R1 // 16 - (CFG['npre'] + 1) // 2
    if doA:
        for _ in kgen(0, s1):
            pass
    mark('s3_w2')
    for cp in in_cp[2]:
        cp.wait()
    mark('s3_A1b')
    zs[0] = pltpu.bitcast(g0b[pl.ds(128, 8), pl.ds(384, 128)], I32)[0, 0]
    zo.append(zs[0] * 8)
    if doA:
        slotno[0] += 100
        ktr = rate(*CFG["ktr1"])
        for i, _ in enumerate(kgen(s1, xw)):
            if i == CFG["gg_at"]:
                ggen()
            if i > CFG["gg_at"]:
                kt_drain(ktr())
        consts()
    mark('s4_waitx')
    in_cp[3][0].wait()
    mark(None)

    def phase_a2():
        slotno[0] += 100
        kg = kgen(xw, NS)
        kgr = rate(*CFG["kgr"])
        for _ in range(CFG["pre"]):
            next(kg)
        for j in range(NCH):
            for k, _ in enumerate(ln_chunk(j)):
                kt_drain(CFG["n01"][0 if k == 0 else 1])
                for _ in range(kgr()):
                    next(kg)
        topk()
        ktr = rate(*CFG["ktr2"])
        xq = list(range(16))
        for i, _ in enumerate(kg):
            kt_drain(ktr())
            if i >= CFG["xs_lag"] and xq:
                xsel(xq.pop(0))
        while xq:
            xsel(xq.pop(0))
        slotno[0] += 1000
        kt_drain(len(ktq) - NCH)

    ffp = [0, 0]

    def ffn_next():
        if ffp[1] < ffp[0] - 1 or (ffp[1] < ffp[0] and ffp[0] >= ffp_max[0]):
            ffn_dn(ffp[1], False)
            ffp[1] += 1
        elif ffp[0] < ffp_max[0]:
            ffn_gu(ffp[0], False)
            ffp[0] += 1
    ffp_max = [0]

    def phase_b(g0, g1):
        inB[0] = True
        lag = CFG["lag"]
        NG = D // 8
        if g0 == 0:
            npre = 16 // utj + (2 * CFG["lead"] * 64 // RU) // utj
            for i in range(0 if CFG["utpre"] else npre):
                ut_piece(*utq.pop(0))
            if CFG["fuse"]:
                for t in range(5):
                    n = 128 if t < 4 else 64
                    deff[pl.ds(128 * t, n), :] = (dkc[pl.ds(128 * t, n), :] + k0c[pl.ds(128 * t, n), :]) * 2.0
        fl = CFG["flag"]
        for s in range(g0, g1):
            for cls in range(2):
                if s < NG:
                    zq[(s, cls)] = mac(s, cls)
                if CFG["order"] == 1 and lag <= s < NG + lag:
                    inv(s - lag, cls)
                if ((2 * s + cls) * 64 // RU) % utj == 0:
                    for _ in range(max(1, 64 // RU // utj)):
                        if utq:
                            ut_piece(*utq.pop(0))
                if cls == 1 and s % 4 == CFG["ktb"] % 4 and s >= CFG["ktb"]:
                    kt_drain(1)
                if CFG["order"] == 0 and lag <= s < NG + lag:
                    inv(s - lag, cls)
                if CFG["fuse"]:
                    q = 2 * (s - lag - fl) + cls - 2
                    if 0 <= q < 4 * NS:
                        fin16(q // 4, 4 * (q % 4), 4 * (q % 4) + 4, None, False)
                if CFG["ffb"] and cls == 0 and s % CFG["ffb"] == 0:
                    ffn_next()

    if only in (None, "A"):
        region('s5_A2', phase_a2)
    elif only == "B":
        ktq.extend([(0, NB - 1, c) for c in range(NCH)])
    HR = CFG["hrows"]
    obb = ob.bitcast(BF16)
    o_cp = [[pltpu.make_async_copy(obb.at[pl.ds(r0, n), pl.ds(128 * t, 128)],
                                   out_hbm.at[pl.ds(r0, n), pl.ds(128 * t, 128)], sem_o.at[hf, t])
             for t in range(16)] for hf, (r0, n) in enumerate([(0, HR), (HR, D - HR)] if HR else [(0, D)])]

    def start_free(hf):
        hit = hit_s[0]
        for t in range(16):
            @pl.when(((hit >> t) & 1) == 0)
            def _():
                o_cp[hf][t].start(priority=1)

    GEND = D // 8 + CFG["lag"] + CFG["flag"] + 2
    if only in (None, "B"):
        def pb():
            g = 0
            for gs, cc in CFG["bw"]:
                if gs > g:
                    phase_b(g, gs)
                    g = gs
                if cc == len(CFG["bw"]) - 1 and only is None and HR:
                    assert (2 * (gs - 1 - CFG["lag"] - CFG["flag"]) + 1 - 2 + 1) // 4 * 16 >= HR
                    start_free(0)
                mark(f's7_w{cc}')
                for cp in w_cp[cc]:
                    cp.wait()
                mark(f's7_B{cc}')
                ffp_max[0] = sum(FCH[:cc + 1]) // 2
                tk["xs"] = _bf(xs_s[...])
            phase_b(g, GEND)
            while CFG["ffb"] and ffp[1] < ffp_max[0]:
                ffn_next()
            if CFG["ffb"]:
                ya_s[...] = tk["y"]
        region('s7_B', pb)
    if only in ("A", "B"):
        for cc in range(len(CFG["bw"]), len(FCH)):
            for cp in w_cp[cc]:
                cp.wait()
        cp = pltpu.make_async_copy(ob.bitcast(BF16), out_hbm, sem_o.at[0, 0])
        cp.start()
        cp.wait()
        cp = pltpu.make_async_copy(yb.bitcast(BF16).at[pl.ds(0, D), :], out_hbm.at[:, pl.ds(0, 1024)], sem_o.at[0, 0])
        cp.start()
        cp.wait()
        for kk in ksps:
            cp = pltpu.make_async_copy(kk.at[:, pl.ds(0, 512)], junk.at[:, pl.ds(0, 512)], sem_o.at[0, 0])
            cp.start()
            cp.wait()
        for kk in (vv, xs_s, kd, umt):
            cp = pltpu.make_async_copy(kk.at[pl.ds(0, 8), pl.ds(0, 512)], oh_s.at[:, pl.ds(0, 512)], sem_o.at[0, 0])
            cp.start()
            cp.wait()
        cp = pltpu.make_async_copy(ya_s, junk.at[pl.ds(0,16), :], sem_o.at[0, 0])
        cp.start()
        cp.wait()
        return
    masks()
    tk["xs"] = _bf(xs_s[...])
    tk["rs"] = rs_s[...]
    tk["oh"] = _bf(oh_s[...])

    mark('s8_ffn')
    start_free(len(o_cp) - 1)
    tk["y"] = ya_s[...]
    for cc in range(len(CFG["bw"]), len(FCH)):
        lastc = cc == len(FCH) - 1
        mark(f's8_w{cc}')
        for cp in (w_cp[cc][:2] if lastc else w_cp[cc]):
            cp.wait()
        mark(f's8_f{cc}')
        ffp_max[0] = sum(FCH[:cc + 1]) // 2
        while ffp[0] < ffp_max[0]:
            ffn_gu(ffp[0], False)
            ffp[0] += 1
            if ffp[1] < ffp[0] - 1 and not lastc:
                ffn_dn(ffp[1], False)
                ffp[1] += 1
        if lastc:
            mark('s8_w5')
            w_cp[cc][2].wait()
            mark('s8_f5')
        while ffp[1] < ffp[0]:
            ffn_dn(ffp[1], False)
            ffp[1] += 1
    rs = jnp.concatenate([tk["rs"]] * 5, axis=1)[:, :D]
    upd = (_rb(_rb(tk["y"]) * rs) * 0.5).astype(BF16)
    updt_s[:, pl.ds(0, 128)] = _u32(lax.dot_general(upd, jnp.eye(16, 128, dtype=BF16), (((0,), (0,)), ((), ())),
                                       preferred_element_type=F32))
    mark('s9_final')
    hit = hit_s[0]
    for t in range(16):
        @pl.when(((hit >> t) & 1) == 1)
        def _():
            ohp = jnp.concatenate([_bf(oh_s[:, pl.ds(128 * t, 128)]), jnp.zeros((112, 128), BF16)], axis=0)
            du = _dot(_bf(updt_s[:, pl.ds(0, 128)]), ohp)
            for i in range(NS):
                fin16(i, t, t + 1, du[16 * i:16 * i + 16], False)
            for hf in range(len(o_cp)):
                o_cp[hf][t].start(priority=1)
    mark('sa_waito')
    for cps in o_cp:
        for cp in cps:
            cp.wait()
    mark(None)


@jax.jit
def pallas_recurrent_scan__ssm_conv_s4__moe_arch_mod__prompt_kernel(A_u, A_A_re, A_A_im, A_B_re, A_B_im, A_C_re, A_C_im, A_log_dt, A_Dskip,
              B_x, B_w_r, B_w_gate, B_w_up, B_w_down):
    xt = jnp.transpose(A_u[0])
    wdt = jnp.transpose(B_w_down)
    scratch = [
        pltpu.SMEM((1,), I32),
        pltpu.VMEM((D, L), BF16),
        pltpu.VMEM((6, D, N), BF16),
        pltpu.VMEM((D,), BF16),
        pltpu.VMEM((D,), BF16),
        pltpu.VMEM((D,), BF16),
        pltpu.VMEM((D // 2, FF), U32),
        pltpu.VMEM((D // 2, FF), U32),
        pltpu.VMEM((D // 2, FF), U32),
        pltpu.VMEM(_UM.shape, U32),
        pltpu.VMEM(_G0.shape, U32),
        pltpu.VMEM((336, 512), U32),
        pltpu.VMEM(_UM.shape, U32),
        pltpu.VMEM((D, 128), F32),
        pltpu.VMEM((D, 128), F32),
        pltpu.VMEM((D, 128), F32),
        pltpu.VMEM((D // 2, 896), U32),
        pltpu.VMEM((D // 2, L), U32),
        pltpu.VMEM((D // 2, L), U32),
        pltpu.VMEM((CFG['RU'], 5120), F32),
        pltpu.VMEM((CFG['RU'], 5120), F32),
        pltpu.VMEM((CFG['RU'], 5120), F32),
        pltpu.VMEM((D, L // 2), U32),
        pltpu.VMEM((D // 2, L), U32),
        pltpu.VMEM((64, D), F32),
        pltpu.VMEM((16, 128), F32),
        pltpu.VMEM((8, L), U32),
        pltpu.VMEM((8, D), U32),
        pltpu.SMEM((1,), I32),
        pltpu.VMEM((8, 128), U32),
        pltpu.VMEM((D, 128), F32),
        pltpu.VMEM((D // 2, 256), U32),
        pltpu.VMEM((16, D), F32),
        pltpu.SemaphoreType.DMA((18,)),
        pltpu.SemaphoreType.DMA((3, len(FCH))),
        pltpu.SemaphoreType.DMA((2, 16)),
    ] + [pltpu.VMEM((RB, 4096), F32)] * NB
    out = pl.pallas_call(
        _kernel,
        out_shape=jax.ShapeDtypeStruct((D, L), BF16),
        in_specs=[pl.BlockSpec(memory_space=pl.ANY)] * 15,
        out_specs=pl.BlockSpec(memory_space=pl.ANY),
        scratch_shapes=scratch,
        compiler_params=pltpu.CompilerParams(vmem_limit_bytes=100 * 2**20, disable_semaphore_checks=True,
                                             disable_bounds_checks=True),
        name="s4_mod",
    )(xt, A_A_re, A_A_im, A_B_re, A_B_im, A_C_re, A_C_im, A_log_dt, A_Dskip,
      B_w_r, B_w_gate, B_w_up, wdt, jnp.asarray(_UM), jnp.asarray(_G0))
    return jnp.transpose(out)[None]
```

```python
import functools
import math

import numpy as np
import jax
import jax.numpy as jnp
from jax import lax
import jax.experimental.pallas as pl
import jax.experimental.pallas.tpu as pltpu

F32 = jnp.float32
BF16 = jnp.bfloat16
U32 = jnp.uint32
I32 = jnp.int32

D = 576
L = 2048
N = 128
FF = 4608
NSEL = 8
NCH = 8
RB = 64
NB = D // RB
NS = D // 16
SPB = RB // 16
FCH = (10, 10, 8, 6, 2)

_TILES = {
    "odd": (1, 3, 5, 7),
    "even": (2, 4, 6, 8),
    "t2": (258, 260, 262, 264),
    "t3": (516, 520, 772, 776),
    "t4": (1032, 1288, 1544, 1800),
}


def _rlag(l):
    u = int(np.float32(l).view(np.uint32))
    u = (u + 0x7FFF + ((u >> 16) & 1)) & 0xFFFF0000
    return int(np.uint32(u).view(np.float32))


def _tile_pts(name):
    base = name.rstrip("v")
    p = np.array([_TILES[base][l // 32] + 8 * (l % 32) for l in range(128)])
    if name == "t3v":
        p[127] = 512
    if name == "t4v":
        p[127] = 1024
    return p


def _fdk_row(r):
    f1 = 4 * np.arange(128) + 1
    f02 = np.concatenate([4 * np.arange(64), 4 * np.arange(64) + 2])
    w = 2 * np.pi / 512
    sgn = (-1.0) ** r
    r02 = np.cos(w * f02 * r)
    i02 = -np.sin(w * f02 * r)
    r02[0] = (-sgn - 1.0) / 4.0
    i02[0] = (1.0 - sgn) / 4.0
    return np.concatenate([np.cos(w * f1 * r), -np.sin(w * f1 * r), r02, i02]) / 128.0


def _gmat(c, tile):
    pts = _tile_pts(tile)
    g = np.zeros((128, 512))
    for r in range(1, 257):
        idx = np.nonzero(pts == _rlag(256 * c + r))[0]
        if len(idx):
            g[idx[0]] += _fdk_row(r)
    return g


def _pack_bf16(a):
    u = np.ascontiguousarray(a, np.float32).view(np.uint32)
    u = ((u + 0x7FFF + ((u >> 16) & 1)) >> 16).astype(np.uint32)
    return (u[0::2] | (u[1::2] << 16)).astype(np.uint32)


def _tables():
    f1 = 4 * np.arange(128) + 1
    w = 2 * np.pi / 512
    t = np.arange(128)[:, None] + 1
    a = np.cos(w * f1 * t)
    b = -np.sin(w * f1 * t)
    f0 = 4 * np.arange(64)
    f2 = f0 + 2
    m0 = np.concatenate([np.cos(w * f0 * t), -np.sin(w * f0 * t)], axis=1)
    m2 = np.concatenate([-np.sin(w * f2 * t), np.cos(w * f2 * t)], axis=1)
    m0[:, 64] = (-1.0) ** t[:, 0]
    um = np.concatenate([m0, a, m2, b - a, a + b], axis=1)
    g0 = np.concatenate([_gmat(0, "odd"), _gmat(0, "even")], axis=0)
    lags = np.concatenate([_tile_pts("odd"), _tile_pts("even")])
    sel = np.full((8, 256), -1, np.int32)
    for k, (c, tile) in enumerate([(1, "t2"), (2, "t3v"), (4, "t4v"), (1, "even")]):
        pts = _tile_pts(tile)
        for rho, r in enumerate(lags):
            idx = np.nonzero(pts == _rlag(256 * c + int(r)))[0]
            if len(idx):
                sel[k, rho] = idx[0]
    selp = np.zeros((8, 512), np.int32)
    selp[:, :256] = sel
    return _pack_bf16(um), np.concatenate([_pack_bf16(g0), selp.view(np.uint32)], axis=0)


_UM, _G0 = _tables()


def _bf(x):
    return pltpu.bitcast(x, BF16)


def _u32(x):
    return pltpu.bitcast(x.astype(BF16), U32)


def _rb(x):
    return x.astype(BF16).astype(F32)


def _cmul(a, b):
    return (a[0] * b[0] - a[1] * b[1], a[0] * b[1] + a[1] * b[0])


def _csq(a):
    t = a[0] * a[1]
    return (a[0] * a[0] - a[1] * a[1], t + t)


def _sincos(th):
    magic = 12582912.0
    kf = th * (2.0 / math.pi) + magic
    ki = pltpu.bitcast(kf, I32)
    k = kf - magic
    r = th - k * 1.5703125
    r = r - k * 4.837512969970703125e-4
    r = r - k * 7.54978995489188216e-8
    r2 = r * r
    s = r + r * r2 * (-1.6666654611e-1 + r2 * (8.3321608736e-3 + r2 * -1.9515295891e-4))
    c = 1.0 + r2 * (-0.5 + r2 * (4.166664568298827e-2 + r2 * (-1.388731625493765e-3 + r2 * 2.443315711809948e-5)))
    swap = (ki & 1) == 1
    sn = jnp.where(swap, c, s)
    cs = jnp.where(swap, s, c)
    sbit = (ki & 2) << 30
    cbit = ((ki + 1) & 2) << 30
    sn = pltpu.bitcast(pltpu.bitcast(sn, I32) ^ sbit, F32)
    cs = pltpu.bitcast(pltpu.bitcast(cs, I32) ^ cbit, F32)
    return cs, sn


def _dot(a, b):
    return jnp.dot(a, b, preferred_element_type=F32)


def _dot_nt(a, b):
    return lax.dot_general(a, b, (((1,), (1,)), ((), ())), preferred_element_type=F32)


def _col_bcast(vec_ref):
    v = vec_ref[...].astype(F32).reshape(1, D)
    vp = jnp.concatenate([v, jnp.zeros((1, 64), F32)], axis=1)
    return [jnp.broadcast_to(vp[:, t * 128:(t + 1) * 128], (128, 128)).T for t in range(5)]


def _base8(p, dt):
    are, aim, bre, bim, cre, cim = p
    y1 = (dt * are) * math.log2(math.e)
    ph = {1: _sincos(dt * aim)}
    e = 1
    while e < 512:
        ph[2 * e] = _csq(ph[e])
        e *= 2
    pw = {}
    for e in (1, 2, 4, 8, 16, 256, 512):
        mg = jnp.exp2(y1 * float(e)) if e > 1 else jnp.exp2(y1)
        pw[e] = (mg * ph[e][0], mg * ph[e][1])
    w = _cmul((cre, cim), (dt * bre, dt * bim))
    k0 = jnp.sum(w[0], axis=1, keepdims=True)
    w1 = _cmul(w, pw[1])
    w2 = _cmul(w1, pw[1])
    w3 = _cmul(w2, pw[1])
    w258 = _cmul(w2, pw[256])

    def rot(z):
        return (pltpu.roll(z[0], 4, 0), pltpu.roll(z[1], 4, 0))
    rots = {e: rot(pw[e]) for e in (2, 4, 8, 16, 512)}
    return (pw, rots, w1, w2, rot(w3), rot(w258)), k0


def _grp_xy(bs, grp, lo4):
    pw, rots, w1, w2, w3r, w258r = bs

    def sel(lo, hi):
        return (jnp.where(lo4, lo[0], hi[0]), jnp.where(lo4, lo[1], hi[1]))
    if grp == 0:
        dup = {e: sel(pw[e], rots[e]) for e in (2, 4, 16, 512)}
        x0, x2, a8 = sel(w1, w3r), sel(w2, w258r), rots[8]
    else:
        dup = {e: sel(rots[e], pw[e]) for e in (2, 4, 16, 512)}
        x0, x2, a8 = sel(w3r, w1), sel(w258r, w2), pw[8]
    xv = [None] * 10
    xv[0] = x0
    xv[1] = _cmul(x0, dup[4])
    xv[2] = x2
    xv[3] = _cmul(xv[2], dup[2])
    xv[4] = _cmul(xv[3], dup[2])
    xv[5] = _cmul(xv[4], dup[2])
    xv[6] = _cmul(xv[3], dup[512])
    xv[7] = _cmul(xv[5], dup[512])
    xv[8] = _cmul(xv[7], dup[512])
    xv[9] = _cmul(xv[8], dup[512])
    y = (jnp.where(lo4, 1.0, a8[0]), jnp.where(lo4, 0.0, -a8[1]))
    m = dup[16]
    ys = [y]
    for _ in range(15):
        y = (y[0] * m[0] + y[1] * m[1], y[1] * m[0] - y[0] * m[1])
        ys.append(y)

    def mat(vs):
        return jnp.concatenate([jnp.concatenate([v[0] for v in vs], 0),
                                jnp.concatenate([v[1] for v in vs], 0)], 1).astype(BF16)
    return mat(xv), mat(ys)


def _pk(a, b):
    return pltpu.pack_elementwise([a, b], packed_dtype=BF16)


def _upk(w, h):
    return pltpu.unpack_elementwise(w, index=h, packed_dtype=BF16, unpacked_dtype=F32)


_KT = [(0, 256, 0), (128, 256, 256), (384, 128, 512), (512, 128, 576),
       (640, 128, 704), (768, 128, 800), (768, 128, 768), (768, 128, 736)]

CFG = dict(tmode=1, n5=(2, 1, 1, 1, 1), xs_per=3, npre=0, kgr=(1, 5), n01=(3, 1), carry=1, r1=128, ktr1=(0, 1), ktr2=(1, 2), lnr=(1, 1), gg_at=3, xs_lag=16, fuse=1, flag=1, ffb=2, bw=[(0, 0), (23, 1), (48, 2)], hrows=0, wall=0, link=0, split=1, ktb=4, RU=16, gw=4, kt0=4, ffn_grp=(3, 1, 1), xsel_at=27, xw=22, kt_ln=4, pre=1, utpre=0, kdyn=1, ktag=0, kt_lag=1, utj=4, order=1, lag=1, lead=1, scopes=False)


def _kernel(x_hbm, are_hbm, aim_hbm, bre_hbm, bim_hbm, cre_hbm, cim_hbm, ldt_hbm, dsk_hbm,
            wr_hbm, wg_hbm, wu_hbm, wd_hbm, um_hbm, g0_hbm, out_hbm,
            zs, xb, prm, ldt, dsk, wr, wg, wu, wd, um, g0b, gm,
            umt, dtc, dkc, k0c, kd, xh, vv, ur0, ur1, ur2, yb, ob, junk, rs_s, oh_s, xs_s, hit_s, zmk, deff, updt_s, ya_s, upt_s,
            sem_small, sem_w, sem_o, *ksps):
    urs = (ur0, ur1, ur2)
    _cur = [None]

    def mark(name):
        if not CFG["scopes"]:
            return
        if _cur[0] is not None:
            _cur[0].__exit__(None, None, None)
            _cur[0] = None
        if name:
            _cur[0] = jax.named_scope(name)
            _cur[0].__enter__()
    R1 = CFG["r1"]
    prs = [are_hbm, aim_hbm, bre_hbm, bim_hbm, cre_hbm, cim_hbm]
    order = (1, 0, 2, 3, 4, 5)
    grp0 = [(ldt_hbm, ldt)]
    grp1 = [(prs[i].at[pl.ds(0, R1)], prm.at[i, pl.ds(0, R1)]) for i in order]
    grp2 = [(prs[i].at[pl.ds(R1, D - R1)], prm.at[i, pl.ds(R1, D - R1)]) for i in order]
    grp2 += [(g0_hbm, g0b), (um_hbm, um), (dsk_hbm, dsk), (wr_hbm, wr)]
    grp3 = [(x_hbm, xb)]
    in_cp = []
    for grp in (grp0, grp1, grp2, grp3):
        n0 = sum(len(g) for g in in_cp)
        in_cp.append([pltpu.make_async_copy(s, d, sem_small.at[n0 + i]) for i, (s, d) in enumerate(grp)])
        for cp in in_cp[-1]:
            cp.start()
    w_cp = []
    off = 0
    for c, n in enumerate(FCH):
        cs = pl.ds(off * 128, n * 128)
        w_cp.append([pltpu.make_async_copy(h.at[:, cs], b.bitcast(BF16).at[:, cs], sem_w.at[i, c])
                     for i, (h, b) in enumerate([(wg_hbm, wg), (wu_hbm, wu), (wd_hbm, wd)])])
        for cp in w_cp[-1]:
            cp.start(priority=1)
        off += n

    class M:
        pass

    def masks():
        sub = lax.broadcasted_iota(I32, (8, 128), 0)
        lane = lax.broadcasted_iota(I32, (8, 128), 1)
        M.lo4 = sub < 4
        M.gidx = 4 * (lane % 32) + (sub % 4)
        M.lo64 = lane < 64
        M.beven = ((lane // 32) % 2) == 0
        M.last = lane == 127
        M.mz = jnp.where(lane == 0, 0.0, 1.0)
        M.row16 = lax.broadcasted_iota(I32, (16, 128), 0)
        M.lane16 = lax.broadcasted_iota(I32, (16, 128), 1)
    masks()

    mark('s0_wait0')
    in_cp[0][0].wait()
    mark('s1_prep')
    dtb = _col_bcast(ldt)
    for t in range(5):
        n = 128 if t < 4 else 64
        dtc[pl.ds(t * 128, n), :] = _rb(jnp.exp(dtb[t][:n]))
    mark('s2_waitp')
    for cp in in_cp[1]:
        cp.wait()
    mark('s3_A1')
    zo = []

    def dyn(r):
        return pl.multiple_of(zo[0] + r, 8)

    inB = [False]

    def kt_unit(b, c):
        l0, kk, g0 = _KT[c]
        gw = g0b[pl.ds(0, 128), :] if c == 0 else gm[pl.ds((g0 - 256) // 2, kk // 2), :]
        raw = _dot(_bf(kd[pl.ds(b * (RB // 2), RB // 2), pl.ds(l0, kk)]), _bf(gw))
        rows = pl.ds(dyn(0), RB) if inB[0] else pl.ds(0, RB)
        ksps[b][rows, pl.ds(512 * c, 512)] = raw
        if CFG["ktag"]:
            tg = pltpu.roll(ksps[b][pl.ds(0, 8), pl.ds(512 * c, 128)], 1, 1)
            junk[pl.ds(8 * ((b * NCH + c) % 8), 8), :] = tg

    def ggen():
        sel = pltpu.bitcast(g0b[pl.ds(128, 8), :], I32)

        def onehot(k, r0, n):
            ri = lax.broadcasted_iota(I32, (n, 256), 0) + r0
            return jnp.where(ri == sel[k:k + 1, :256], 1.0, 0.0)
        e = jnp.concatenate([onehot(0, 0, 128), onehot(1, 0, 64), onehot(2, 0, 32),
                             onehot(1, 112, 16), onehot(2, 112, 16), onehot(3, 112, 16)], axis=0).astype(BF16)
        g = _dot(e, _bf(g0b[pl.ds(0, 128), :]))

        def put(r, v):
            gm[pl.ds((r - 256) // 2, v.shape[0] // 2), :] = _u32(v)

        def zero(r, n):
            gm[pl.ds((r - 256) // 2, n // 2), :] = jnp.zeros((n // 2, 512), U32)
        zero(256, 112)
        put(368, g[256:272])
        put(384, g[0:128])
        put(512, g[128:192])
        zero(576, 48)
        put(624, g[224:240])
        put(640, g[128:192])
        put(704, g[192:224])
        zero(736, 80)
        put(816, g[240:256])
        put(832, g[192:224])
        zero(864, 64)

    def extract(st, o4):
        g = [[jnp.take_along_axis(_pk(o4[0][grp][8 * v:8 * v + 8], o4[1][grp][8 * v:8 * v + 8]), M.gidx, axis=1,
                                  mode="promise_in_bounds") for v in range(10)] for grp in range(2)]

        def mix(a, b):
            return jnp.where(M.lo4, a, b), pltpu.roll(jnp.where(M.lo4, b, a), 4, 0)

        def two(va, vb, m1, m2):
            p, q = mix(jnp.where(m1, g[0][va], g[0][vb]), jnp.where(m1, g[1][va], g[1][vb]))
            return jnp.where(m2, p, q)

        def four(gg):
            return jnp.where(M.lo64, jnp.where(M.beven, gg[2], gg[3]), jnp.where(M.beven, gg[4], gg[5]))
        t_odd = two(0, 1, M.lo64, M.beven)
        t_even, t_2 = mix(four(g[0]), four(g[1]))
        t_3 = two(6, 7, M.beven, M.lo64)
        t_4 = two(8, 9, M.lo64, M.beven)
        tl = [t_odd, t_even, t_2, jnp.where(M.last, t_2, t_3), t_3, jnp.where(M.last, t_3, t_4), t_4]
        for t in range(7):
            kd[pl.ds(st * 8, 8), pl.ds(128 * t, 128)] = tl[t]

    tk = {}

    def ln_chunk(j):
        cj = slice(256 * j, 256 * j + 256)
        s1 = s2 = None
        for i in range(NS):
            v16 = xb[pl.ds(i * 16, 16), cj].astype(F32)
            for v in (v16[:8], v16[8:]):
                s1, s2 = (v, v * v) if s1 is None else (s1 + v, s2 + v * v)
        mean = jnp.sum(s1, axis=0, keepdims=True) * (1.0 / D)
        var = jnp.sum(s2, axis=0, keepdims=True) * (1.0 / D) - mean * mean
        var = jnp.maximum(var, 0.0)
        sd = _rb(jnp.sqrt(_rb(_rb(var) + 1e-5)))
        mb = jnp.broadcast_to(_rb(mean), (16, 256))
        hi = jnp.broadcast_to(0.5 / sd, (16, 256))
        if j == 0:
            wrow = wr[...].astype(F32).reshape(1, D)
            tk["w"] = [(jnp.broadcast_to(wrow[:, k0:min(k0 + 128, D)], (16, min(128, D - k0)))
                        + jnp.zeros((16, min(128, D - k0)), F32)).astype(BF16) for k0 in range(0, D, 128)]
        r = None
        for i in range(NS):
            rw = pl.ds(dyn(i * 8), 8)
            hv = _rb(xb[pl.ds(i * 16, 16), cj].astype(F32) - mb) * hi
            h0, h1 = hv[:, :128], hv[:, 128:]
            xh[rw, pl.ds(256 * j, 128)] = _u32(h0)
            xh[rw, pl.ds(256 * j + 128, 128)] = _u32(h1)
            vv[pl.ds(i * 8, 8), pl.ds(256 * j, 128)] = _u32(h0 + h1)
            vv[pl.ds(i * 8, 8), pl.ds(256 * j + 128, 128)] = _u32(h0 - h1)
            if i % 8 == 7 or i == NS - 1:
                k0, k1 = (i // 8) * 128, (i + 1) * 16
                yield
                p = _dot(tk["w"][i // 8], _bf(xh[pl.ds(k0 // 2, (k1 - k0) // 2), cj]))
                r = p if r is None else r + p
        for t in range(2):
            r_t = r[:, 128 * t:128 * t + 128]
            tk["rc"] = r_t if (j == 0 and t == 0) else jnp.where(M.row16 == 2 * j + t, r_t, tk["rc"])

    def topk():
        bits = pltpu.bitcast(_rb(tk["rc"] * 2.0), I32)
        mono = (jnp.where(bits < 0, bits ^ 0x7FFF0000, bits) >> 16) + 32768
        key = pltpu.bitcast(0x30000000 + (mono << 11) + (2047 - (M.row16 * 128 + M.lane16)), F32)
        kcol = jnp.zeros((16, 128), I32)
        for j in range(NSEL):
            mx = jnp.max(jnp.max(key, axis=0, keepdims=True), axis=1, keepdims=True)
            mxb = jnp.broadcast_to(mx, (16, 128))
            key = jnp.where(key == mxb, 0.0, key)
            kcol = jnp.where(M.row16 == j, pltpu.bitcast(mxb, I32), kcol)
        kcol = kcol - 0x30000000
        idxcol = jnp.where(M.row16 < NSEL, 2047 - (kcol & 2047), -1)
        hb = ((kcol >> 11) - 32768) << 16
        rsel = pltpu.bitcast(jnp.where(hb < 0, hb ^ 0x7FFF0000, hb), F32)
        rsel = jnp.where(M.row16 < NSEL, rsel, 0.0)
        rs_s[...] = _rb(jax.nn.sigmoid(rsel))
        tk["oh"] = jnp.concatenate(
            [jnp.where(idxcol == M.lane16 + 128 * t, 1.0, 0.0) for t in range(16)], axis=1).astype(BF16)
        oh_s[...] = pltpu.bitcast(tk["oh"], U32)
        hb_ = jnp.where(M.row16[:8] < NSEL, jnp.left_shift(1, jnp.maximum(idxcol[:8], 0) >> 7), 0)
        for sh in (4, 2, 1):
            hb_ = hb_ | pltpu.roll(hb_, sh, 0)
        hit_s[0] = hb_[0, 0]
        tcol = jnp.maximum(idxcol, 0) >> 7
        tk["tj"] = [tcol[j, 0] for j in range(NSEL)]
        tk["ol"] = jnp.where((idxcol & 127) == M.lane16, 1.0, 0.0)

    def xsel(j):
        off = pl.multiple_of(tk["tj"][j] * 128, 128)
        lhs = jnp.where(M.row16 == j, tk["ol"], 0.0).astype(BF16)
        v = _dot_nt(lhs, _bf(xh[:, pl.ds(off, 128)]))
        tk["xa"] = v if j == 0 else tk["xa"] + v
        if j == NSEL - 1:
            xs_s[...] = _u32(tk["xa"] * 2.0)

    def link(v):
        if not CFG["link"]:
            return v
        w = pltpu.bitcast(v, U32)
        dep = ob[pl.ds(0, 8), pl.ds(0, 128)] & tk["zm"]
        return pltpu.bitcast(jnp.concatenate([w[:, :128] | dep, w[:, 128:]], axis=1), BF16)

    def ffn_gu(p, lk):
        cs = pl.ds(256 * p, 256)
        xs = link(tk["xs"]) if lk else tk["xs"]
        gu = _dot(xs, _bf(jnp.concatenate([wg[:, cs], wu[:, cs]], axis=1)))
        g = _rb(gu[:, :256])
        u = _rb(gu[:, 256:])
        sg = _rb(0.5 * jnp.tanh(0.5 * g) + 0.5)
        tk["h", p] = (_rb(g * sg) * u).astype(BF16)

    def ffn_dn(p, lk):
        h = tk.pop(("h", p))
        y = _dot_nt(link(h) if lk else h, _bf(wd[:, pl.ds(256 * p, 256)]))
        tk["y"] = y if p == 0 else tk["y"] + y

    def fin16(i, c0, c1, du, dynst):
        r16 = pl.ds(16 * i, 16)
        cs = pl.ds(128 * c0, 128 * (c1 - c0))
        h = _bf(xh[pl.ds(8 * i, 8), cs]).astype(F32)
        y = jnp.concatenate([_upk(yb[r16, pl.ds(256 * (c // 4) + 128 * (c % 2), 128)], (c // 2) % 2)
                             for c in range(c0, c1)], axis=1)
        dv = deff[r16, :]
        s_ = y + h * jnp.concatenate([dv] * (c1 - c0), axis=1)
        zh = h if du is None else h + du
        g = zh * jnp.tanh(zh) + zh
        rw = pl.ds(dyn(8 * i), 8) if dynst else pl.ds(8 * i, 8)
        ob[rw, cs] = _u32(xb[r16, cs].astype(F32) + s_ * g)

    utj = CFG["utj"]
    RU = CFG["RU"]

    def ut_piece(b, k, j0):
        rw = pl.ds(b * (RU // 2), RU // 2)
        rows = pl.ds(dyn(0), RU)
        ur = urs[b % 3]
        js = range(j0, j0 + utj)

        def lhs(ref, o):
            return _bf(jnp.concatenate([ref[rw, pl.ds(256 * j + o, 128)] for j in js], axis=0))

        def put(val, col):
            for i, j in enumerate(js):
                ur[rows, pl.ds(640 * j + col, 128)] = val[i * RU:(i + 1) * RU]
        if k == 0:
            v = _dot(lhs(vv, 0), _bf(um[:, 0:256]))
            b2 = _dot(lhs(vv, 128), _bf(um[:, 256:384]))
            a0 = v[:, :128]

            def sel(p, q):
                return jnp.concatenate([jnp.where(M.lo64, p[8 * i:8 * i + 8], q[8 * i:8 * i + 8])
                                        for i in range(a0.shape[0] // 8)], axis=0)
            put(sel(a0, b2), 0)
            put(v[:, 128:], 128)
            put(pltpu.roll(sel(b2, a0), 64, 1), 256)
        else:
            put(_dot(lhs(xh, 128), _bf(um[:, 384:512])), 384)
            put(_dot(lhs(xh, 0), _bf(um[:, 512:640])), 512)

    def mac(g, cls):
        ur = urs[(8 * g // RU) % 3]

        @functools.lru_cache(None)
        def us(j):
            def ld(c):
                return ur[pl.ds((8 * g) % RU, 8), pl.ds(640 * j + c, 128)]
            if cls == 0:
                a, b = ld(0), ld(256)
                return (a, b, a + b)
            t1, t2, t3 = ld(128), ld(384), ld(512)
            return (t1 + t2, t3 - t1, t2 + t3)

        @functools.lru_cache(None)
        def kraw(j):
            o = 512 * j + 256 * (1 - cls)
            ksp, kr = ksps[8 * g // RB], pl.ds((8 * g) % RB, 8)
            return ksp[kr, pl.ds(o, 128)], ksp[kr, pl.ds(o + 128, 128)]

        @functools.lru_cache(None)
        def ks(j):
            sr, si = kraw(j)
            if j > 0:
                pr, pi_ = kraw(j - 1)
                sr, si = (sr + pr, si + pi_) if cls == 0 else (sr - pr, si - pi_)
            return (sr * M.mz if cls == 0 else sr, si - sr, sr + si)
        outs = []
        prev = None
        for m in range(NCH):
            acc = None
            for j in range(m + 1):
                a, b, s = us(j)
                c_, e_, g_ = ks(m - j)
                t = (c_ * s, a * e_, b * g_)
                acc = t if acc is None else tuple(x + y for x, y in zip(acc, t))
            z = (acc[0] - acc[2], acc[0] + acc[1])
            if m % 2:
                za, zb = prev, z
                if cls == 0:
                    zr = _pk(za[0], zb[0])
                    zis = _pk(za[1], zb[1]) if CFG.get('nrz') else pltpu.roll(_pk(za[1], zb[1]), 64, 1)
                    outs.append((jnp.where(M.lo64, zr, zis), jnp.where(M.lo64, zis, zr)))
                else:
                    outs.append((_pk(za[0] + za[1], zb[0] + zb[1]), _pk(za[1], zb[1]), _pk(za[0], zb[0])))
            prev = z
        return outs

    zq, wq = {}, {}

    def inv(g, cls):
        zo_ = zq.pop((g, cls))

        def st(t):
            return _bf(jnp.concatenate([zo_[p][t] for p in range(4)], axis=0))
        if cls == 0:
            wq[g] = [_dot(st(t), _bf(umt[:, c:c + 128])) for t, c in ((0, 0), (1, 256))]
        else:
            q1, q2, q3 = [_dot(st(t), _bf(umt[:, c:c + 128])) for t, c in ((0, 128), (1, 384), (2, 512))]
            w0, w2 = wq.pop(g)
            p_ = q1 + w2
            y0 = p_ + (q2 + w0)
            y1 = (q3 + w0) - p_
            yr = pl.ds(dyn(8 * g), 8) if CFG["fuse"] else pl.ds(8 * g, 8)
            for p in range(4):
                yb[yr, pl.ds(256 * p, 128)] = _u32(y0[16 * p:16 * p + 16])
                yb[yr, pl.ds(256 * p + 128, 128)] = _u32(y1[16 * p:16 * p + 16])

    ktq = []
    slotno = [0]
    pat = CFG.get("kt_pat", [1, 0, 1, 1, 0, 1, 0, 1, 1, 0, 1, 1, 0, 1, 0, 1])
    xw = CFG["xw"]

    def kt_drain(n):
        for _ in range(n):
            if ktq and ktq[0][0] <= slotno[0]:
                kt_unit(*ktq.pop(0)[1:])

    utq = [(b, k, j) for b in range(D // RU) for j in range(0, NCH, utj) for k in range(2)]
    pend = [None]

    pre_xy = {}

    def kxy(st, half):
        r0 = st * 16
        pk = [pltpu.bitcast(prm[k, pl.ds(r0, 16), :], U32) for k in range(6)]
        rows = pl.ds(r0 + half, 8, stride=2)
        bs, k0 = _base8([_upk(w, half) for w in pk], dtc[rows, :])
        k0c[rows, :] = jnp.broadcast_to(k0, (8, 128))
        return [_grp_xy(bs, grp, M.lo4) for grp in range(2)]

    def kgen(s0, s1):
        for st in range(s0, s1):
            o4 = []
            for half in range(2):
                xy = pre_xy.pop((st, half)) if (st, half) in pre_xy else kxy(st, half)
                if half == 0 and pend[0] is not None:
                    flush()
                oo = []
                for grp in range(2):
                    yield
                    slotno[0] += 1
                    oo.append(_dot_nt(*xy[grp]))
                o4.append(oo)
            pend[0] = (st, o4)
        if s1 == NS or not CFG["carry"]:
            flush()
        else:
            for h in range(CFG["npre"]):
                pre_xy[(s1 + h // 2, h % 2)] = kxy(s1 + h // 2, h % 2)

    def flush():
        extract(*pend[0])
        if (pend[0][0] + 1) % SPB == 0:
            ktq.extend([(slotno[0] + 4 * CFG["kt_lag"], pend[0][0] // SPB, c) for c in range(NCH)])
        pend[0] = None

    def region(name, fn):
        def body():
            masks()
            mark(name)
            fn()
            mark(None)
        if CFG["split"]:
            pl.when(zs[0] == 0)(body)
        else:
            body()

    def consts():
        dkb = _col_bcast(dsk)
        for t in range(5):
            n = 128 if t < 4 else 64
            dkc[pl.ds(t * 128, n), :] = dkb[t][:n]
            mt = _bf(um[:, 128 * t:128 * t + 128]).T
            if t == 0:
                ri = lax.broadcasted_iota(I32, (128, 128), 0)
                ci = lax.broadcasted_iota(I32, (128, 128), 1)
                alt = jnp.where(ci % 2 == 1, 1.0, -1.0)
                mt = jnp.where(ri == 0, alt, jnp.where(ri == 64, 1.0, mt.astype(F32))).astype(BF16)
            umt[:, pl.ds(128 * t, 128)] = pltpu.bitcast(mt, U32)

    def rate(num, den):
        acc = [0]

        def step():
            acc[0] += num
            n = acc[0] // den
            acc[0] -= n * den
            return n
        return step

    only = CFG.get("only")
    doA = only in (None, "A")
    s1 = R1 // 16 - (CFG['npre'] + 1) // 2
    if doA:
        for _ in kgen(0, s1):
            pass
    mark('s3_w2')
    for cp in in_cp[2]:
        cp.wait()
    mark('s3_A1b')
    zs[0] = pltpu.bitcast(g0b[pl.ds(128, 8), pl.ds(384, 128)], I32)[0, 0]
    zo.append(zs[0] * 8)
    if doA:
        slotno[0] += 100
        ktr = rate(*CFG["ktr1"])
        for i, _ in enumerate(kgen(s1, xw)):
            if i == CFG["gg_at"]:
                ggen()
            if i > CFG["gg_at"]:
                kt_drain(ktr())
        consts()
    mark('s4_waitx')
    in_cp[3][0].wait()
    mark(None)

    def phase_a2():
        slotno[0] += 100
        kg = kgen(xw, NS)
        kgr = rate(*CFG["kgr"])
        for _ in range(CFG["pre"]):
            next(kg)
        for j in range(NCH):
            for k, _ in enumerate(ln_chunk(j)):
                kt_drain(CFG["n5"][k])
                for _ in range(kgr()):
                    next(kg)
        topk()
        ktr = rate(*CFG["ktr2"])
        xq = list(range(NSEL))
        for i, _ in enumerate(kg):
            kt_drain(ktr())
            if i >= CFG["xs_lag"] and xq and (i - CFG["xs_lag"]) % CFG["xs_per"] == 0:
                xsel(xq.pop(0))
        while xq:
            xsel(xq.pop(0))
        slotno[0] += 1000
        kt_drain(len(ktq) - NCH)

    ffp = [0, 0]

    def ffn_next():
        if ffp[1] < ffp[0] - 1 or (ffp[1] < ffp[0] and ffp[0] >= ffp_max[0]):
            ffn_dn(ffp[1], False)
            ffp[1] += 1
        elif ffp[0] < ffp_max[0]:
            ffn_gu(ffp[0], False)
            ffp[0] += 1
    ffp_max = [0]

    def phase_b(g0, g1):
        inB[0] = True
        lag = CFG["lag"]
        NG = D // 8
        if g0 == 0:
            npre = 16 // utj + (2 * CFG["lead"] * 64 // RU) // utj
            for i in range(0 if CFG["utpre"] else npre):
                ut_piece(*utq.pop(0))
            if CFG["fuse"]:
                for t in range(5):
                    n = 128 if t < 4 else 64
                    deff[pl.ds(128 * t, n), :] = (dkc[pl.ds(128 * t, n), :] + k0c[pl.ds(128 * t, n), :]) * 2.0
        fl = CFG["flag"]
        for s in range(g0, g1):
            for cls in range(2):
                if s < NG:
                    zq[(s, cls)] = mac(s, cls)
                if CFG["order"] == 1 and lag <= s < NG + lag:
                    inv(s - lag, cls)
                if ((2 * s + cls) * 64 // RU) % utj == 0:
                    for _ in range(max(1, 64 // RU // utj)):
                        if utq:
                            ut_piece(*utq.pop(0))
                if cls == 1 and s % 4 == CFG["ktb"] % 4 and s >= CFG["ktb"]:
                    kt_drain(1)
                if CFG["order"] == 0 and lag <= s < NG + lag:
                    inv(s - lag, cls)
                if CFG["fuse"]:
                    q = 2 * (s - lag - fl) + cls - 2
                    if 0 <= q < 4 * NS:
                        fin16(q // 4, 4 * (q % 4), 4 * (q % 4) + 4, None, False)
                if CFG["ffb"] and cls == 0 and s % CFG["ffb"] == 0:
                    ffn_next()

    if only in (None, "A"):
        region('s5_A2', phase_a2)
    elif only == "B":
        ktq.extend([(0, NB - 1, c) for c in range(NCH)])
    HR = CFG["hrows"]
    obb = ob.bitcast(BF16)
    o_cp = [[pltpu.make_async_copy(obb.at[pl.ds(r0, n), pl.ds(128 * t, 128)],
                                   out_hbm.at[pl.ds(r0, n), pl.ds(128 * t, 128)], sem_o.at[hf, t])
             for t in range(16)] for hf, (r0, n) in enumerate([(0, HR), (HR, D - HR)] if HR else [(0, D)])]

    def start_free(hf):
        hit = hit_s[0]
        for t in range(16):
            @pl.when(((hit >> t) & 1) == 0)
            def _():
                o_cp[hf][t].start(priority=1)

    GEND = D // 8 + CFG["lag"] + CFG["flag"] + 2
    if only in (None, "B"):
        def pb():
            g = 0
            for gs, cc in CFG["bw"]:
                if gs > g:
                    phase_b(g, gs)
                    g = gs
                if cc == len(CFG["bw"]) - 1 and only is None and HR:
                    assert (2 * (gs - 1 - CFG["lag"] - CFG["flag"]) + 1 - 2 + 1) // 4 * 16 >= HR
                    start_free(0)
                mark(f's7_w{cc}')
                for cp in w_cp[cc]:
                    cp.wait()
                mark(f's7_B{cc}')
                ffp_max[0] = sum(FCH[:cc + 1]) // 2
                tk["xs"] = _bf(xs_s[...])
            phase_b(g, GEND)
            while CFG["ffb"] and ffp[1] < ffp_max[0]:
                ffn_next()
            if CFG["ffb"]:
                ya_s[...] = tk["y"]
        region('s7_B', pb)
    if only in ("A", "B"):
        for cc in range(len(CFG["bw"]), len(FCH)):
            for cp in w_cp[cc]:
                cp.wait()
        cp = pltpu.make_async_copy(ob.bitcast(BF16), out_hbm, sem_o.at[0, 0])
        cp.start()
        cp.wait()
        cp = pltpu.make_async_copy(yb.bitcast(BF16).at[pl.ds(0, D), :], out_hbm.at[:, pl.ds(0, 1024)], sem_o.at[0, 0])
        cp.start()
        cp.wait()
        for kk in ksps:
            cp = pltpu.make_async_copy(kk.at[:, pl.ds(0, 512)], junk.at[:, pl.ds(0, 512)], sem_o.at[0, 0])
            cp.start()
            cp.wait()
        for kk in (vv, xs_s, kd, umt):
            cp = pltpu.make_async_copy(kk.at[pl.ds(0, 8), pl.ds(0, 512)], oh_s.at[:, pl.ds(0, 512)], sem_o.at[0, 0])
            cp.start()
            cp.wait()
        cp = pltpu.make_async_copy(ya_s, junk.at[pl.ds(0,16), :], sem_o.at[0, 0])
        cp.start()
        cp.wait()
        return
    masks()
    tk["xs"] = _bf(xs_s[...])
    tk["rs"] = rs_s[...]
    tk["oh"] = _bf(oh_s[...])

    mark('s8_ffn')
    start_free(len(o_cp) - 1)
    tk["y"] = ya_s[...]
    for cc in range(len(CFG["bw"]), len(FCH)):
        lastc = cc == len(FCH) - 1
        mark(f's8_w{cc}')
        for cp in (w_cp[cc][:2] if lastc else w_cp[cc]):
            cp.wait()
        mark(f's8_f{cc}')
        ffp_max[0] = sum(FCH[:cc + 1]) // 2
        while ffp[0] < ffp_max[0]:
            ffn_gu(ffp[0], False)
            ffp[0] += 1
            if ffp[1] < ffp[0] - 1 and not lastc:
                ffn_dn(ffp[1], False)
                ffp[1] += 1
        if lastc:
            mark('s8_w5')
            w_cp[cc][2].wait()
            mark('s8_f5')
        while ffp[1] < ffp[0]:
            ffn_dn(ffp[1], False)
            ffp[1] += 1
    rs = jnp.concatenate([tk["rs"]] * 5, axis=1)[:, :D]
    upd = (_rb(_rb(tk["y"]) * rs) * 0.5).astype(BF16)
    if CFG["tmode"] == 0:
        updt_s[:, pl.ds(0, 128)] = _u32(lax.dot_general(upd, jnp.eye(16, 128, dtype=BF16), (((0,), (0,)), ((), ())),
                                                        preferred_element_type=F32))
    else:
        upt_s[...] = jnp.concatenate([upd, jnp.zeros((16, 64), BF16)], axis=1).T
    mark('s9_final')
    hit = hit_s[0]
    for t in range(16):
        @pl.when(((hit >> t) & 1) == 1)
        def _():
            if CFG["tmode"] == 0:
                ohp = jnp.concatenate([_bf(oh_s[:, pl.ds(128 * t, 128)]), jnp.zeros((112, 128), BF16)], axis=0)
                du = _dot(_bf(updt_s[:, pl.ds(0, 128)]), ohp)
            else:
                du = _dot(upt_s[pl.ds(0, D), :], _bf(oh_s[:, pl.ds(128 * t, 128)]))
            for i in range(NS):
                fin16(i, t, t + 1, du[16 * i:16 * i + 16], False)
            for hf in range(len(o_cp)):
                o_cp[hf][t].start(priority=1)
    mark('sa_waito')
    for cps in o_cp:
        for cp in cps:
            cp.wait()
    mark(None)


@jax.jit
def pallas_recurrent_scan__ssm_conv_s4__moe_arch_mod__prompt_kernel(A_u, A_A_re, A_A_im, A_B_re, A_B_im, A_C_re, A_C_im, A_log_dt, A_Dskip,
              B_x, B_w_r, B_w_gate, B_w_up, B_w_down):
    xt = jnp.transpose(A_u[0])
    wdt = jnp.transpose(B_w_down)
    scratch = [
        pltpu.SMEM((1,), I32),
        pltpu.VMEM((D, L), BF16),
        pltpu.VMEM((6, D, N), BF16),
        pltpu.VMEM((D,), BF16),
        pltpu.VMEM((D,), BF16),
        pltpu.VMEM((D,), BF16),
        pltpu.VMEM((D // 2, FF), U32),
        pltpu.VMEM((D // 2, FF), U32),
        pltpu.VMEM((D // 2, FF), U32),
        pltpu.VMEM(_UM.shape, U32),
        pltpu.VMEM(_G0.shape, U32),
        pltpu.VMEM((336, 512), U32),
        pltpu.VMEM(_UM.shape, U32),
        pltpu.VMEM((D, 128), F32),
        pltpu.VMEM((D, 128), F32),
        pltpu.VMEM((D, 128), F32),
        pltpu.VMEM((D // 2, 896), U32),
        pltpu.VMEM((D // 2, L), U32),
        pltpu.VMEM((D // 2, L), U32),
        pltpu.VMEM((CFG['RU'], 5120), F32),
        pltpu.VMEM((CFG['RU'], 5120), F32),
        pltpu.VMEM((CFG['RU'], 5120), F32),
        pltpu.VMEM((D, L // 2), U32),
        pltpu.VMEM((D // 2, L), U32),
        pltpu.VMEM((64, D), F32),
        pltpu.VMEM((16, 128), F32),
        pltpu.VMEM((8, L), U32),
        pltpu.VMEM((8, D), U32),
        pltpu.SMEM((1,), I32),
        pltpu.VMEM((8, 128), U32),
        pltpu.VMEM((D, 128), F32),
        pltpu.VMEM((D // 2, 256), U32),
        pltpu.VMEM((16, D), F32),
        pltpu.VMEM((640, 16), BF16),
        pltpu.SemaphoreType.DMA((18,)),
        pltpu.SemaphoreType.DMA((3, len(FCH))),
        pltpu.SemaphoreType.DMA((2, 16)),
    ] + [pltpu.VMEM((RB, 4096), F32)] * NB
    out = pl.pallas_call(
        _kernel,
        out_shape=jax.ShapeDtypeStruct((D, L), BF16),
        in_specs=[pl.BlockSpec(memory_space=pl.ANY)] * 15,
        out_specs=pl.BlockSpec(memory_space=pl.ANY),
        scratch_shapes=scratch,
        compiler_params=pltpu.CompilerParams(vmem_limit_bytes=100 * 2**20, disable_semaphore_checks=True,
                                             disable_bounds_checks=True),
        name="s4_mod",
    )(xt, A_A_re, A_A_im, A_B_re, A_B_im, A_C_re, A_C_im, A_log_dt, A_Dskip,
      B_w_r, B_w_gate, B_w_up, wdt, jnp.asarray(_UM), jnp.asarray(_G0))
    return jnp.transpose(out)[None]
```

```python
import functools
import math

import numpy as np
import jax
import jax.numpy as jnp
from jax import lax
import jax.experimental.pallas as pl
import jax.experimental.pallas.tpu as pltpu

F32 = jnp.float32
BF16 = jnp.bfloat16
U32 = jnp.uint32
I32 = jnp.int32

D = 576
L = 2048
N = 128
FF = 4608
NSEL = 8
NCH = 8
RB = 64
NB = D // RB
NS = D // 16
SPB = RB // 16
FCH = (10, 10, 8, 6, 2)

_TILES = {
    "odd": (1, 3, 5, 7),
    "even": (2, 4, 6, 8),
    "t2": (258, 260, 262, 264),
    "t3": (516, 520, 772, 776),
    "t4": (1032, 1288, 1544, 1800),
}


def _rlag(l):
    u = int(np.float32(l).view(np.uint32))
    u = (u + 0x7FFF + ((u >> 16) & 1)) & 0xFFFF0000
    return int(np.uint32(u).view(np.float32))


def _tile_pts(name):
    base = name.rstrip("v")
    p = np.array([_TILES[base][l // 32] + 8 * (l % 32) for l in range(128)])
    if name == "t3v":
        p[127] = 512
    if name == "t4v":
        p[127] = 1024
    return p


def _sel_table():
    lags = np.concatenate([_tile_pts("odd"), _tile_pts("even")])
    sel = np.full((8, 256), -1, np.int32)
    for k, (c, tile) in enumerate([(1, "t2"), (2, "t3v"), (4, "t4v"), (1, "even")]):
        pts = _tile_pts(tile)
        for rho, r in enumerate(lags):
            idx = np.nonzero(pts == _rlag(256 * c + int(r)))[0]
            if len(idx):
                sel[k, rho] = idx[0]
    sel[4:] = 0
    return sel


_SEL = _sel_table()


def _bf(x):
    return pltpu.bitcast(x, BF16)


def _u32(x):
    return pltpu.bitcast(x.astype(BF16), U32)


def _rb(x):
    return x.astype(BF16).astype(F32)


def _cmul(a, b):
    return (a[0] * b[0] - a[1] * b[1], a[0] * b[1] + a[1] * b[0])


def _csq(a):
    t = a[0] * a[1]
    return (a[0] * a[0] - a[1] * a[1], t + t)


def _sincos(th):
    magic = 12582912.0
    kf = th * (2.0 / math.pi) + magic
    ki = pltpu.bitcast(kf, I32)
    k = kf - magic
    r = th - k * 1.5703125
    r = r - k * 4.837512969970703125e-4
    r = r - k * 7.54978995489188216e-8
    r2 = r * r
    s = r + r * r2 * (-1.6666654611e-1 + r2 * (8.3321608736e-3 + r2 * -1.9515295891e-4))
    c = 1.0 + r2 * (-0.5 + r2 * (4.166664568298827e-2 + r2 * (-1.388731625493765e-3 + r2 * 2.443315711809948e-5)))
    swap = (ki & 1) == 1
    sn = jnp.where(swap, c, s)
    cs = jnp.where(swap, s, c)
    sbit = (ki & 2) << 30
    cbit = ((ki + 1) & 2) << 30
    sn = pltpu.bitcast(pltpu.bitcast(sn, I32) ^ sbit, F32)
    cs = pltpu.bitcast(pltpu.bitcast(cs, I32) ^ cbit, F32)
    return cs, sn


def _dot(a, b):
    return jnp.dot(a, b, preferred_element_type=F32)


def _dot_nt(a, b):
    return lax.dot_general(a, b, (((1,), (1,)), ((), ())), preferred_element_type=F32)


def _col_bcast(vec_ref):
    v = vec_ref[...].astype(F32).reshape(1, D)
    vp = jnp.concatenate([v, jnp.zeros((1, 64), F32)], axis=1)
    return [jnp.broadcast_to(vp[:, t * 128:(t + 1) * 128], (128, 128)).T for t in range(5)]


def _base8(p, dt):
    are, aim, bre, bim, cre, cim = p
    y1 = (dt * are) * math.log2(math.e)
    ph = {1: _sincos(dt * aim)}
    e = 1
    while e < 512:
        ph[2 * e] = _csq(ph[e])
        e *= 2
    pw = {}
    for e in (1, 2, 4, 8, 16, 256, 512):
        mg = jnp.exp2(y1 * float(e)) if e > 1 else jnp.exp2(y1)
        pw[e] = (mg * ph[e][0], mg * ph[e][1])
    w = _cmul((cre, cim), (dt * bre, dt * bim))
    k0 = jnp.sum(w[0], axis=1, keepdims=True)
    w1 = _cmul(w, pw[1])
    w2 = _cmul(w1, pw[1])
    w3 = _cmul(w2, pw[1])
    w258 = _cmul(w2, pw[256])

    def rot(z):
        return (pltpu.roll(z[0], 4, 0), pltpu.roll(z[1], 4, 0))
    rots = {e: rot(pw[e]) for e in (2, 4, 8, 16, 512)}
    return (pw, rots, w1, w2, rot(w3), rot(w258)), k0


def _grp_xy(bs, grp, lo4):
    pw, rots, w1, w2, w3r, w258r = bs

    def sel(lo, hi):
        return (jnp.where(lo4, lo[0], hi[0]), jnp.where(lo4, lo[1], hi[1]))
    if grp == 0:
        dup = {e: sel(pw[e], rots[e]) for e in (2, 4, 16, 512)}
        x0, x2, a8 = sel(w1, w3r), sel(w2, w258r), rots[8]
    else:
        dup = {e: sel(rots[e], pw[e]) for e in (2, 4, 16, 512)}
        x0, x2, a8 = sel(w3r, w1), sel(w258r, w2), pw[8]
    xv = [None] * 10
    xv[0] = x0
    xv[1] = _cmul(x0, dup[4])
    xv[2] = x2
    xv[3] = _cmul(xv[2], dup[2])
    xv[4] = _cmul(xv[3], dup[2])
    xv[5] = _cmul(xv[4], dup[2])
    xv[6] = _cmul(xv[3], dup[512])
    xv[7] = _cmul(xv[5], dup[512])
    xv[8] = _cmul(xv[7], dup[512])
    xv[9] = _cmul(xv[8], dup[512])
    y = (jnp.where(lo4, 1.0, a8[0]), jnp.where(lo4, 0.0, -a8[1]))
    m = dup[16]
    ys = [y]
    for _ in range(15):
        y = (y[0] * m[0] + y[1] * m[1], y[1] * m[0] - y[0] * m[1])
        ys.append(y)

    def mat(vs):
        return jnp.concatenate([jnp.concatenate([v[0] for v in vs], 0),
                                jnp.concatenate([v[1] for v in vs], 0)], 1).astype(BF16)
    return mat(xv), mat(ys)


def _pk(a, b):
    return pltpu.pack_elementwise([a, b], packed_dtype=BF16)


def _upk(w, h):
    return pltpu.unpack_elementwise(w, index=h, packed_dtype=BF16, unpacked_dtype=F32)


_KT = [(0, 256, 0), (128, 256, 256), (384, 128, 512), (512, 128, 576),
       (640, 128, 704), (768, 128, 800), (768, 128, 768), (768, 128, 736)]

CFG = dict(merge=0, ffc=0, ffo=0, hold=0, mord=0, ktr0=(0, 1), tmode=1, n5=(2, 1, 1, 1, 1), xs_per=3, npre=0, kgr=(1, 5), n01=(3, 1), carry=1, r1=128, ktr1=(0, 1), ktr2=(1, 2), lnr=(1, 1), gg_at=3, xs_lag=16, fuse=1, flag=1, ffb=2, bw=[(0, 0), (24, 1), (49, 2)], hrows=0, wall=0, link=0, split=1, ktb=2, RU=16, gw=4, kt0=4, ffn_grp=(3, 1, 1), xsel_at=27, xw=22, kt_ln=4, pre=1, utpre=0, kdyn=1, ktag=0, kt_lag=1, utj=4, order=1, lag=1, lead=2, scopes=False)


def _kernel(x_hbm, are_hbm, aim_hbm, bre_hbm, bim_hbm, cre_hbm, cim_hbm, ldt_hbm, dsk_hbm,
            wr_hbm, wg_hbm, wu_hbm, wd_hbm, sel_hbm, out_hbm,
            zs, xb, prm, ldt, dsk, wr, wg, wu, wd, um, g0b, gm, selb,
            umt, dtc, dkc, k0c, kd, xh, vv, ur0, ur1, ur2, yb, ob, junk, rs_s, oh_s, xs_s, hit_s, zmk, deff, updt_s, ya_s, upt_s,
            sem_small, sem_w, sem_o, *ksps):
    urs = (ur0, ur1, ur2)
    _cur = [None]

    def mark(name):
        if not CFG["scopes"]:
            return
        if _cur[0] is not None:
            _cur[0].__exit__(None, None, None)
            _cur[0] = None
        if name:
            _cur[0] = jax.named_scope(name)
            _cur[0].__enter__()
    R1 = CFG["r1"]
    prs = [are_hbm, aim_hbm, bre_hbm, bim_hbm, cre_hbm, cim_hbm]
    order = (1, 0, 2, 3, 4, 5)
    grp0 = [(ldt_hbm, ldt), (sel_hbm, selb)]
    grp1 = [(prs[i].at[pl.ds(0, R1)], prm.at[i, pl.ds(0, R1)]) for i in order]
    grp2 = [(prs[i].at[pl.ds(R1, D - R1)], prm.at[i, pl.ds(R1, D - R1)]) for i in order]
    grp2 += [(dsk_hbm, dsk), (wr_hbm, wr)]
    grp3 = [(x_hbm, xb)]
    in_cp = []
    for grp in (grp0, grp1, grp2, grp3):
        n0 = sum(len(g) for g in in_cp)
        in_cp.append([pltpu.make_async_copy(s, d, sem_small.at[n0 + i]) for i, (s, d) in enumerate(grp)])
        for cp in in_cp[-1]:
            cp.start()
    w_cp = []
    off = 0
    for c, n in enumerate(FCH):
        cs = pl.ds(off * 128, n * 128)
        w_cp.append([pltpu.make_async_copy(h.at[:, cs], b.bitcast(BF16).at[:, cs], sem_w.at[i, c])
                     for i, (h, b) in enumerate([(wg_hbm, wg), (wu_hbm, wu), (wd_hbm, wd)])])
        for cp in w_cp[-1]:
            cp.start(priority=1)
        off += n

    class M:
        pass

    def masks():
        sub = lax.broadcasted_iota(I32, (8, 128), 0)
        lane = lax.broadcasted_iota(I32, (8, 128), 1)
        M.lo4 = sub < 4
        M.gidx = 4 * (lane % 32) + (sub % 4)
        M.lo64 = lane < 64
        M.beven = ((lane // 32) % 2) == 0
        M.last = lane == 127
        M.mz = jnp.where(lane == 0, 0.0, 1.0)
        M.row16 = lax.broadcasted_iota(I32, (16, 128), 0)
        M.lane16 = lax.broadcasted_iota(I32, (16, 128), 1)
    masks()

    def dft_tables():
        sub = lax.broadcasted_iota(I32, (8, 128), 0)
        lane = lax.broadcasted_iota(I32, (8, 128), 1)
        lo = lane < 64

        def e512(m):
            return _sincos((m & 511).astype(F32) * (-2.0 * math.pi / 512.0))

        def chain(base, step, n):
            out = [base]
            for _ in range(n - 1):
                out.append(_cmul(out[-1], step))
            return out

        def row(z, r):
            return tuple(jnp.broadcast_to(c[r:r + 1], (8, 128)) for c in z)

        def put(ref, r0, c0, vs):
            for i in range(0, len(vs), 2):
                ref[pl.ds(r0 + 4 * i, 8), pl.ds(c0, 128)] = _u32(jnp.concatenate([vs[i], vs[i + 1]], axis=0))
        f1 = 4 * lane + 1
        k4 = 4 * (lane & 63)
        alt_r = jnp.where((sub & 1) == 1, 1.0, -1.0)
        alt_l = jnp.where((lane & 1) == 1, 1.0, -1.0)
        b1 = e512(f1 * (sub + 1))
        c1 = chain(b1, row(b1, 7), 16)
        put(um, 0, 128, [z[0] for z in c1])
        put(um, 0, 384, [z[1] - z[0] for z in c1])
        put(um, 0, 512, [z[0] + z[1] for z in c1])
        for col, off, q in ((0, 0, jnp.where(lo, 0, 128)), (256, 2, jnp.where(lo, 128, 0))):
            b = e512((k4 + off) * (sub + 1))
            c = chain(e512((k4 + off) * (sub + 1) + q), row(b, 7), 16)
            vs = [z[0] for z in c]
            if off == 0:
                vs = [jnp.where(lane == 64, alt_r, v) for v in vs]
            put(um, 0, col, vs)
        st = e512(32 * (lane + 1))
        c = chain(e512((4 * sub + 1) * (lane + 1)), st, 16)
        put(umt, 0, 128, [z[0] for z in c])
        put(umt, 0, 384, [z[1] - z[0] for z in c])
        put(umt, 0, 512, [z[0] + z[1] for z in c])
        c = chain(e512(4 * sub * (lane + 1)), st, 8)
        re = [z[0] for z in c]
        im = [z[1] for z in c]
        re[0] = jnp.where(sub == 0, alt_l, re[0])
        im[0] = jnp.where(sub == 0, 1.0, im[0])
        put(umt, 0, 0, re + im)
        c = chain(e512((4 * sub + 2) * (lane + 1)), st, 8)
        put(umt, 0, 256, [z[1] for z in c] + [z[0] for z in c])
        for cls, f in ((0, f1), (1, k4 + jnp.where(lo, 0, 2))):
            b = e512(f * (1 + 8 * sub))
            s1_ = row(b, 0)
            s64 = e512(f * 64)
            cur = chain((b[0] * (1.0 / 128), b[1] * (1.0 / 128)), s64, 4)
            for lag in range(1, 9):
                re = [z[0] for z in cur]
                im = [z[1] for z in cur]
                if cls == 1:
                    sg = (-1.0) ** lag
                    re = [jnp.where(lane == 0, (-sg - 1.0) / 512, v) for v in re]
                    im = [jnp.where(lane == 0, (1.0 - sg) / 512, v) for v in im]
                r0 = 64 * ((lag - 1) % 2) + 16 * ((lag - 1) // 2)
                put(g0b, r0, 256 * cls, re)
                put(g0b, r0, 256 * cls + 128, im)
                if lag < 8:
                    cur = [_cmul(z, s1_) for z in cur]
    dft_tables()

    mark('s0_wait0')
    for cp in in_cp[0]:
        cp.wait()
    mark('s1_prep')
    zs[0] = selb[pl.ds(0, 8), pl.ds(0, 128)][4, 0]
    dtb = _col_bcast(ldt)
    for t in range(5):
        n = 128 if t < 4 else 64
        dtc[pl.ds(t * 128, n), :] = _rb(jnp.exp(dtb[t][:n]))
    mark('s2_waitp')
    for cp in in_cp[1]:
        cp.wait()
    mark('s3_A1')
    zo = [zs[0] * 8]

    def dyn(r):
        return pl.multiple_of(zo[0] + r, 8)

    inB = [False]

    def kt_unit(b, c):
        l0, kk, g0 = _KT[c]
        gw = g0b[pl.ds(0, 128), :] if c == 0 else gm[pl.ds((g0 - 256) // 2, kk // 2), :]
        raw = _dot(_bf(kd[pl.ds(b * (RB // 2), RB // 2), pl.ds(l0, kk)]), _bf(gw))
        rows = pl.ds(dyn(0), RB) if inB[0] else pl.ds(0, RB)
        ksps[b][rows, pl.ds(512 * c, 512)] = raw
        if CFG["ktag"]:
            tg = pltpu.roll(ksps[b][pl.ds(0, 8), pl.ds(512 * c, 128)], 1, 1)
            junk[pl.ds(8 * ((b * NCH + c) % 8), 8), :] = tg

    def ggen():
        sel = selb[...]

        def onehot(k, r0, n):
            ri = lax.broadcasted_iota(I32, (n, 256), 0) + r0
            return jnp.where(ri == sel[k:k + 1, :], 1.0, 0.0)
        e = jnp.concatenate([onehot(0, 0, 128), onehot(1, 0, 64), onehot(2, 0, 32),
                             onehot(1, 112, 16), onehot(2, 112, 16), onehot(3, 112, 16)], axis=0).astype(BF16)
        g = _dot(e, _bf(g0b[pl.ds(0, 128), :]))

        def put(r, v):
            gm[pl.ds((r - 256) // 2, v.shape[0] // 2), :] = _u32(v)

        def zero(r, n):
            gm[pl.ds((r - 256) // 2, n // 2), :] = jnp.zeros((n // 2, 512), U32)
        zero(256, 112)
        put(368, g[256:272])
        put(384, g[0:128])
        put(512, g[128:192])
        zero(576, 48)
        put(624, g[224:240])
        put(640, g[128:192])
        put(704, g[192:224])
        zero(736, 80)
        put(816, g[240:256])
        put(832, g[192:224])
        zero(864, 64)

    def extract(st, o4):
        g = [[jnp.take_along_axis(_pk(o4[0][grp][8 * v:8 * v + 8], o4[1][grp][8 * v:8 * v + 8]), M.gidx, axis=1,
                                  mode="promise_in_bounds") for v in range(10)] for grp in range(2)]

        def mix(a, b):
            return jnp.where(M.lo4, a, b), pltpu.roll(jnp.where(M.lo4, b, a), 4, 0)

        def two(va, vb, m1, m2):
            p, q = mix(jnp.where(m1, g[0][va], g[0][vb]), jnp.where(m1, g[1][va], g[1][vb]))
            return jnp.where(m2, p, q)

        def four(gg):
            return jnp.where(M.lo64, jnp.where(M.beven, gg[2], gg[3]), jnp.where(M.beven, gg[4], gg[5]))
        t_odd = two(0, 1, M.lo64, M.beven)
        t_even, t_2 = mix(four(g[0]), four(g[1]))
        t_3 = two(6, 7, M.beven, M.lo64)
        t_4 = two(8, 9, M.lo64, M.beven)
        tl = [t_odd, t_even, t_2, jnp.where(M.last, t_2, t_3), t_3, jnp.where(M.last, t_3, t_4), t_4]
        for t in range(7):
            kd[pl.ds(st * 8, 8), pl.ds(128 * t, 128)] = tl[t]

    tk = {}

    def ln_chunk(j):
        cj = slice(256 * j, 256 * j + 256)
        s1 = s2 = None
        for i in range(NS):
            v16 = xb[pl.ds(i * 16, 16), cj].astype(F32)
            for v in (v16[:8], v16[8:]):
                s1, s2 = (v, v * v) if s1 is None else (s1 + v, s2 + v * v)
        mean = jnp.sum(s1, axis=0, keepdims=True) * (1.0 / D)
        var = jnp.sum(s2, axis=0, keepdims=True) * (1.0 / D) - mean * mean
        var = jnp.maximum(var, 0.0)
        sd = _rb(jnp.sqrt(_rb(_rb(var) + 1e-5)))
        mb = jnp.broadcast_to(_rb(mean), (16, 256))
        hi = jnp.broadcast_to(0.5 / sd, (16, 256))
        if j == 0:
            wrow = wr[...].astype(F32).reshape(1, D)
            tk["w"] = [(jnp.broadcast_to(wrow[:, k0:min(k0 + 128, D)], (16, min(128, D - k0)))
                        + jnp.zeros((16, min(128, D - k0)), F32)).astype(BF16) for k0 in range(0, D, 128)]
        r = None
        for i in range(NS):
            rw = pl.ds(dyn(i * 8), 8)
            hv = _rb(xb[pl.ds(i * 16, 16), cj].astype(F32) - mb) * hi
            h0, h1 = hv[:, :128], hv[:, 128:]
            xh[rw, pl.ds(256 * j, 128)] = _u32(h0)
            xh[rw, pl.ds(256 * j + 128, 128)] = _u32(h1)
            rv = rw if CFG["merge"] else pl.ds(i * 8, 8)
            vv[rv, pl.ds(256 * j, 128)] = _u32(h0 + h1)
            vv[rv, pl.ds(256 * j + 128, 128)] = _u32(h0 - h1)
            if i % 8 == 7 or i == NS - 1:
                k0, k1 = (i // 8) * 128, (i + 1) * 16
                yield
                p = _dot(tk["w"][i // 8], _bf(xh[pl.ds(k0 // 2, (k1 - k0) // 2), cj]))
                r = p if r is None else r + p
        for t in range(2):
            r_t = r[:, 128 * t:128 * t + 128]
            tk["rc"] = r_t if (j == 0 and t == 0) else jnp.where(M.row16 == 2 * j + t, r_t, tk["rc"])

    def topk():
        bits = pltpu.bitcast(_rb(tk["rc"] * 2.0), I32)
        mono = (jnp.where(bits < 0, bits ^ 0x7FFF0000, bits) >> 16) + 32768
        key = pltpu.bitcast(0x30000000 + (mono << 11) + (2047 - (M.row16 * 128 + M.lane16)), F32)
        kcol = jnp.zeros((16, 128), I32)
        for j in range(NSEL):
            mx = jnp.max(jnp.max(key, axis=0, keepdims=True), axis=1, keepdims=True)
            mxb = jnp.broadcast_to(mx, (16, 128))
            key = jnp.where(key == mxb, 0.0, key)
            kcol = jnp.where(M.row16 == j, pltpu.bitcast(mxb, I32), kcol)
        kcol = kcol - 0x30000000
        idxcol = jnp.where(M.row16 < NSEL, 2047 - (kcol & 2047), -1)
        hb = ((kcol >> 11) - 32768) << 16
        rsel = pltpu.bitcast(jnp.where(hb < 0, hb ^ 0x7FFF0000, hb), F32)
        rsel = jnp.where(M.row16 < NSEL, rsel, 0.0)
        rs_s[...] = _rb(jax.nn.sigmoid(rsel))
        tk["oh"] = jnp.concatenate(
            [jnp.where(idxcol == M.lane16 + 128 * t, 1.0, 0.0) for t in range(16)], axis=1).astype(BF16)
        oh_s[...] = pltpu.bitcast(tk["oh"], U32)
        hb_ = jnp.where(M.row16[:8] < NSEL, jnp.left_shift(1, jnp.maximum(idxcol[:8], 0) >> 7), 0)
        for sh in (4, 2, 1):
            hb_ = hb_ | pltpu.roll(hb_, sh, 0)
        hit_s[0] = hb_[0, 0]
        tcol = jnp.maximum(idxcol, 0) >> 7
        tk["tj"] = [tcol[j, 0] for j in range(NSEL)]
        tk["ol"] = jnp.where((idxcol & 127) == M.lane16, 1.0, 0.0)

    def xsel(j):
        off = pl.multiple_of(tk["tj"][j] * 128, 128)
        lhs = jnp.where(M.row16 == j, tk["ol"], 0.0).astype(BF16)
        v = _dot_nt(lhs, _bf(xh[:, pl.ds(off, 128)]))
        tk["xa"] = v if j == 0 else tk["xa"] + v
        if j == NSEL - 1:
            xs_s[...] = _u32(tk["xa"] * 2.0)

    def link(v):
        if not CFG["link"]:
            return v
        w = pltpu.bitcast(v, U32)
        dep = ob[pl.ds(0, 8), pl.ds(0, 128)] & tk["zm"]
        return pltpu.bitcast(jnp.concatenate([w[:, :128] | dep, w[:, 128:]], axis=1), BF16)

    def ffn_gu(p, lk):
        cs = pl.ds(256 * p, 256)
        xs = link(tk["xs"]) if lk else tk["xs"]
        gu = _dot(xs, _bf(jnp.concatenate([wg[:, cs], wu[:, cs]], axis=1)))
        g = _rb(gu[:, :256])
        u = _rb(gu[:, 256:])
        sg = _rb(0.5 * jnp.tanh(0.5 * g) + 0.5)
        tk["h", p] = (_rb(g * sg) * u).astype(BF16)

    def ffn_dn(p, lk):
        h = tk.pop(("h", p))
        y = _dot_nt(link(h) if lk else h, _bf(wd[:, pl.ds(256 * p, 256)]))
        tk["y"] = y if p == 0 else tk["y"] + y

    def fin16(i, c0, c1, du, dynst):
        r16 = pl.ds(16 * i, 16)
        cs = pl.ds(128 * c0, 128 * (c1 - c0))
        h = _bf(xh[pl.ds(8 * i, 8), cs]).astype(F32)
        y = jnp.concatenate([_upk(yb[r16, pl.ds(256 * (c // 4) + 128 * (c % 2), 128)], (c // 2) % 2)
                             for c in range(c0, c1)], axis=1)
        dv = deff[r16, :]
        s_ = y + h * jnp.concatenate([dv] * (c1 - c0), axis=1)
        zh = h if du is None else h + du
        g = zh * jnp.tanh(zh) + zh
        rw = pl.ds(dyn(8 * i), 8) if dynst else pl.ds(8 * i, 8)
        ob[rw, cs] = _u32(xb[r16, cs].astype(F32) + s_ * g)

    utj = CFG["utj"]
    RU = CFG["RU"]

    def ut_piece(b, k, j0):
        rw = pl.ds(b * (RU // 2), RU // 2)
        rows = pl.ds(dyn(0), RU)
        ur = urs[b % 3]
        js = range(j0, j0 + utj)

        def lhs(ref, o):
            return _bf(jnp.concatenate([ref[rw, pl.ds(256 * j + o, 128)] for j in js], axis=0))

        def put(val, col):
            for i, j in enumerate(js):
                ur[rows, pl.ds(640 * j + col, 128)] = val[i * RU:(i + 1) * RU]
        if k == 0:
            v = _dot(lhs(vv, 0), _bf(um[:, 0:256]))
            b2 = _dot(lhs(vv, 128), _bf(um[:, 256:384]))
            a0 = v[:, :128]

            def sel(p, q):
                return jnp.concatenate([jnp.where(M.lo64, p[8 * i:8 * i + 8], q[8 * i:8 * i + 8])
                                        for i in range(a0.shape[0] // 8)], axis=0)
            put(sel(a0, b2), 0)
            put(v[:, 128:], 128)
            put(pltpu.roll(sel(b2, a0), 64, 1), 256)
        else:
            put(_dot(lhs(xh, 128), _bf(um[:, 384:512])), 384)
            put(_dot(lhs(xh, 0), _bf(um[:, 512:640])), 512)

    def mac(g, cls):
        ur = urs[(8 * g // RU) % 3]

        @functools.lru_cache(None)
        def us(j):
            def ld(c):
                return ur[pl.ds((8 * g) % RU, 8), pl.ds(640 * j + c, 128)]
            if cls == 0:
                a, b = ld(0), ld(256)
                return (a, b, a + b)
            t1, t2, t3 = ld(128), ld(384), ld(512)
            return (t1 + t2, t3 - t1, t2 + t3)

        @functools.lru_cache(None)
        def kraw(j):
            o = 512 * j + 256 * (1 - cls)
            ksp, kr = ksps[8 * g // RB], pl.ds((8 * g) % RB, 8)
            return ksp[kr, pl.ds(o, 128)], ksp[kr, pl.ds(o + 128, 128)]

        @functools.lru_cache(None)
        def ks(j):
            sr, si = kraw(j)
            if j > 0:
                pr, pi_ = kraw(j - 1)
                sr, si = (sr + pr, si + pi_) if cls == 0 else (sr - pr, si - pi_)
            return (sr * M.mz if cls == 0 else sr, si - sr, sr + si)
        outs = []
        prev = None
        for m in (range(NCH) if CFG["mord"] == 0 else range(NCH - 1, -1, -1)):
            acc = None
            for j in range(m + 1):
                a, b, s = us(j)
                c_, e_, g_ = ks(m - j)
                t = (c_ * s, a * e_, b * g_)
                acc = t if acc is None else tuple(x + y for x, y in zip(acc, t))
            z = (acc[0] - acc[2], acc[0] + acc[1])
            if (m % 2 == 1) == (CFG["mord"] == 0):
                za, zb = (prev, z) if CFG["mord"] == 0 else (z, prev)
                if cls == 0:
                    zr = _pk(za[0], zb[0])
                    zis = _pk(za[1], zb[1]) if CFG.get('nrz') else pltpu.roll(_pk(za[1], zb[1]), 64, 1)
                    outs.append((jnp.where(M.lo64, zr, zis), jnp.where(M.lo64, zis, zr)))
                else:
                    outs.append((_pk(za[0] + za[1], zb[0] + zb[1]), _pk(za[1], zb[1]), _pk(za[0], zb[0])))
            prev = z
        return outs if CFG['mord'] == 0 else outs[::-1]

    zq, wq = {}, {}

    def inv(g, cls):
        zo_ = zq.pop((g, cls))

        def st(t):
            return _bf(jnp.concatenate([zo_[p][t] for p in range(4)], axis=0))
        if cls == 0:
            wq[g] = [_dot(st(t), _bf(umt[:, c:c + 128])) for t, c in ((0, 0), (1, 256))]
        else:
            q1, q2, q3 = [_dot(st(t), _bf(umt[:, c:c + 128])) for t, c in ((0, 128), (1, 384), (2, 512))]
            w0, w2 = wq.pop(g)
            p_ = q1 + w2
            y0 = p_ + (q2 + w0)
            y1 = (q3 + w0) - p_
            yr = pl.ds(dyn(8 * g), 8) if CFG["fuse"] else pl.ds(8 * g, 8)
            for p in range(4):
                yb[yr, pl.ds(256 * p, 128)] = _u32(y0[16 * p:16 * p + 16])
                yb[yr, pl.ds(256 * p + 128, 128)] = _u32(y1[16 * p:16 * p + 16])

    ktq = []
    slotno = [0]
    pat = CFG.get("kt_pat", [1, 0, 1, 1, 0, 1, 0, 1, 1, 0, 1, 1, 0, 1, 0, 1])
    xw = CFG["xw"]

    def kt_drain(n):
        for _ in range(n):
            if ktq and ktq[0][0] <= slotno[0]:
                kt_unit(*ktq.pop(0)[1:])

    utq = [(b, k, j) for b in range(D // RU) for j in range(0, NCH, utj) for k in range(2)]
    pend = [None]

    pre_xy = {}

    def kxy(st, half):
        r0 = st * 16
        pk = [pltpu.bitcast(prm[k, pl.ds(r0, 16), :], U32) for k in range(6)]
        rows = pl.ds(r0 + half, 8, stride=2)
        bs, k0 = _base8([_upk(w, half) for w in pk], dtc[rows, :])
        k0c[rows, :] = jnp.broadcast_to(k0, (8, 128))
        return [_grp_xy(bs, grp, M.lo4) for grp in range(2)]

    def kgen(s0, s1):
        for st in range(s0, s1):
            o4 = []
            for half in range(2):
                xy = pre_xy.pop((st, half)) if (st, half) in pre_xy else kxy(st, half)
                if half == 0 and pend[0] is not None:
                    flush()
                oo = []
                for grp in range(2):
                    yield
                    slotno[0] += 1
                    oo.append(_dot_nt(*xy[grp]))
                o4.append(oo)
            pend[0] = (st, o4)
        if s1 == NS or not CFG["carry"]:
            flush()
        else:
            for h in range(CFG["npre"]):
                pre_xy[(s1 + h // 2, h % 2)] = kxy(s1 + h // 2, h % 2)

    def flush():
        extract(*pend[0])
        if (pend[0][0] + 1) % SPB == 0:
            ktq.extend([(slotno[0] + 4 * CFG["kt_lag"], pend[0][0] // SPB, c) for c in range(NCH)])
        pend[0] = None

    def region(name, fn):
        def body():
            masks()
            mark(name)
            fn()
            mark(None)
        if CFG["split"]:
            pl.when(zs[0] == 0)(body)
        else:
            body()

    def consts():
        dkb = _col_bcast(dsk)
        for t in range(5):
            n = 128 if t < 4 else 64
            dkc[pl.ds(t * 128, n), :] = dkb[t][:n]

    def rate(num, den):
        acc = [0]

        def step():
            acc[0] += num
            n = acc[0] // den
            acc[0] -= n * den
            return n
        return step

    only = CFG.get("only")
    doA = only in (None, "A")
    s1 = R1 // 16 - (CFG['npre'] + 1) // 2
    if doA:
        ktr = rate(*CFG["ktr0"])
        for i, _ in enumerate(kgen(0, s1)):
            if i == CFG["gg_at"]:
                ggen()
            if i > CFG["gg_at"]:
                kt_drain(ktr())
    mark('s3_w2')
    for cp in in_cp[2]:
        cp.wait()
    mark('s3_A1b')
    if doA:
        slotno[0] += 100
        ktr = rate(*CFG["ktr1"])
        for i, _ in enumerate(kgen(s1, xw)):
            kt_drain(ktr())
        consts()
    mark('s4_waitx')
    in_cp[3][0].wait()
    mark(None)

    def phase_a2():
        slotno[0] += 100
        kg = kgen(xw, NS)
        kgr = rate(*CFG["kgr"])
        for _ in range(CFG["pre"]):
            next(kg)
        for j in range(NCH):
            for k, _ in enumerate(ln_chunk(j)):
                kt_drain(CFG["n5"][k])
                for _ in range(kgr()):
                    next(kg)
        topk()
        ktr = rate(*CFG["ktr2"])
        xq = list(range(NSEL))
        for i, _ in enumerate(kg):
            kt_drain(ktr())
            if i >= CFG["xs_lag"] and xq and (i - CFG["xs_lag"]) % CFG["xs_per"] == 0:
                xsel(xq.pop(0))
        while xq:
            xsel(xq.pop(0))
        slotno[0] += 1000
        kt_drain(len(ktq) - NCH)

    ffp = [0, 0]

    def ffn_next():
        if ffp[1] < ffp[0] - 1 or (ffp[1] < ffp[0] and ffp[0] >= ffp_max[0]):
            ffn_dn(ffp[1], False)
            ffp[1] += 1
        elif ffp[0] < ffp_max[0]:
            ffn_gu(ffp[0], False)
            ffp[0] += 1
    ffp_max = [0]
    utdue = [0]
    GEND_ = D // 8 + CFG['lag'] + CFG['flag'] + 2

    def phase_b(g0, g1):
        inB[0] = True
        lag = CFG["lag"]
        NG = D // 8
        if g0 == 0:
            npre = 16 // utj + (2 * CFG["lead"] * 64 // RU) // utj
            for i in range(0 if CFG["utpre"] else npre):
                ut_piece(*utq.pop(0))
            if CFG["fuse"]:
                for t in range(5):
                    n = 128 if t < 4 else 64
                    deff[pl.ds(128 * t, n), :] = (dkc[pl.ds(128 * t, n), :] + k0c[pl.ds(128 * t, n), :]) * 2.0
        fl = CFG["flag"]
        for s in range(g0, g1):
            for cls in range(2):
                if s < NG:
                    zq[(s, cls)] = mac(s, cls)
                if CFG["order"] == 1 and lag <= s < NG + lag:
                    inv(s - lag, cls)
                if ((2 * s + cls) * 64 // RU) % utj == 0:
                    utdue[0] += max(1, 64 // RU // utj)
                if not (g1 < GEND_ and 2 * (g1 - s) - cls <= CFG["hold"]):
                    while utdue[0] and utq:
                        utdue[0] -= 1
                        ut_piece(*utq.pop(0))
                if cls == 1 and s % 4 == CFG["ktb"] % 4 and s >= CFG["ktb"]:
                    kt_drain(1)
                if CFG["order"] == 0 and lag <= s < NG + lag:
                    inv(s - lag, cls)
                if CFG["fuse"]:
                    q = 2 * (s - lag - fl) + cls - 2
                    if 0 <= q < 4 * NS:
                        fin16(q // 4, 4 * (q % 4), 4 * (q % 4) + 4, None, False)
                if CFG["ffb"] and cls == CFG["ffc"] and (s - g0) % CFG["ffb"] == CFG["ffo"] % CFG["ffb"]:
                    ffn_next()

    merge = CFG["merge"] and only is None
    if merge:
        inB[0] = True
    elif only in (None, "A"):
        region('s5_A2', phase_a2)
    elif only == "B":
        ktq.extend([(0, NB - 1, c) for c in range(NCH)])
    HR = CFG["hrows"]
    obb = ob.bitcast(BF16)
    o_cp = [[pltpu.make_async_copy(obb.at[pl.ds(r0, n), pl.ds(128 * t, 128)],
                                   out_hbm.at[pl.ds(r0, n), pl.ds(128 * t, 128)], sem_o.at[hf, t])
             for t in range(16)] for hf, (r0, n) in enumerate([(0, HR), (HR, D - HR)] if HR else [(0, D)])]

    def start_free(hf):
        hit = hit_s[0]
        for t in range(16):
            @pl.when(((hit >> t) & 1) == 0)
            def _():
                o_cp[hf][t].start(priority=1)

    GEND = D // 8 + CFG["lag"] + CFG["flag"] + 2
    if only in (None, "B"):
        def pb():
            if merge:
                phase_a2()
            g = 0
            for gs, cc in CFG["bw"]:
                if gs > g:
                    phase_b(g, gs)
                    g = gs
                if cc == len(CFG["bw"]) - 1 and only is None and HR:
                    assert (2 * (gs - 1 - CFG["lag"] - CFG["flag"]) + 1 - 2 + 1) // 4 * 16 >= HR
                    start_free(0)
                mark(f's7_w{cc}')
                if not (merge and cc == 0):
                    for cp in w_cp[cc]:
                        cp.wait()
                mark(f's7_B{cc}')
                ffp_max[0] = sum(FCH[:cc + 1]) // 2
                tk["xs"] = _bf(xs_s[...])
            phase_b(g, GEND)
            while CFG["ffb"] and ffp[1] < ffp_max[0]:
                ffn_next()
            if CFG["ffb"]:
                ya_s[...] = tk["y"]
        region('s7_B', pb)
    if only in ("A", "B"):
        for cc in range(len(CFG["bw"]), len(FCH)):
            for cp in w_cp[cc]:
                cp.wait()
        cp = pltpu.make_async_copy(ob.bitcast(BF16), out_hbm, sem_o.at[0, 0])
        cp.start()
        cp.wait()
        cp = pltpu.make_async_copy(yb.bitcast(BF16).at[pl.ds(0, D), :], out_hbm.at[:, pl.ds(0, 1024)], sem_o.at[0, 0])
        cp.start()
        cp.wait()
        for kk in ksps:
            cp = pltpu.make_async_copy(kk.at[:, pl.ds(0, 512)], junk.at[:, pl.ds(0, 512)], sem_o.at[0, 0])
            cp.start()
            cp.wait()
        for kk in (vv, xs_s, kd, umt):
            cp = pltpu.make_async_copy(kk.at[pl.ds(0, 8), pl.ds(0, 512)], oh_s.at[:, pl.ds(0, 512)], sem_o.at[0, 0])
            cp.start()
            cp.wait()
        cp = pltpu.make_async_copy(ya_s, junk.at[pl.ds(0,16), :], sem_o.at[0, 0])
        cp.start()
        cp.wait()
        return
    masks()
    tk["xs"] = _bf(xs_s[...])
    tk["rs"] = rs_s[...]
    tk["oh"] = _bf(oh_s[...])

    mark('s8_ffn')
    start_free(len(o_cp) - 1)
    tk["y"] = ya_s[...]
    for cc in range(len(CFG["bw"]), len(FCH)):
        lastc = cc == len(FCH) - 1
        mark(f's8_w{cc}')
        for cp in (w_cp[cc][:2] if lastc else w_cp[cc]):
            cp.wait()
        mark(f's8_f{cc}')
        ffp_max[0] = sum(FCH[:cc + 1]) // 2
        while ffp[0] < ffp_max[0]:
            ffn_gu(ffp[0], False)
            ffp[0] += 1
            if ffp[1] < ffp[0] - 1 and not lastc:
                ffn_dn(ffp[1], False)
                ffp[1] += 1
        if lastc:
            mark('s8_w5')
            w_cp[cc][2].wait()
            mark('s8_f5')
        while ffp[1] < ffp[0]:
            ffn_dn(ffp[1], False)
            ffp[1] += 1
    rs = jnp.concatenate([tk["rs"]] * 5, axis=1)[:, :D]
    upd = (_rb(_rb(tk["y"]) * rs) * 0.5).astype(BF16)
    if CFG["tmode"] == 0:
        updt_s[:, pl.ds(0, 128)] = _u32(lax.dot_general(upd, jnp.eye(16, 128, dtype=BF16), (((0,), (0,)), ((), ())),
                                                        preferred_element_type=F32))
    else:
        upt_s[...] = jnp.concatenate([upd, jnp.zeros((16, 64), BF16)], axis=1).T
    mark('s9_final')
    hit = hit_s[0]
    for t in range(16):
        @pl.when(((hit >> t) & 1) == 1)
        def _():
            if CFG["tmode"] == 0:
                ohp = jnp.concatenate([_bf(oh_s[:, pl.ds(128 * t, 128)]), jnp.zeros((112, 128), BF16)], axis=0)
                du = _dot(_bf(updt_s[:, pl.ds(0, 128)]), ohp)
            else:
                du = _dot(upt_s[pl.ds(0, D), :], _bf(oh_s[:, pl.ds(128 * t, 128)]))
            for i in range(NS):
                fin16(i, t, t + 1, du[16 * i:16 * i + 16], False)
            for hf in range(len(o_cp)):
                o_cp[hf][t].start(priority=1)
    mark('sa_waito')
    for cps in o_cp:
        for cp in cps:
            cp.wait()
    mark(None)


@jax.jit
def pallas_recurrent_scan__ssm_conv_s4__moe_arch_mod__prompt_kernel(A_u, A_A_re, A_A_im, A_B_re, A_B_im, A_C_re, A_C_im, A_log_dt, A_Dskip,
              B_x, B_w_r, B_w_gate, B_w_up, B_w_down):
    xt = jnp.transpose(A_u[0])
    wdt = jnp.transpose(B_w_down)
    scratch = [
        pltpu.SMEM((1,), I32),
        pltpu.VMEM((D, L), BF16),
        pltpu.VMEM((6, D, N), BF16),
        pltpu.VMEM((D,), BF16),
        pltpu.VMEM((D,), BF16),
        pltpu.VMEM((D,), BF16),
        pltpu.VMEM((D // 2, FF), U32),
        pltpu.VMEM((D // 2, FF), U32),
        pltpu.VMEM((D // 2, FF), U32),
        pltpu.VMEM((64, 640), U32),
        pltpu.VMEM((128, 512), U32),
        pltpu.VMEM((336, 512), U32),
        pltpu.VMEM((8, 256), I32),
        pltpu.VMEM((64, 640), U32),
        pltpu.VMEM((D, 128), F32),
        pltpu.VMEM((D, 128), F32),
        pltpu.VMEM((D, 128), F32),
        pltpu.VMEM((D // 2, 896), U32),
        pltpu.VMEM((D // 2, L), U32),
        pltpu.VMEM((D // 2, L), U32),
        pltpu.VMEM((CFG['RU'], 5120), F32),
        pltpu.VMEM((CFG['RU'], 5120), F32),
        pltpu.VMEM((CFG['RU'], 5120), F32),
        pltpu.VMEM((D, L // 2), U32),
        pltpu.VMEM((D // 2, L), U32),
        pltpu.VMEM((64, D), F32),
        pltpu.VMEM((16, 128), F32),
        pltpu.VMEM((8, L), U32),
        pltpu.VMEM((8, D), U32),
        pltpu.SMEM((1,), I32),
        pltpu.VMEM((8, 128), U32),
        pltpu.VMEM((D, 128), F32),
        pltpu.VMEM((D // 2, 256), U32),
        pltpu.VMEM((16, D), F32),
        pltpu.VMEM((640, 16), BF16),
        pltpu.SemaphoreType.DMA((17,)),
        pltpu.SemaphoreType.DMA((3, len(FCH))),
        pltpu.SemaphoreType.DMA((2, 16)),
    ] + [pltpu.VMEM((RB, 4096), F32)] * NB
    out = pl.pallas_call(
        _kernel,
        out_shape=jax.ShapeDtypeStruct((D, L), BF16),
        in_specs=[pl.BlockSpec(memory_space=pl.ANY)] * 14,
        out_specs=pl.BlockSpec(memory_space=pl.ANY),
        scratch_shapes=scratch,
        compiler_params=pltpu.CompilerParams(vmem_limit_bytes=100 * 2**20, disable_semaphore_checks=True,
                                             disable_bounds_checks=True),
        name="s4_mod",
    )(xt, A_A_re, A_A_im, A_B_re, A_B_im, A_C_re, A_C_im, A_log_dt, A_Dskip,
      B_w_r, B_w_gate, B_w_up, wdt, jnp.asarray(_SEL))
    return jnp.transpose(out)[None]
```

```python
import functools
import math

import numpy as np
import jax
import jax.numpy as jnp
from jax import lax
import jax.experimental.pallas as pl
import jax.experimental.pallas.tpu as pltpu

F32 = jnp.float32
BF16 = jnp.bfloat16
U32 = jnp.uint32
I32 = jnp.int32

D = 576
L = 2048
N = 128
FF = 4608
NSEL = 8
NCH = 8
RB = 64
NB = D // RB
NS = D // 16
SPB = RB // 16
FCH = (10, 10, 8, 8)

_TILES = {
    "odd": (1, 3, 5, 7),
    "even": (2, 4, 6, 8),
    "t2": (258, 260, 262, 264),
    "t3": (516, 520, 772, 776),
    "t4": (1032, 1288, 1544, 1800),
}


def _rlag(l):
    u = int(np.float32(l).view(np.uint32))
    u = (u + 0x7FFF + ((u >> 16) & 1)) & 0xFFFF0000
    return int(np.uint32(u).view(np.float32))


def _tile_pts(name):
    base = name.rstrip("v")
    p = np.array([_TILES[base][l // 32] + 8 * (l % 32) for l in range(128)])
    if name == "t3v":
        p[127] = 512
    if name == "t4v":
        p[127] = 1024
    return p


def _sel_table():
    lags = np.concatenate([_tile_pts("odd"), _tile_pts("even")])
    sel = np.full((8, 256), -1, np.int32)
    for k, (c, tile) in enumerate([(1, "t2"), (2, "t3v"), (4, "t4v"), (1, "even")]):
        pts = _tile_pts(tile)
        for rho, r in enumerate(lags):
            idx = np.nonzero(pts == _rlag(256 * c + int(r)))[0]
            if len(idx):
                sel[k, rho] = idx[0]
    sel[4:] = 0
    return sel


_SEL = _sel_table()


def _bf(x):
    return pltpu.bitcast(x, BF16)


def _u32(x):
    return pltpu.bitcast(x.astype(BF16), U32)


def _rb(x):
    return x.astype(BF16).astype(F32)


def _cmul(a, b):
    return (a[0] * b[0] - a[1] * b[1], a[0] * b[1] + a[1] * b[0])


def _csq(a):
    t = a[0] * a[1]
    return (a[0] * a[0] - a[1] * a[1], t + t)


def _sincos(th):
    magic = 12582912.0
    kf = th * (2.0 / math.pi) + magic
    ki = pltpu.bitcast(kf, I32)
    k = kf - magic
    r = th - k * 1.5703125
    r = r - k * 4.837512969970703125e-4
    r = r - k * 7.54978995489188216e-8
    r2 = r * r
    s = r + r * r2 * (-1.6666654611e-1 + r2 * (8.3321608736e-3 + r2 * -1.9515295891e-4))
    c = 1.0 + r2 * (-0.5 + r2 * (4.166664568298827e-2 + r2 * (-1.388731625493765e-3 + r2 * 2.443315711809948e-5)))
    swap = (ki & 1) == 1
    sn = jnp.where(swap, c, s)
    cs = jnp.where(swap, s, c)
    sbit = (ki & 2) << 30
    cbit = ((ki + 1) & 2) << 30
    sn = pltpu.bitcast(pltpu.bitcast(sn, I32) ^ sbit, F32)
    cs = pltpu.bitcast(pltpu.bitcast(cs, I32) ^ cbit, F32)
    return cs, sn


def _dot(a, b):
    return jnp.dot(a, b, preferred_element_type=F32)


def _dot_nt(a, b):
    return lax.dot_general(a, b, (((1,), (1,)), ((), ())), preferred_element_type=F32)


def _col_bcast(vec_ref):
    v = vec_ref[...].astype(F32).reshape(1, D)
    vp = jnp.concatenate([v, jnp.zeros((1, 64), F32)], axis=1)
    return [jnp.broadcast_to(vp[:, t * 128:(t + 1) * 128], (128, 128)).T for t in range(5)]


def _base8(p, dt):
    are, aim, bre, bim, cre, cim = p
    y1 = (dt * are) * math.log2(math.e)
    ph = {1: _sincos(dt * aim)}
    e = 1
    while e < 512:
        ph[2 * e] = _csq(ph[e])
        e *= 2
    pw = {}
    for e in (1, 2, 4, 8, 16, 256, 512):
        mg = jnp.exp2(y1 * float(e)) if e > 1 else jnp.exp2(y1)
        pw[e] = (mg * ph[e][0], mg * ph[e][1])
    w = _cmul((cre, cim), (dt * bre, dt * bim))
    k0 = jnp.sum(w[0], axis=1, keepdims=True)
    w1 = _cmul(w, pw[1])
    w2 = _cmul(w1, pw[1])
    w3 = _cmul(w2, pw[1])
    w258 = _cmul(w2, pw[256])

    def rot(z):
        return (pltpu.roll(z[0], 4, 0), pltpu.roll(z[1], 4, 0))
    rots = {e: rot(pw[e]) for e in (2, 4, 8, 16, 512)}
    return (pw, rots, w1, w2, rot(w3), rot(w258)), k0


def _grp_xy(bs, grp, lo4):
    pw, rots, w1, w2, w3r, w258r = bs

    def sel(lo, hi):
        return (jnp.where(lo4, lo[0], hi[0]), jnp.where(lo4, lo[1], hi[1]))
    if grp == 0:
        dup = {e: sel(pw[e], rots[e]) for e in (2, 4, 16, 512)}
        x0, x2, a8 = sel(w1, w3r), sel(w2, w258r), rots[8]
    else:
        dup = {e: sel(rots[e], pw[e]) for e in (2, 4, 16, 512)}
        x0, x2, a8 = sel(w3r, w1), sel(w258r, w2), pw[8]
    xv = [None] * 10
    xv[0] = x0
    xv[1] = _cmul(x0, dup[4])
    xv[2] = x2
    xv[3] = _cmul(xv[2], dup[2])
    xv[4] = _cmul(xv[3], dup[2])
    xv[5] = _cmul(xv[4], dup[2])
    xv[6] = _cmul(xv[3], dup[512])
    xv[7] = _cmul(xv[5], dup[512])
    xv[8] = _cmul(xv[7], dup[512])
    xv[9] = _cmul(xv[8], dup[512])
    y = (jnp.where(lo4, 1.0, a8[0]), jnp.where(lo4, 0.0, -a8[1]))
    m = dup[16]
    ys = [y]
    for _ in range(15):
        y = (y[0] * m[0] + y[1] * m[1], y[1] * m[0] - y[0] * m[1])
        ys.append(y)

    def mat(vs):
        return jnp.concatenate([jnp.concatenate([v[0] for v in vs], 0),
                                jnp.concatenate([v[1] for v in vs], 0)], 1).astype(BF16)
    return mat(xv), mat(ys)


def _pk(a, b):
    return pltpu.pack_elementwise([a, b], packed_dtype=BF16)


def _upk(w, h):
    return pltpu.unpack_elementwise(w, index=h, packed_dtype=BF16, unpacked_dtype=F32)


_KT = [(0, 256, 0), (128, 256, 256), (384, 128, 512), (512, 128, 576),
       (640, 128, 704), (768, 128, 800), (768, 128, 768), (768, 128, 736)]

CFG = dict(zsrc=3, udyn=1, ydyn=0, xdyn=0, wcast=1, ocast=0, sf_late=1, tailp=0, merge=0, ffc=0, ffo=0, hold=0, mord=0, ktr0=(0, 1), tmode=1, n5=(2, 1, 1, 1, 1), xs_per=3, npre=0, kgr=(1, 5), n01=(3, 1), carry=1, r1=128, ktr1=(0, 1), ktr2=(1, 2), lnr=(1, 1), gg_at=3, xs_lag=16, fuse=1, flag=1, ffb=2, bw=[(0, 0), (24, 1), (49, 2)], hrows=0, wall=0, link=0, split=1, ktb=2, RU=16, gw=4, kt0=4, ffn_grp=(3, 1, 1), xsel_at=27, xw=22, kt_ln=4, pre=1, utpre=0, kdyn=1, ktag=0, kt_lag=1, utj=4, order=1, lag=1, lead=2, scopes=False)


def _kernel(x_hbm, are_hbm, aim_hbm, bre_hbm, bim_hbm, cre_hbm, cim_hbm, ldt_hbm, dsk_hbm,
            wr_hbm, wg_hbm, wu_hbm, wd_hbm, sel_hbm, out_hbm,
            zs, xb, prm, ldt, dsk, wr, um, g0b, gm, selb,
            umt, dtc, dkc, k0c, kd, xh, vv, ur0, ur1, ur2, yb, ob, junk, rs_s, oh_s, xs_s, hit_s, zmk, deff, updt_s, ya_s, upt_s,
            sem_small, sem_w, sem_o, *rest):
    ksps = rest[:NB]
    wbuf = [rest[NB + 3 * c:NB + 3 * c + 3] for c in range(len(FCH))]
    urs = (ur0, ur1, ur2)
    _cur = [None]

    def mark(name):
        if not CFG["scopes"]:
            return
        if _cur[0] is not None:
            _cur[0].__exit__(None, None, None)
            _cur[0] = None
        if name:
            _cur[0] = jax.named_scope(name)
            _cur[0].__enter__()
    R1 = CFG["r1"]
    prs = [are_hbm, aim_hbm, bre_hbm, bim_hbm, cre_hbm, cim_hbm]
    order = (1, 0, 2, 3, 4, 5)
    grp0 = [(ldt_hbm, ldt), (sel_hbm, selb)]
    grp1 = [(prs[i].at[pl.ds(0, R1)], prm.at[i, pl.ds(0, R1)]) for i in order]
    grp2 = [(prs[i].at[pl.ds(R1, D - R1)], prm.at[i, pl.ds(R1, D - R1)]) for i in order]
    grp2 += [(dsk_hbm, dsk), (wr_hbm, wr)]
    grp3 = [(x_hbm, xb)]
    in_cp = []
    for grp in (grp0, grp1, grp2, grp3):
        n0 = sum(len(g) for g in in_cp)
        in_cp.append([pltpu.make_async_copy(s, d, sem_small.at[n0 + i]) for i, (s, d) in enumerate(grp)])
        for cp in in_cp[-1]:
            cp.start()
    w_cp = []
    off = 0
    for c, n in enumerate(FCH):
        cs = pl.ds(off * 128, n * 128)
        w_cp.append([pltpu.make_async_copy(h.at[:, cs], wbuf[c][i].bitcast(BF16) if CFG["wcast"] else wbuf[c][i], sem_w.at[i, c])
                     for i, h in enumerate([wg_hbm, wu_hbm, wd_hbm])])
        for cp in w_cp[-1]:
            cp.start(priority=1)
        off += n

    class M:
        pass

    def masks():
        sub = lax.broadcasted_iota(I32, (8, 128), 0)
        lane = lax.broadcasted_iota(I32, (8, 128), 1)
        M.lo4 = sub < 4
        M.gidx = 4 * (lane % 32) + (sub % 4)
        M.lo64 = lane < 64
        M.beven = ((lane // 32) % 2) == 0
        M.last = lane == 127
        M.mz = jnp.where(lane == 0, 0.0, 1.0)
        M.row16 = lax.broadcasted_iota(I32, (16, 128), 0)
        M.lane16 = lax.broadcasted_iota(I32, (16, 128), 1)
    masks()

    def dft_tables():
        sub = lax.broadcasted_iota(I32, (8, 128), 0)
        lane = lax.broadcasted_iota(I32, (8, 128), 1)
        lo = lane < 64

        def e512(m):
            return _sincos((m & 511).astype(F32) * (-2.0 * math.pi / 512.0))

        def chain(base, step, n):
            out = [base]
            for _ in range(n - 1):
                out.append(_cmul(out[-1], step))
            return out

        def row(z, r):
            return tuple(jnp.broadcast_to(c[r:r + 1], (8, 128)) for c in z)

        def put(ref, r0, c0, vs):
            for i in range(0, len(vs), 2):
                ref[pl.ds(r0 + 4 * i, 8), pl.ds(c0, 128)] = _u32(jnp.concatenate([vs[i], vs[i + 1]], axis=0))
        f1 = 4 * lane + 1
        k4 = 4 * (lane & 63)
        alt_r = jnp.where((sub & 1) == 1, 1.0, -1.0)
        alt_l = jnp.where((lane & 1) == 1, 1.0, -1.0)
        b1 = e512(f1 * (sub + 1))
        c1 = chain(b1, row(b1, 7), 16)
        put(um, 0, 128, [z[0] for z in c1])
        put(um, 0, 384, [z[1] - z[0] for z in c1])
        put(um, 0, 512, [z[0] + z[1] for z in c1])
        for col, off, q in ((0, 0, jnp.where(lo, 0, 128)), (256, 2, jnp.where(lo, 128, 0))):
            b = e512((k4 + off) * (sub + 1))
            c = chain(e512((k4 + off) * (sub + 1) + q), row(b, 7), 16)
            vs = [z[0] for z in c]
            if off == 0:
                vs = [jnp.where(lane == 64, alt_r, v) for v in vs]
            put(um, 0, col, vs)
        st = e512(32 * (lane + 1))
        c = chain(e512((4 * sub + 1) * (lane + 1)), st, 16)
        put(umt, 0, 128, [z[0] for z in c])
        put(umt, 0, 384, [z[1] - z[0] for z in c])
        put(umt, 0, 512, [z[0] + z[1] for z in c])
        c = chain(e512(4 * sub * (lane + 1)), st, 8)
        re = [z[0] for z in c]
        im = [z[1] for z in c]
        re[0] = jnp.where(sub == 0, alt_l, re[0])
        im[0] = jnp.where(sub == 0, 1.0, im[0])
        put(umt, 0, 0, re + im)
        c = chain(e512((4 * sub + 2) * (lane + 1)), st, 8)
        put(umt, 0, 256, [z[1] for z in c] + [z[0] for z in c])
        for cls, f in ((0, f1), (1, k4 + jnp.where(lo, 0, 2))):
            b = e512(f * (1 + 8 * sub))
            s1_ = row(b, 0)
            s64 = e512(f * 64)
            cur = chain((b[0] * (1.0 / 128), b[1] * (1.0 / 128)), s64, 4)
            for lag in range(1, 9):
                re = [z[0] for z in cur]
                im = [z[1] for z in cur]
                if cls == 1:
                    sg = (-1.0) ** lag
                    re = [jnp.where(lane == 0, (-sg - 1.0) / 512, v) for v in re]
                    im = [jnp.where(lane == 0, (1.0 - sg) / 512, v) for v in im]
                r0 = 64 * ((lag - 1) % 2) + 16 * ((lag - 1) // 2)
                put(g0b, r0, 256 * cls, re)
                put(g0b, r0, 256 * cls + 128, im)
                if lag < 8:
                    cur = [_cmul(z, s1_) for z in cur]
    dft_tables()

    mark('s0_wait0')
    for cp in in_cp[0]:
        cp.wait()
    mark('s1_prep')
    zs[0] = {0: lambda: jnp.int32(0), 1: lambda: pl.program_id(0), 2: lambda: selb[pl.ds(0, 8), pl.ds(0, 128)][4, 0],
             3: lambda: lax.broadcasted_iota(I32, (8, 128), 1)[0, 0],
             4: lambda: jnp.min(lax.broadcasted_iota(I32, (8, 128), 1).astype(F32)).astype(I32)}[CFG['zsrc']]()
    dtb = _col_bcast(ldt)
    for t in range(5):
        n = 128 if t < 4 else 64
        dtc[pl.ds(t * 128, n), :] = _rb(jnp.exp(dtb[t][:n]))
    mark('s2_waitp')
    for cp in in_cp[1]:
        cp.wait()
    mark('s3_A1')
    if CFG.get('zaddr'):
        hit_s[0] = jnp.int32(0)
        zo = [hit_s[0] * 8]
    else:
        zo = [zs[0] * 8]

    def dyn(r):
        return pl.multiple_of(zo[0] + r, 8)

    inB = [False]

    def kt_unit(b, c):
        l0, kk, g0 = _KT[c]
        gw = g0b[pl.ds(0, 128), :] if c == 0 else gm[pl.ds((g0 - 256) // 2, kk // 2), :]
        raw = _dot(_bf(kd[pl.ds(b * (RB // 2), RB // 2), pl.ds(l0, kk)]), _bf(gw))
        rows = pl.ds(dyn(0), RB) if (inB[0] and CFG['kdyn']) else pl.ds(0, RB)
        ksps[b][rows, pl.ds(512 * c, 512)] = raw
        if CFG["ktag"]:
            tg = pltpu.roll(ksps[b][pl.ds(0, 8), pl.ds(512 * c, 128)], 1, 1)
            junk[pl.ds(8 * ((b * NCH + c) % 8), 8), :] = tg

    def ggen():
        sel = selb[...]

        def onehot(k, r0, n):
            ri = lax.broadcasted_iota(I32, (n, 256), 0) + r0
            return jnp.where(ri == sel[k:k + 1, :], 1.0, 0.0)
        e = jnp.concatenate([onehot(0, 0, 128), onehot(1, 0, 64), onehot(2, 0, 32),
                             onehot(1, 112, 16), onehot(2, 112, 16), onehot(3, 112, 16)], axis=0).astype(BF16)
        g = _dot(e, _bf(g0b[pl.ds(0, 128), :]))

        def put(r, v):
            gm[pl.ds((r - 256) // 2, v.shape[0] // 2), :] = _u32(v)

        def zero(r, n):
            gm[pl.ds((r - 256) // 2, n // 2), :] = jnp.zeros((n // 2, 512), U32)
        zero(256, 112)
        put(368, g[256:272])
        put(384, g[0:128])
        put(512, g[128:192])
        zero(576, 48)
        put(624, g[224:240])
        put(640, g[128:192])
        put(704, g[192:224])
        zero(736, 80)
        put(816, g[240:256])
        put(832, g[192:224])
        zero(864, 64)

    def extract(st, o4):
        g = [[jnp.take_along_axis(_pk(o4[0][grp][8 * v:8 * v + 8], o4[1][grp][8 * v:8 * v + 8]), M.gidx, axis=1,
                                  mode="promise_in_bounds") for v in range(10)] for grp in range(2)]

        def mix(a, b):
            return jnp.where(M.lo4, a, b), pltpu.roll(jnp.where(M.lo4, b, a), 4, 0)

        def two(va, vb, m1, m2):
            p, q = mix(jnp.where(m1, g[0][va], g[0][vb]), jnp.where(m1, g[1][va], g[1][vb]))
            return jnp.where(m2, p, q)

        def four(gg):
            return jnp.where(M.lo64, jnp.where(M.beven, gg[2], gg[3]), jnp.where(M.beven, gg[4], gg[5]))
        t_odd = two(0, 1, M.lo64, M.beven)
        t_even, t_2 = mix(four(g[0]), four(g[1]))
        t_3 = two(6, 7, M.beven, M.lo64)
        t_4 = two(8, 9, M.lo64, M.beven)
        tl = [t_odd, t_even, t_2, jnp.where(M.last, t_2, t_3), t_3, jnp.where(M.last, t_3, t_4), t_4]
        for t in range(7):
            kd[pl.ds(st * 8, 8), pl.ds(128 * t, 128)] = tl[t]

    tk = {}

    def ln_chunk(j):
        cj = slice(256 * j, 256 * j + 256)
        s1 = s2 = None
        for i in range(NS):
            v16 = xb[pl.ds(i * 16, 16), cj].astype(F32)
            for v in (v16[:8], v16[8:]):
                s1, s2 = (v, v * v) if s1 is None else (s1 + v, s2 + v * v)
        mean = jnp.sum(s1, axis=0, keepdims=True) * (1.0 / D)
        var = jnp.sum(s2, axis=0, keepdims=True) * (1.0 / D) - mean * mean
        var = jnp.maximum(var, 0.0)
        sd = _rb(jnp.sqrt(_rb(_rb(var) + 1e-5)))
        mb = jnp.broadcast_to(_rb(mean), (16, 256))
        hi = jnp.broadcast_to(0.5 / sd, (16, 256))
        if j == 0:
            wrow = wr[...].astype(F32).reshape(1, D)
            tk["w"] = [(jnp.broadcast_to(wrow[:, k0:min(k0 + 128, D)], (16, min(128, D - k0)))
                        + jnp.zeros((16, min(128, D - k0)), F32)).astype(BF16) for k0 in range(0, D, 128)]
        r = None
        for i in range(NS):
            rw = pl.ds(dyn(i * 8), 8) if CFG['xdyn'] else pl.ds(i * 8, 8)
            hv = _rb(xb[pl.ds(i * 16, 16), cj].astype(F32) - mb) * hi
            h0, h1 = hv[:, :128], hv[:, 128:]
            xh[rw, pl.ds(256 * j, 128)] = _u32(h0)
            xh[rw, pl.ds(256 * j + 128, 128)] = _u32(h1)
            rv = rw if CFG["merge"] else pl.ds(i * 8, 8)
            vv[rv, pl.ds(256 * j, 128)] = _u32(h0 + h1)
            vv[rv, pl.ds(256 * j + 128, 128)] = _u32(h0 - h1)
            if i % 8 == 7 or i == NS - 1:
                k0, k1 = (i // 8) * 128, (i + 1) * 16
                yield
                p = _dot(tk["w"][i // 8], _bf(xh[pl.ds(k0 // 2, (k1 - k0) // 2), cj]))
                r = p if r is None else r + p
        for t in range(2):
            r_t = r[:, 128 * t:128 * t + 128]
            tk["rc"] = r_t if (j == 0 and t == 0) else jnp.where(M.row16 == 2 * j + t, r_t, tk["rc"])

    def topk():
        bits = pltpu.bitcast(_rb(tk["rc"] * 2.0), I32)
        mono = (jnp.where(bits < 0, bits ^ 0x7FFF0000, bits) >> 16) + 32768
        key = pltpu.bitcast(0x30000000 + (mono << 11) + (2047 - (M.row16 * 128 + M.lane16)), F32)
        kcol = jnp.zeros((16, 128), I32)
        for j in range(NSEL):
            mx = jnp.max(jnp.max(key, axis=0, keepdims=True), axis=1, keepdims=True)
            mxb = jnp.broadcast_to(mx, (16, 128))
            key = jnp.where(key == mxb, 0.0, key)
            kcol = jnp.where(M.row16 == j, pltpu.bitcast(mxb, I32), kcol)
        kcol = kcol - 0x30000000
        idxcol = jnp.where(M.row16 < NSEL, 2047 - (kcol & 2047), -1)
        hb = ((kcol >> 11) - 32768) << 16
        rsel = pltpu.bitcast(jnp.where(hb < 0, hb ^ 0x7FFF0000, hb), F32)
        rsel = jnp.where(M.row16 < NSEL, rsel, 0.0)
        rs_s[...] = _rb(jax.nn.sigmoid(rsel))
        tk["oh"] = jnp.concatenate(
            [jnp.where(idxcol == M.lane16 + 128 * t, 1.0, 0.0) for t in range(16)], axis=1).astype(BF16)
        oh_s[...] = pltpu.bitcast(tk["oh"], U32)
        hb_ = jnp.where(M.row16[:8] < NSEL, jnp.left_shift(1, jnp.maximum(idxcol[:8], 0) >> 7), 0)
        for sh in (4, 2, 1):
            hb_ = hb_ | pltpu.roll(hb_, sh, 0)
        hit_s[0] = hb_[0, 0]
        tcol = jnp.maximum(idxcol, 0) >> 7
        tk["tj"] = [tcol[j, 0] for j in range(NSEL)]
        tk["ol"] = jnp.where((idxcol & 127) == M.lane16, 1.0, 0.0)

    def xsel(j):
        off = pl.multiple_of(tk["tj"][j] * 128, 128)
        lhs = jnp.where(M.row16 == j, tk["ol"], 0.0).astype(BF16)
        v = _dot_nt(lhs, _bf(xh[:, pl.ds(off, 128)]))
        tk["xa"] = v if j == 0 else tk["xa"] + v
        if j == NSEL - 1:
            xs_s[...] = _u32(tk["xa"] * 2.0)

    def link(v):
        if not CFG["link"]:
            return v
        w = pltpu.bitcast(v, U32)
        dep = ob[pl.ds(0, 8), pl.ds(0, 128)] & tk["zm"]
        return pltpu.bitcast(jnp.concatenate([w[:, :128] | dep, w[:, 128:]], axis=1), BF16)

    def wpiece(i, p):
        c = 0
        while 2 * p >= sum(FCH[:c + 1]):
            c += 1
        v = wbuf[c][i][:, pl.ds(256 * p - 128 * sum(FCH[:c]), 256)]
        return _bf(v) if CFG["wcast"] else v

    def ffn_gu(p, lk):
        xs = link(tk["xs"]) if lk else tk["xs"]
        gu = _dot(xs, jnp.concatenate([wpiece(0, p), wpiece(1, p)], axis=1))
        g = _rb(gu[:, :256])
        u = _rb(gu[:, 256:])
        sg = _rb(0.5 * jnp.tanh(0.5 * g) + 0.5)
        tk["h", p] = (_rb(g * sg) * u).astype(BF16)

    def ffn_dn(p, lk):
        h = tk.pop(("h", p))
        y = _dot_nt(link(h) if lk else h, wpiece(2, p))
        tk["y"] = y if p == 0 else tk["y"] + y

    def fin16(i, c0, c1, du, dynst):
        r16 = pl.ds(16 * i, 16)
        cs = pl.ds(128 * c0, 128 * (c1 - c0))
        h = _bf(xh[pl.ds(8 * i, 8), cs]).astype(F32)
        y = jnp.concatenate([_upk(yb[r16, pl.ds(256 * (c // 4) + 128 * (c % 2), 128)], (c // 2) % 2)
                             for c in range(c0, c1)], axis=1)
        dv = deff[r16, :]
        s_ = y + h * jnp.concatenate([dv] * (c1 - c0), axis=1)
        zh = h if du is None else h + du
        g = zh * jnp.tanh(zh) + zh
        res = xb[r16, cs].astype(F32) + s_ * g
        if CFG["ocast"]:
            ob[pl.ds(8 * i, 8), cs] = _u32(res)
        else:
            ob[r16, cs] = res.astype(BF16)

    utj = CFG["utj"]
    RU = CFG["RU"]

    def ut_piece(b, k, j0):
        rw = pl.ds(b * (RU // 2), RU // 2)
        rows = pl.ds(dyn(0), RU) if CFG['udyn'] else pl.ds(0, RU)
        ur = urs[b % 3]
        js = range(j0, j0 + utj)

        def lhs(ref, o):
            return _bf(jnp.concatenate([ref[rw, pl.ds(256 * j + o, 128)] for j in js], axis=0))

        def put(val, col):
            for i, j in enumerate(js):
                ur[rows, pl.ds(640 * j + col, 128)] = val[i * RU:(i + 1) * RU]
        if k == 0:
            v = _dot(lhs(vv, 0), _bf(um[:, 0:256]))
            b2 = _dot(lhs(vv, 128), _bf(um[:, 256:384]))
            a0 = v[:, :128]

            def sel(p, q):
                return jnp.concatenate([jnp.where(M.lo64, p[8 * i:8 * i + 8], q[8 * i:8 * i + 8])
                                        for i in range(a0.shape[0] // 8)], axis=0)
            put(sel(a0, b2), 0)
            put(v[:, 128:], 128)
            put(pltpu.roll(sel(b2, a0), 64, 1), 256)
        else:
            put(_dot(lhs(xh, 128), _bf(um[:, 384:512])), 384)
            put(_dot(lhs(xh, 0), _bf(um[:, 512:640])), 512)

    def mac(g, cls):
        ur = urs[(8 * g // RU) % 3]

        @functools.lru_cache(None)
        def us(j):
            def ld(c):
                return ur[pl.ds((8 * g) % RU, 8), pl.ds(640 * j + c, 128)]
            if cls == 0:
                a, b = ld(0), ld(256)
                return (a, b, a + b)
            t1, t2, t3 = ld(128), ld(384), ld(512)
            return (t1 + t2, t3 - t1, t2 + t3)

        @functools.lru_cache(None)
        def kraw(j):
            o = 512 * j + 256 * (1 - cls)
            ksp, kr = ksps[8 * g // RB], pl.ds((8 * g) % RB, 8)
            return ksp[kr, pl.ds(o, 128)], ksp[kr, pl.ds(o + 128, 128)]

        @functools.lru_cache(None)
        def ks(j):
            sr, si = kraw(j)
            if j > 0:
                pr, pi_ = kraw(j - 1)
                sr, si = (sr + pr, si + pi_) if cls == 0 else (sr - pr, si - pi_)
            return (sr * M.mz if cls == 0 else sr, si - sr, sr + si)
        outs = []
        prev = None
        for m in (range(NCH) if CFG["mord"] == 0 else range(NCH - 1, -1, -1)):
            acc = None
            for j in range(m + 1):
                a, b, s = us(j)
                c_, e_, g_ = ks(m - j)
                t = (c_ * s, a * e_, b * g_)
                acc = t if acc is None else tuple(x + y for x, y in zip(acc, t))
            z = (acc[0] - acc[2], acc[0] + acc[1])
            if (m % 2 == 1) == (CFG["mord"] == 0):
                za, zb = (prev, z) if CFG["mord"] == 0 else (z, prev)
                if cls == 0:
                    zr = _pk(za[0], zb[0])
                    zis = _pk(za[1], zb[1]) if CFG.get('nrz') else pltpu.roll(_pk(za[1], zb[1]), 64, 1)
                    outs.append((jnp.where(M.lo64, zr, zis), jnp.where(M.lo64, zis, zr)))
                else:
                    outs.append((_pk(za[0] + za[1], zb[0] + zb[1]), _pk(za[1], zb[1]), _pk(za[0], zb[0])))
            prev = z
        return outs if CFG['mord'] == 0 else outs[::-1]

    zq, wq = {}, {}

    def inv(g, cls):
        zo_ = zq.pop((g, cls))

        def st(t):
            return _bf(jnp.concatenate([zo_[p][t] for p in range(4)], axis=0))
        if cls == 0:
            wq[g] = [_dot(st(t), _bf(umt[:, c:c + 128])) for t, c in ((0, 0), (1, 256))]
        else:
            q1, q2, q3 = [_dot(st(t), _bf(umt[:, c:c + 128])) for t, c in ((0, 128), (1, 384), (2, 512))]
            w0, w2 = wq.pop(g)
            p_ = q1 + w2
            y0 = p_ + (q2 + w0)
            y1 = (q3 + w0) - p_
            yr = pl.ds(dyn(8 * g), 8) if CFG["ydyn"] else pl.ds(8 * g, 8)
            for p in range(4):
                yb[yr, pl.ds(256 * p, 128)] = _u32(y0[16 * p:16 * p + 16])
                yb[yr, pl.ds(256 * p + 128, 128)] = _u32(y1[16 * p:16 * p + 16])

    ktq = []
    slotno = [0]
    pat = CFG.get("kt_pat", [1, 0, 1, 1, 0, 1, 0, 1, 1, 0, 1, 1, 0, 1, 0, 1])
    xw = CFG["xw"]

    def kt_drain(n):
        for _ in range(n):
            if ktq and ktq[0][0] <= slotno[0]:
                kt_unit(*ktq.pop(0)[1:])

    utq = [(b, k, j) for b in range(D // RU) for j in range(0, NCH, utj) for k in range(2)]
    pend = [None]

    pre_xy = {}

    def kxy(st, half):
        r0 = st * 16
        pk = [pltpu.bitcast(prm[k, pl.ds(r0, 16), :], U32) for k in range(6)]
        rows = pl.ds(r0 + half, 8, stride=2)
        bs, k0 = _base8([_upk(w, half) for w in pk], dtc[rows, :])
        k0c[rows, :] = jnp.broadcast_to(k0, (8, 128))
        return [_grp_xy(bs, grp, M.lo4) for grp in range(2)]

    def kgen(s0, s1):
        for st in range(s0, s1):
            o4 = []
            for half in range(2):
                xy = pre_xy.pop((st, half)) if (st, half) in pre_xy else kxy(st, half)
                if half == 0 and pend[0] is not None:
                    flush()
                oo = []
                for grp in range(2):
                    yield
                    slotno[0] += 1
                    oo.append(_dot_nt(*xy[grp]))
                o4.append(oo)
            pend[0] = (st, o4)
        if s1 == NS or not CFG["carry"]:
            flush()
        else:
            for h in range(CFG["npre"]):
                pre_xy[(s1 + h // 2, h % 2)] = kxy(s1 + h // 2, h % 2)

    def flush():
        extract(*pend[0])
        if (pend[0][0] + 1) % SPB == 0:
            ktq.extend([(slotno[0] + 4 * CFG["kt_lag"], pend[0][0] // SPB, c) for c in range(NCH)])
        pend[0] = None

    def region(name, fn):
        def body():
            masks()
            mark(name)
            fn()
            mark(None)
        if CFG["split"]:
            pl.when(zs[0] == 0)(body)
        else:
            body()

    def consts():
        dkb = _col_bcast(dsk)
        for t in range(5):
            n = 128 if t < 4 else 64
            dkc[pl.ds(t * 128, n), :] = dkb[t][:n]

    def rate(num, den):
        acc = [0]

        def step():
            acc[0] += num
            n = acc[0] // den
            acc[0] -= n * den
            return n
        return step

    only = CFG.get("only")
    doA = only in (None, "A")
    s1 = R1 // 16 - (CFG['npre'] + 1) // 2
    if doA:
        ktr = rate(*CFG["ktr0"])
        for i, _ in enumerate(kgen(0, s1)):
            if i == CFG["gg_at"]:
                ggen()
            if i > CFG["gg_at"]:
                kt_drain(ktr())
    mark('s3_w2')
    for cp in in_cp[2]:
        cp.wait()
    mark('s3_A1b')
    if doA:
        slotno[0] += 100
        ktr = rate(*CFG["ktr1"])
        for i, _ in enumerate(kgen(s1, xw)):
            kt_drain(ktr())
        consts()
    mark('s4_waitx')
    in_cp[3][0].wait()
    mark(None)

    def phase_a2():
        slotno[0] += 100
        kg = kgen(xw, NS)
        kgr = rate(*CFG["kgr"])
        for _ in range(CFG["pre"]):
            next(kg)
        for j in range(NCH):
            for k, _ in enumerate(ln_chunk(j)):
                kt_drain(CFG["n5"][k])
                for _ in range(kgr()):
                    next(kg)
        topk()
        ktr = rate(*CFG["ktr2"])
        xq = list(range(NSEL))
        for i, _ in enumerate(kg):
            kt_drain(ktr())
            if i >= CFG["xs_lag"] and xq and (i - CFG["xs_lag"]) % CFG["xs_per"] == 0:
                xsel(xq.pop(0))
        while xq:
            xsel(xq.pop(0))
        slotno[0] += 1000
        kt_drain(len(ktq) - NCH)

    ffp = [0, 0]

    def ffn_next():
        if ffp[1] < ffp[0] - 1 or (ffp[1] < ffp[0] and ffp[0] >= ffp_max[0]):
            ffn_dn(ffp[1], False)
            ffp[1] += 1
        elif ffp[0] < ffp_max[0]:
            ffn_gu(ffp[0], False)
            ffp[0] += 1
    ffp_max = [0]
    utdue = [0]
    GEND_ = D // 8 + CFG['lag'] + CFG['flag'] + 2

    def phase_b(g0, g1):
        inB[0] = True
        lag = CFG["lag"]
        NG = D // 8
        if g0 == 0:
            npre = 16 // utj + (2 * CFG["lead"] * 64 // RU) // utj
            for i in range(0 if CFG["utpre"] else npre):
                ut_piece(*utq.pop(0))
            if CFG["fuse"]:
                for t in range(5):
                    n = 128 if t < 4 else 64
                    deff[pl.ds(128 * t, n), :] = (dkc[pl.ds(128 * t, n), :] + k0c[pl.ds(128 * t, n), :]) * 2.0
        fl = CFG["flag"]
        for s in range(g0, g1):
            for cls in range(2):
                if s < NG:
                    zq[(s, cls)] = mac(s, cls)
                if CFG["order"] == 1 and lag <= s < NG + lag:
                    inv(s - lag, cls)
                if ((2 * s + cls) * 64 // RU) % utj == 0:
                    utdue[0] += max(1, 64 // RU // utj)
                if not (g1 < GEND_ and 2 * (g1 - s) - cls <= CFG["hold"]):
                    while utdue[0] and utq:
                        utdue[0] -= 1
                        ut_piece(*utq.pop(0))
                if cls == 1 and s % 4 == CFG["ktb"] % 4 and s >= CFG["ktb"]:
                    kt_drain(1)
                if CFG["order"] == 0 and lag <= s < NG + lag:
                    inv(s - lag, cls)
                if CFG["fuse"]:
                    q = 2 * (s - lag - fl) + cls - 2
                    if 0 <= q < 4 * NS:
                        fin16(q // 4, 4 * (q % 4), 4 * (q % 4) + 4, None, False)
                if CFG["ffb"] and cls == CFG["ffc"] and (s - g0) % CFG["ffb"] == CFG["ffo"] % CFG["ffb"]:
                    ffn_next()

    merge = CFG["merge"] and only is None
    if merge:
        inB[0] = True
    elif only in (None, "A"):
        region('s5_A2', phase_a2)
    elif only == "B":
        ktq.extend([(0, NB - 1, c) for c in range(NCH)])
    HR = CFG["hrows"]
    obb = ob.bitcast(BF16) if CFG['ocast'] else ob
    o_cp = [[pltpu.make_async_copy(obb.at[pl.ds(r0, n), pl.ds(128 * t, 128)],
                                   out_hbm.at[pl.ds(r0, n), pl.ds(128 * t, 128)], sem_o.at[hf, t])
             for t in range(16)] for hf, (r0, n) in enumerate([(0, HR), (HR, D - HR)] if HR else [(0, D)])]

    def start_free(hf):
        hit = hit_s[0]
        for t in range(16):
            @pl.when(((hit >> t) & 1) == 0)
            def _():
                o_cp[hf][t].start(priority=1)

    GEND = D // 8 + CFG["lag"] + CFG["flag"] + 2
    if only in (None, "B"):
        def pb():
            if merge:
                phase_a2()
            g = 0
            for gs, cc in CFG["bw"]:
                if gs > g:
                    phase_b(g, gs)
                    g = gs
                if cc == len(CFG["bw"]) - 1 and only is None and HR:
                    assert (2 * (gs - 1 - CFG["lag"] - CFG["flag"]) + 1 - 2 + 1) // 4 * 16 >= HR
                    start_free(0)
                mark(f's7_w{cc}')
                if not (merge and cc == 0):
                    for cp in w_cp[cc]:
                        cp.wait()
                mark(f's7_B{cc}')
                ffp_max[0] = sum(FCH[:cc + 1]) // 2
                tk["xs"] = _bf(xs_s[...])
            phase_b(g, GEND)
            while CFG["ffb"] and ffp[1] < ffp_max[0]:
                ffn_next()
            if CFG["ffb"]:
                ya_s[...] = tk["y"]
        region('s7_B', pb)
    if only in ("A", "B"):
        for cc in range(len(CFG["bw"]), len(FCH)):
            for cp in w_cp[cc]:
                cp.wait()
        cp = pltpu.make_async_copy(obb, out_hbm, sem_o.at[0, 0])
        cp.start()
        cp.wait()
        cp = pltpu.make_async_copy(yb.bitcast(BF16).at[pl.ds(0, D), :], out_hbm.at[:, pl.ds(0, 1024)], sem_o.at[0, 0])
        cp.start()
        cp.wait()
        for kk in ksps:
            cp = pltpu.make_async_copy(kk.at[:, pl.ds(0, 512)], junk.at[:, pl.ds(0, 512)], sem_o.at[0, 0])
            cp.start()
            cp.wait()
        for kk in (vv, xs_s, kd, umt):
            cp = pltpu.make_async_copy(kk.at[pl.ds(0, 8), pl.ds(0, 512)], oh_s.at[:, pl.ds(0, 512)], sem_o.at[0, 0])
            cp.start()
            cp.wait()
        cp = pltpu.make_async_copy(ya_s, junk.at[pl.ds(0,16), :], sem_o.at[0, 0])
        cp.start()
        cp.wait()
        return
    masks()
    tk["xs"] = _bf(xs_s[...])
    tk["rs"] = rs_s[...]
    tk["oh"] = _bf(oh_s[...])

    mark('s8_ffn')
    if not CFG['sf_late']:
        start_free(len(o_cp) - 1)
    tk["y"] = ya_s[...]
    mark('s8_w')
    for cc in range(len(CFG["bw"]), len(FCH)):
        for cp in w_cp[cc]:
            cp.wait()
    mark('s8_f')
    if CFG["sf_late"]:
        start_free(len(o_cp) - 1)
    npc = sum(FCH) // 2
    if CFG["tailp"] == 0:
        while ffp[0] < npc:
            ffn_gu(ffp[0], False)
            ffp[0] += 1
            if ffp[1] < ffp[0] - 1:
                ffn_dn(ffp[1], False)
                ffp[1] += 1
    else:
        while ffp[0] < npc:
            ffn_gu(ffp[0], False)
            ffp[0] += 1
    while ffp[1] < ffp[0]:
        ffn_dn(ffp[1], False)
        ffp[1] += 1
    rs = jnp.concatenate([tk["rs"]] * 5, axis=1)[:, :D]
    upd = (_rb(_rb(tk["y"]) * rs) * 0.5).astype(BF16)
    if CFG["tmode"] == 0:
        updt_s[:, pl.ds(0, 128)] = _u32(lax.dot_general(upd, jnp.eye(16, 128, dtype=BF16), (((0,), (0,)), ((), ())),
                                                        preferred_element_type=F32))
    else:
        upt_s[...] = jnp.concatenate([upd, jnp.zeros((16, 64), BF16)], axis=1).T
    mark('s9_final')
    hit = hit_s[0]
    for t in range(16):
        @pl.when(((hit >> t) & 1) == 1)
        def _():
            if CFG["tmode"] == 0:
                ohp = jnp.concatenate([_bf(oh_s[:, pl.ds(128 * t, 128)]), jnp.zeros((112, 128), BF16)], axis=0)
                du = _dot(_bf(updt_s[:, pl.ds(0, 128)]), ohp)
            else:
                du = _dot(upt_s[pl.ds(0, D), :], _bf(oh_s[:, pl.ds(128 * t, 128)]))
            for i in range(NS):
                fin16(i, t, t + 1, du[16 * i:16 * i + 16], False)
            for hf in range(len(o_cp)):
                o_cp[hf][t].start(priority=1)
    mark('sa_waito')
    for cps in o_cp:
        for cp in cps:
            cp.wait()
    mark(None)


@jax.jit
def pallas_recurrent_scan__ssm_conv_s4__moe_arch_mod__prompt_kernel(A_u, A_A_re, A_A_im, A_B_re, A_B_im, A_C_re, A_C_im, A_log_dt, A_Dskip,
              B_x, B_w_r, B_w_gate, B_w_up, B_w_down):
    xt = jnp.transpose(A_u[0])
    wdt = jnp.transpose(B_w_down)
    scratch = [
        pltpu.SMEM((1,), I32),
        pltpu.VMEM((D, L), BF16),
        pltpu.VMEM((6, D, N), BF16),
        pltpu.VMEM((D,), BF16),
        pltpu.VMEM((D,), BF16),
        pltpu.VMEM((D,), BF16),
        pltpu.VMEM((64, 640), U32),
        pltpu.VMEM((128, 512), U32),
        pltpu.VMEM((336, 512), U32),
        pltpu.VMEM((8, 256), I32),
        pltpu.VMEM((64, 640), U32),
        pltpu.VMEM((D, 128), F32),
        pltpu.VMEM((D, 128), F32),
        pltpu.VMEM((D, 128), F32),
        pltpu.VMEM((D // 2, 896), U32),
        pltpu.VMEM((D // 2, L), U32),
        pltpu.VMEM((D // 2, L), U32),
        pltpu.VMEM((CFG['RU'], 5120), F32),
        pltpu.VMEM((CFG['RU'], 5120), F32),
        pltpu.VMEM((CFG['RU'], 5120), F32),
        pltpu.VMEM((D, L // 2), U32),
        pltpu.VMEM((D // 2, L), U32) if CFG['ocast'] else pltpu.VMEM((D, L), BF16),
        pltpu.VMEM((64, D), F32),
        pltpu.VMEM((16, 128), F32),
        pltpu.VMEM((8, L), U32),
        pltpu.VMEM((8, D), U32),
        pltpu.SMEM((1,), I32),
        pltpu.VMEM((8, 128), U32),
        pltpu.VMEM((D, 128), F32),
        pltpu.VMEM((D // 2, 256), U32),
        pltpu.VMEM((16, D), F32),
        pltpu.VMEM((640, 16), BF16),
        pltpu.SemaphoreType.DMA((17,)),
        pltpu.SemaphoreType.DMA((3, len(FCH))),
        pltpu.SemaphoreType.DMA((2, 16)),
    ] + [pltpu.VMEM((RB, 4096), F32)] * NB + [
        (pltpu.VMEM((D // 2, 128 * n), U32) if CFG['wcast'] else pltpu.VMEM((D, 128 * n), BF16)) for n in FCH for _ in range(3)]
    out = pl.pallas_call(
        _kernel,
        out_shape=jax.ShapeDtypeStruct((D, L), BF16),
        in_specs=[pl.BlockSpec(memory_space=pl.ANY)] * 14,
        out_specs=pl.BlockSpec(memory_space=pl.ANY),
        scratch_shapes=scratch,
        grid=(1,) if CFG['zsrc'] == 1 else (),
        compiler_params=pltpu.CompilerParams(vmem_limit_bytes=100 * 2**20, disable_semaphore_checks=True,
                                             disable_bounds_checks=True),
        name="s4_mod",
    )(xt, A_A_re, A_A_im, A_B_re, A_B_im, A_C_re, A_C_im, A_log_dt, A_Dskip,
      B_w_r, B_w_gate, B_w_up, wdt, jnp.asarray(_SEL))
    return jnp.transpose(out)[None]
```

```python
import functools
import math

import numpy as np
import jax
import jax.numpy as jnp
from jax import lax
import jax.experimental.pallas as pl
import jax.experimental.pallas.tpu as pltpu

F32 = jnp.float32
BF16 = jnp.bfloat16
U32 = jnp.uint32
I32 = jnp.int32

D = 576
L = 2048
N = 128
NSEL = 8
NCH = 8
NS = D // 16
NG = D // 8
RB = 64
NB = D // RB
SPB = RB // 16
RU = 16
UTJ = 4
R1 = 128
XW = 22
FCH = (10, 10, 8, 8)
FWAIT = ((0, 0), (24, 1), (49, 2))

_TILES = {
    "odd": (1, 3, 5, 7),
    "even": (2, 4, 6, 8),
    "t2": (258, 260, 262, 264),
    "t3": (516, 520, 772, 776),
    "t4": (1032, 1288, 1544, 1800),
}
_KT = [(0, 256, 0), (128, 256, 256), (384, 128, 512), (512, 128, 576),
       (640, 128, 704), (768, 128, 800), (768, 128, 768), (768, 128, 736)]


def _rlag(l):
    u = int(np.float32(l).view(np.uint32))
    u = (u + 0x7FFF + ((u >> 16) & 1)) & 0xFFFF0000
    return int(np.uint32(u).view(np.float32))


def _tile_pts(name):
    base = name.rstrip("v")
    p = np.array([_TILES[base][l // 32] + 8 * (l % 32) for l in range(128)])
    if name == "t3v":
        p[127] = 512
    if name == "t4v":
        p[127] = 1024
    return p


def _sel_table():
    lags = np.concatenate([_tile_pts("odd"), _tile_pts("even")])
    sel = np.full((8, 256), -1, np.int32)
    for k, (c, tile) in enumerate([(1, "t2"), (2, "t3v"), (4, "t4v"), (1, "even")]):
        pts = _tile_pts(tile)
        for rho, r in enumerate(lags):
            idx = np.nonzero(pts == _rlag(256 * c + int(r)))[0]
            if len(idx):
                sel[k, rho] = idx[0]
    return sel


_SEL = _sel_table()


def _bf(x):
    return pltpu.bitcast(x, BF16)


def _u32(x):
    return pltpu.bitcast(x.astype(BF16), U32)


def _rb(x):
    return x.astype(BF16).astype(F32)


def _pk(a, b):
    return pltpu.pack_elementwise([a, b], packed_dtype=BF16)


def _upk(w, h):
    return pltpu.unpack_elementwise(w, index=h, packed_dtype=BF16, unpacked_dtype=F32)


def _cmul(a, b):
    return (a[0] * b[0] - a[1] * b[1], a[0] * b[1] + a[1] * b[0])


def _csq(a):
    t = a[0] * a[1]
    return (a[0] * a[0] - a[1] * a[1], t + t)


def _sincos(th):
    magic = 12582912.0
    kf = th * (2.0 / math.pi) + magic
    ki = pltpu.bitcast(kf, I32)
    k = kf - magic
    r = th - k * 1.5703125
    r = r - k * 4.837512969970703125e-4
    r = r - k * 7.54978995489188216e-8
    r2 = r * r
    s = r + r * r2 * (-1.6666654611e-1 + r2 * (8.3321608736e-3 + r2 * -1.9515295891e-4))
    c = 1.0 + r2 * (-0.5 + r2 * (4.166664568298827e-2 + r2 * (-1.388731625493765e-3 + r2 * 2.443315711809948e-5)))
    swap = (ki & 1) == 1
    sn = jnp.where(swap, c, s)
    cs = jnp.where(swap, s, c)
    sbit = (ki & 2) << 30
    cbit = ((ki + 1) & 2) << 30
    sn = pltpu.bitcast(pltpu.bitcast(sn, I32) ^ sbit, F32)
    cs = pltpu.bitcast(pltpu.bitcast(cs, I32) ^ cbit, F32)
    return cs, sn


def _dot(a, b):
    return jnp.dot(a, b, preferred_element_type=F32)


def _dot_nt(a, b):
    return lax.dot_general(a, b, (((1,), (1,)), ((), ())), preferred_element_type=F32)


def _col_bcast(vec_ref):
    v = vec_ref[...].astype(F32).reshape(1, D)
    vp = jnp.concatenate([v, jnp.zeros((1, 64), F32)], axis=1)
    return [jnp.broadcast_to(vp[:, t * 128:(t + 1) * 128], (128, 128)).T for t in range(5)]


def _base8(p, dt):
    are, aim, bre, bim, cre, cim = p
    y1 = (dt * are) * math.log2(math.e)
    ph = {1: _sincos(dt * aim)}
    e = 1
    while e < 512:
        ph[2 * e] = _csq(ph[e])
        e *= 2
    pw = {}
    for e in (1, 2, 4, 8, 16, 256, 512):
        mg = jnp.exp2(y1 * float(e)) if e > 1 else jnp.exp2(y1)
        pw[e] = (mg * ph[e][0], mg * ph[e][1])
    w = _cmul((cre, cim), (dt * bre, dt * bim))
    k0 = jnp.sum(w[0], axis=1, keepdims=True)
    w1 = _cmul(w, pw[1])
    w2 = _cmul(w1, pw[1])
    w3 = _cmul(w2, pw[1])
    w258 = _cmul(w2, pw[256])

    def rot(z):
        return (pltpu.roll(z[0], 4, 0), pltpu.roll(z[1], 4, 0))
    rots = {e: rot(pw[e]) for e in (2, 4, 8, 16, 512)}
    return (pw, rots, w1, w2, rot(w3), rot(w258)), k0


def _grp_xy(bs, grp, lo4):
    pw, rots, w1, w2, w3r, w258r = bs

    def sel(lo, hi):
        return (jnp.where(lo4, lo[0], hi[0]), jnp.where(lo4, lo[1], hi[1]))
    if grp == 0:
        dup = {e: sel(pw[e], rots[e]) for e in (2, 4, 16, 512)}
        x0, x2, a8 = sel(w1, w3r), sel(w2, w258r), rots[8]
    else:
        dup = {e: sel(rots[e], pw[e]) for e in (2, 4, 16, 512)}
        x0, x2, a8 = sel(w3r, w1), sel(w258r, w2), pw[8]
    xv = [None] * 10
    xv[0] = x0
    xv[1] = _cmul(x0, dup[4])
    xv[2] = x2
    xv[3] = _cmul(xv[2], dup[2])
    xv[4] = _cmul(xv[3], dup[2])
    xv[5] = _cmul(xv[4], dup[2])
    xv[6] = _cmul(xv[3], dup[512])
    xv[7] = _cmul(xv[5], dup[512])
    xv[8] = _cmul(xv[7], dup[512])
    xv[9] = _cmul(xv[8], dup[512])
    y = (jnp.where(lo4, 1.0, a8[0]), jnp.where(lo4, 0.0, -a8[1]))
    m = dup[16]
    ys = [y]
    for _ in range(15):
        y = (y[0] * m[0] + y[1] * m[1], y[1] * m[0] - y[0] * m[1])
        ys.append(y)

    def mat(vs):
        return jnp.concatenate([jnp.concatenate([v[0] for v in vs], 0),
                                jnp.concatenate([v[1] for v in vs], 0)], 1).astype(BF16)
    return mat(xv), mat(ys)


def _dft_tables(um, umt, g0b):
    sub = lax.broadcasted_iota(I32, (8, 128), 0)
    lane = lax.broadcasted_iota(I32, (8, 128), 1)
    lo = lane < 64

    def e512(m):
        return _sincos((m & 511).astype(F32) * (-2.0 * math.pi / 512.0))

    def chain(base, step, n):
        out = [base]
        for _ in range(n - 1):
            out.append(_cmul(out[-1], step))
        return out

    def row(z, r):
        return tuple(jnp.broadcast_to(c[r:r + 1], (8, 128)) for c in z)

    def put(ref, r0, c0, vs):
        for i in range(0, len(vs), 2):
            ref[pl.ds(r0 + 4 * i, 8), pl.ds(c0, 128)] = _u32(jnp.concatenate([vs[i], vs[i + 1]], axis=0))
    f1 = 4 * lane + 1
    k4 = 4 * (lane & 63)
    alt_r = jnp.where((sub & 1) == 1, 1.0, -1.0)
    alt_l = jnp.where((lane & 1) == 1, 1.0, -1.0)
    b1 = e512(f1 * (sub + 1))
    c1 = chain(b1, row(b1, 7), 16)
    put(um, 0, 128, [z[0] for z in c1])
    put(um, 0, 384, [z[1] - z[0] for z in c1])
    put(um, 0, 512, [z[0] + z[1] for z in c1])
    for col, off, q in ((0, 0, jnp.where(lo, 0, 128)), (256, 2, jnp.where(lo, 128, 0))):
        b = e512((k4 + off) * (sub + 1))
        c = chain(e512((k4 + off) * (sub + 1) + q), row(b, 7), 16)
        vs = [z[0] for z in c]
        if off == 0:
            vs = [jnp.where(lane == 64, alt_r, v) for v in vs]
        put(um, 0, col, vs)
    st = e512(32 * (lane + 1))
    c = chain(e512((4 * sub + 1) * (lane + 1)), st, 16)
    put(umt, 0, 128, [z[0] for z in c])
    put(umt, 0, 384, [z[1] - z[0] for z in c])
    put(umt, 0, 512, [z[0] + z[1] for z in c])
    c = chain(e512(4 * sub * (lane + 1)), st, 8)
    re = [z[0] for z in c]
    im = [z[1] for z in c]
    re[0] = jnp.where(sub == 0, alt_l, re[0])
    im[0] = jnp.where(sub == 0, 1.0, im[0])
    put(umt, 0, 0, re + im)
    c = chain(e512((4 * sub + 2) * (lane + 1)), st, 8)
    put(umt, 0, 256, [z[1] for z in c] + [z[0] for z in c])
    for cls, f in ((0, f1), (1, k4 + jnp.where(lo, 0, 2))):
        b = e512(f * (1 + 8 * sub))
        s1 = row(b, 0)
        s64 = e512(f * 64)
        cur = chain((b[0] * (1.0 / 128), b[1] * (1.0 / 128)), s64, 4)
        for lag in range(1, 9):
            re = [z[0] for z in cur]
            im = [z[1] for z in cur]
            if cls == 1:
                sg = (-1.0) ** lag
                re = [jnp.where(lane == 0, (-sg - 1.0) / 512, v) for v in re]
                im = [jnp.where(lane == 0, (1.0 - sg) / 512, v) for v in im]
            r0 = 64 * ((lag - 1) % 2) + 16 * ((lag - 1) // 2)
            put(g0b, r0, 256 * cls, re)
            put(g0b, r0, 256 * cls + 128, im)
            if lag < 8:
                cur = [_cmul(z, s1) for z in cur]


def _ggen(selb, g0b, gm):
    sel = selb[...]

    def onehot(k, r0, n):
        ri = lax.broadcasted_iota(I32, (n, 256), 0) + r0
        return jnp.where(ri == sel[k:k + 1, :], 1.0, 0.0)
    e = jnp.concatenate([onehot(0, 0, 128), onehot(1, 0, 64), onehot(2, 0, 32),
                         onehot(1, 112, 16), onehot(2, 112, 16), onehot(3, 112, 16)], axis=0).astype(BF16)
    g = _dot(e, _bf(g0b[...]))

    def put(r, v):
        gm[pl.ds((r - 256) // 2, v.shape[0] // 2), :] = _u32(v)

    def zero(r, n):
        gm[pl.ds((r - 256) // 2, n // 2), :] = jnp.zeros((n // 2, 512), U32)
    zero(256, 112)
    put(368, g[256:272])
    put(384, g[0:128])
    put(512, g[128:192])
    zero(576, 48)
    put(624, g[224:240])
    put(640, g[128:192])
    put(704, g[192:224])
    zero(736, 80)
    put(816, g[240:256])
    put(832, g[192:224])
    zero(864, 64)


class _Masks:
    def __init__(self):
        sub = lax.broadcasted_iota(I32, (8, 128), 0)
        lane = lax.broadcasted_iota(I32, (8, 128), 1)
        self.lo4 = sub < 4
        self.gidx = 4 * (lane % 32) + (sub % 4)
        self.lo64 = lane < 64
        self.beven = ((lane // 32) % 2) == 0
        self.last = lane == 127
        self.mz = jnp.where(lane == 0, 0.0, 1.0)
        self.row16 = lax.broadcasted_iota(I32, (16, 128), 0)
        self.lane16 = lax.broadcasted_iota(I32, (16, 128), 1)


def _kernel(x_hbm, are_hbm, aim_hbm, bre_hbm, bim_hbm, cre_hbm, cim_hbm, ldt_hbm, dsk_hbm,
            wr_hbm, wg_hbm, wu_hbm, wd_hbm, sel_hbm, out_hbm,
            zs, xb, prm, ldt, dsk, wr, um, g0b, gm, selb,
            umt, dtc, dkc, k0c, kd, xh, vv, ur0, ur1, ur2, yb, ob, rs_s, oh_s, xs_s, hit_s, deff, ya_s, upt_s,
            sem_in, sem_w, sem_o, *rest):
    ksps = rest[:NB]
    wbuf = [rest[NB + 3 * c:NB + 3 * c + 3] for c in range(len(FCH))]
    urs = (ur0, ur1, ur2)

    prs = [are_hbm, aim_hbm, bre_hbm, bim_hbm, cre_hbm, cim_hbm]
    order = (1, 0, 2, 3, 4, 5)
    grp0 = [(ldt_hbm, ldt), (sel_hbm, selb)]
    grp1 = [(prs[i].at[pl.ds(0, R1)], prm.at[i, pl.ds(0, R1)]) for i in order]
    grp2 = [(prs[i].at[pl.ds(R1, D - R1)], prm.at[i, pl.ds(R1, D - R1)]) for i in order]
    grp2 += [(dsk_hbm, dsk), (wr_hbm, wr)]
    grp3 = [(x_hbm, xb)]
    in_cp = []
    for grp in (grp0, grp1, grp2, grp3):
        n0 = sum(len(g) for g in in_cp)
        in_cp.append([pltpu.make_async_copy(s, d, sem_in.at[n0 + i]) for i, (s, d) in enumerate(grp)])
        for cp in in_cp[-1]:
            cp.start()
    w_cp = []
    off = 0
    for c, n in enumerate(FCH):
        cs = pl.ds(off * 128, n * 128)
        w_cp.append([pltpu.make_async_copy(h.at[:, cs], wbuf[c][i].bitcast(BF16), sem_w.at[i, c])
                     for i, h in enumerate([wg_hbm, wu_hbm, wd_hbm])])
        for cp in w_cp[-1]:
            cp.start(priority=1)
        off += n

    mk = [_Masks()]
    _dft_tables(um, umt, g0b)

    for cp in in_cp[0]:
        cp.wait()
    zs[0] = lax.broadcasted_iota(I32, (8, 128), 1)[0, 0]
    dtb = _col_bcast(ldt)
    for t in range(5):
        n = 128 if t < 4 else 64
        dtc[pl.ds(t * 128, n), :] = _rb(jnp.exp(dtb[t][:n]))
    for cp in in_cp[1]:
        cp.wait()
    zrow = pl.multiple_of(zs[0] * 8 + 0, 8)

    in_mac = [False]
    ktq = []
    slotno = [0]
    pend = [None]

    def kt_unit(b, c):
        l0, kk, g0 = _KT[c]
        gw = g0b[...] if c == 0 else gm[pl.ds((g0 - 256) // 2, kk // 2), :]
        raw = _dot(_bf(kd[pl.ds(b * (RB // 2), RB // 2), pl.ds(l0, kk)]), _bf(gw))
        rows = pl.ds(zrow, RB) if in_mac[0] else pl.ds(0, RB)
        ksps[b][rows, pl.ds(512 * c, 512)] = raw

    def kt_drain(n):
        for _ in range(n):
            if ktq and ktq[0][0] <= slotno[0]:
                kt_unit(*ktq.pop(0)[1:])

    def extract(st, o4):
        m = mk[0]
        g = [[jnp.take_along_axis(_pk(o4[0][grp][8 * v:8 * v + 8], o4[1][grp][8 * v:8 * v + 8]), m.gidx, axis=1,
                                  mode="promise_in_bounds") for v in range(10)] for grp in range(2)]

        def mix(a, b):
            return jnp.where(m.lo4, a, b), pltpu.roll(jnp.where(m.lo4, b, a), 4, 0)

        def two(va, vb, m1, m2):
            p, q = mix(jnp.where(m1, g[0][va], g[0][vb]), jnp.where(m1, g[1][va], g[1][vb]))
            return jnp.where(m2, p, q)

        def four(gg):
            return jnp.where(m.lo64, jnp.where(m.beven, gg[2], gg[3]), jnp.where(m.beven, gg[4], gg[5]))
        t_odd = two(0, 1, m.lo64, m.beven)
        t_even, t_2 = mix(four(g[0]), four(g[1]))
        t_3 = two(6, 7, m.beven, m.lo64)
        t_4 = two(8, 9, m.lo64, m.beven)
        tl = [t_odd, t_even, t_2, jnp.where(m.last, t_2, t_3), t_3, jnp.where(m.last, t_3, t_4), t_4]
        for t in range(7):
            kd[pl.ds(st * 8, 8), pl.ds(128 * t, 128)] = tl[t]

    def flush():
        extract(*pend[0])
        if (pend[0][0] + 1) % SPB == 0:
            ktq.extend([(slotno[0] + 4, pend[0][0] // SPB, c) for c in range(NCH)])
        pend[0] = None

    def kgen(s0, s1):
        for st in range(s0, s1):
            o4 = []
            for half in range(2):
                r0 = st * 16
                pk = [pltpu.bitcast(prm[k, pl.ds(r0, 16), :], U32) for k in range(6)]
                rows = pl.ds(r0 + half, 8, stride=2)
                bs, k0 = _base8([_upk(w, half) for w in pk], dtc[rows, :])
                k0c[rows, :] = jnp.broadcast_to(k0, (8, 128))
                xy = [_grp_xy(bs, grp, mk[0].lo4) for grp in range(2)]
                if half == 0 and pend[0] is not None:
                    flush()
                oo = []
                for grp in range(2):
                    yield
                    slotno[0] += 1
                    oo.append(_dot_nt(*xy[grp]))
                o4.append(oo)
            pend[0] = (st, o4)
        if s1 == NS:
            flush()

    tk = {}

    def ln_chunk(j):
        cj = slice(256 * j, 256 * j + 256)
        s1 = s2 = None
        for i in range(NS):
            v16 = xb[pl.ds(i * 16, 16), cj].astype(F32)
            for v in (v16[:8], v16[8:]):
                s1, s2 = (v, v * v) if s1 is None else (s1 + v, s2 + v * v)
        mean = jnp.sum(s1, axis=0, keepdims=True) * (1.0 / D)
        var = jnp.sum(s2, axis=0, keepdims=True) * (1.0 / D) - mean * mean
        var = jnp.maximum(var, 0.0)
        sd = _rb(jnp.sqrt(_rb(_rb(var) + 1e-5)))
        mb = jnp.broadcast_to(_rb(mean), (16, 256))
        hi = jnp.broadcast_to(0.5 / sd, (16, 256))
        if j == 0:
            wrow = wr[...].astype(F32).reshape(1, D)
            tk["w"] = [(jnp.broadcast_to(wrow[:, k0:min(k0 + 128, D)], (16, min(128, D - k0)))
                        + jnp.zeros((16, min(128, D - k0)), F32)).astype(BF16) for k0 in range(0, D, 128)]
        r = None
        for i in range(NS):
            rw = pl.ds(i * 8, 8)
            hv = _rb(xb[pl.ds(i * 16, 16), cj].astype(F32) - mb) * hi
            h0, h1 = hv[:, :128], hv[:, 128:]
            xh[rw, pl.ds(256 * j, 128)] = _u32(h0)
            xh[rw, pl.ds(256 * j + 128, 128)] = _u32(h1)
            vv[rw, pl.ds(256 * j, 128)] = _u32(h0 + h1)
            vv[rw, pl.ds(256 * j + 128, 128)] = _u32(h0 - h1)
            if i % 8 == 7 or i == NS - 1:
                k0, k1 = (i // 8) * 128, (i + 1) * 16
                yield
                p = _dot(tk["w"][i // 8], _bf(xh[pl.ds(k0 // 2, (k1 - k0) // 2), cj]))
                r = p if r is None else r + p
        for t in range(2):
            r_t = r[:, 128 * t:128 * t + 128]
            tk["rc"] = r_t if (j == 0 and t == 0) else jnp.where(mk[0].row16 == 2 * j + t, r_t, tk["rc"])

    def topk():
        m = mk[0]
        bits = pltpu.bitcast(_rb(tk["rc"] * 2.0), I32)
        mono = (jnp.where(bits < 0, bits ^ 0x7FFF0000, bits) >> 16) + 32768
        key = pltpu.bitcast(0x30000000 + (mono << 11) + (2047 - (m.row16 * 128 + m.lane16)), F32)
        kcol = jnp.zeros((16, 128), I32)
        for j in range(NSEL):
            mx = jnp.max(jnp.max(key, axis=0, keepdims=True), axis=1, keepdims=True)
            mxb = jnp.broadcast_to(mx, (16, 128))
            key = jnp.where(key == mxb, 0.0, key)
            kcol = jnp.where(m.row16 == j, pltpu.bitcast(mxb, I32), kcol)
        kcol = kcol - 0x30000000
        idxcol = jnp.where(m.row16 < NSEL, 2047 - (kcol & 2047), -1)
        hb = ((kcol >> 11) - 32768) << 16
        rsel = pltpu.bitcast(jnp.where(hb < 0, hb ^ 0x7FFF0000, hb), F32)
        rsel = jnp.where(m.row16 < NSEL, rsel, 0.0)
        rs_s[...] = _rb(jax.nn.sigmoid(rsel))
        oh = jnp.concatenate(
            [jnp.where(idxcol == m.lane16 + 128 * t, 1.0, 0.0) for t in range(16)], axis=1).astype(BF16)
        oh_s[...] = pltpu.bitcast(oh, U32)
        hits = jnp.where(m.row16[:8] < NSEL, jnp.left_shift(1, jnp.maximum(idxcol[:8], 0) >> 7), 0)
        for sh in (4, 2, 1):
            hits = hits | pltpu.roll(hits, sh, 0)
        hit_s[0] = hits[0, 0]
        tcol = jnp.maximum(idxcol, 0) >> 7
        tk["tj"] = [tcol[j, 0] for j in range(NSEL)]
        tk["ol"] = jnp.where((idxcol & 127) == m.lane16, 1.0, 0.0)

    def xsel(j):
        off = pl.multiple_of(tk["tj"][j] * 128, 128)
        lhs = jnp.where(mk[0].row16 == j, tk["ol"], 0.0).astype(BF16)
        v = _dot_nt(lhs, _bf(xh[:, pl.ds(off, 128)]))
        tk["xa"] = v if j == 0 else tk["xa"] + v
        if j == NSEL - 1:
            xs_s[...] = _u32(tk["xa"] * 2.0)

    ffp = [0, 0]
    ffp_max = [0]

    def wpiece(i, p):
        c = 0
        while 2 * p >= sum(FCH[:c + 1]):
            c += 1
        return _bf(wbuf[c][i][:, pl.ds(256 * p - 128 * sum(FCH[:c]), 256)])

    def ffn_gu():
        p = ffp[0]
        ffp[0] += 1
        gu = _dot(tk["xs"], jnp.concatenate([wpiece(0, p), wpiece(1, p)], axis=1))
        g = _rb(gu[:, :256])
        u = _rb(gu[:, 256:])
        sg = _rb(0.5 * jnp.tanh(0.5 * g) + 0.5)
        tk["h", p] = (_rb(g * sg) * u).astype(BF16)

    def ffn_dn():
        p = ffp[1]
        ffp[1] += 1
        y = _dot_nt(tk.pop(("h", p)), wpiece(2, p))
        tk["y"] = y if p == 0 else tk["y"] + y

    def ffn_next():
        if ffp[1] < ffp[0] - 1 or (ffp[1] < ffp[0] and ffp[0] >= ffp_max[0]):
            ffn_dn()
        elif ffp[0] < ffp_max[0]:
            ffn_gu()

    def fin16(i, c0, c1, du):
        r16 = pl.ds(16 * i, 16)
        cs = pl.ds(128 * c0, 128 * (c1 - c0))
        h = _bf(xh[pl.ds(8 * i, 8), cs]).astype(F32)
        y = jnp.concatenate([_upk(yb[r16, pl.ds(256 * (c // 4) + 128 * (c % 2), 128)], (c // 2) % 2)
                             for c in range(c0, c1)], axis=1)
        dv = deff[r16, :]
        s = y + h * jnp.concatenate([dv] * (c1 - c0), axis=1)
        zh = h if du is None else h + du
        g = zh * jnp.tanh(zh) + zh
        ob[r16, cs] = (xb[r16, cs].astype(F32) + s * g).astype(BF16)

    def ut_piece(b, k, j0):
        rw = pl.ds(b * (RU // 2), RU // 2)
        rows = pl.ds(zrow, RU)
        ur = urs[b % 3]
        js = range(j0, j0 + UTJ)

        def lhs(ref, o):
            return _bf(jnp.concatenate([ref[rw, pl.ds(256 * j + o, 128)] for j in js], axis=0))

        def put(val, col):
            for i, j in enumerate(js):
                ur[rows, pl.ds(640 * j + col, 128)] = val[i * RU:(i + 1) * RU]
        if k == 0:
            v = _dot(lhs(vv, 0), _bf(um[:, 0:256]))
            b2 = _dot(lhs(vv, 128), _bf(um[:, 256:384]))
            a0 = v[:, :128]

            def sel(p, q):
                return jnp.concatenate([jnp.where(mk[0].lo64, p[8 * i:8 * i + 8], q[8 * i:8 * i + 8])
                                        for i in range(a0.shape[0] // 8)], axis=0)
            put(sel(a0, b2), 0)
            put(v[:, 128:], 128)
            put(pltpu.roll(sel(b2, a0), 64, 1), 256)
        else:
            put(_dot(lhs(xh, 128), _bf(um[:, 384:512])), 384)
            put(_dot(lhs(xh, 0), _bf(um[:, 512:640])), 512)

    def mac(g, cls):
        ur = urs[(8 * g // RU) % 3]
        m = mk[0]

        @functools.lru_cache(None)
        def us(j):
            def ld(c):
                return ur[pl.ds((8 * g) % RU, 8), pl.ds(640 * j + c, 128)]
            if cls == 0:
                a, b = ld(0), ld(256)
                return (a, b, a + b)
            t1, t2, t3 = ld(128), ld(384), ld(512)
            return (t1 + t2, t3 - t1, t2 + t3)

        @functools.lru_cache(None)
        def kraw(j):
            o = 512 * j + 256 * (1 - cls)
            ksp, kr = ksps[8 * g // RB], pl.ds((8 * g) % RB, 8)
            return ksp[kr, pl.ds(o, 128)], ksp[kr, pl.ds(o + 128, 128)]

        @functools.lru_cache(None)
        def ks(j):
            sr, si = kraw(j)
            if j > 0:
                pr, pi_ = kraw(j - 1)
                sr, si = (sr + pr, si + pi_) if cls == 0 else (sr - pr, si - pi_)
            return (sr * m.mz if cls == 0 else sr, si - sr, sr + si)
        outs = []
        prev = None
        for mo in range(NCH):
            acc = None
            for j in range(mo + 1):
                a, b, s = us(j)
                c_, e_, g_ = ks(mo - j)
                t = (c_ * s, a * e_, b * g_)
                acc = t if acc is None else tuple(x + y for x, y in zip(acc, t))
            z = (acc[0] - acc[2], acc[0] + acc[1])
            if mo % 2 == 1:
                za, zb = prev, z
                if cls == 0:
                    zr = _pk(za[0], zb[0])
                    zis = pltpu.roll(_pk(za[1], zb[1]), 64, 1)
                    outs.append((jnp.where(m.lo64, zr, zis), jnp.where(m.lo64, zis, zr)))
                else:
                    outs.append((_pk(za[0] + za[1], zb[0] + zb[1]), _pk(za[1], zb[1]), _pk(za[0], zb[0])))
            prev = z
        return outs

    zq, wq = {}, {}

    def inv(g, cls):
        zo = zq.pop((g, cls))

        def st(t):
            return _bf(jnp.concatenate([zo[p][t] for p in range(4)], axis=0))
        if cls == 0:
            wq[g] = [_dot(st(t), _bf(umt[:, c:c + 128])) for t, c in ((0, 0), (1, 256))]
        else:
            q1, q2, q3 = [_dot(st(t), _bf(umt[:, c:c + 128])) for t, c in ((0, 128), (1, 384), (2, 512))]
            w0, w2 = wq.pop(g)
            p_ = q1 + w2
            y0 = p_ + (q2 + w0)
            y1 = (q3 + w0) - p_
            for p in range(4):
                yb[pl.ds(8 * g, 8), pl.ds(256 * p, 128)] = _u32(y0[16 * p:16 * p + 16])
                yb[pl.ds(8 * g, 8), pl.ds(256 * p + 128, 128)] = _u32(y1[16 * p:16 * p + 16])

    def region(fn):
        @pl.when(zs[0] == 0)
        def _():
            mk[0] = _Masks()
            fn()

    for i, _ in enumerate(kgen(0, R1 // 16)):
        if i == 3:
            _ggen(selb, g0b, gm)
    for cp in in_cp[2]:
        cp.wait()
    slotno[0] += 100
    for _ in kgen(R1 // 16, XW):
        pass
    dkb = _col_bcast(dsk)
    for t in range(5):
        n = 128 if t < 4 else 64
        dkc[pl.ds(t * 128, n), :] = dkb[t][:n]
    in_cp[3][0].wait()

    def phase_a2():
        slotno[0] += 100
        kg = kgen(XW, NS)
        next(kg)
        nslot = 0
        for j in range(NCH):
            for k, _ in enumerate(ln_chunk(j)):
                kt_drain(2 if k == 0 else 1)
                nslot += 1
                if nslot % 5 == 0:
                    next(kg)
        topk()
        xq = list(range(NSEL))
        for i, _ in enumerate(kg):
            kt_drain(i % 2)
            if i >= 16 and xq and (i - 16) % 3 == 0:
                xsel(xq.pop(0))
        while xq:
            xsel(xq.pop(0))
        slotno[0] += 1000
        kt_drain(len(ktq) - NCH)

    region(phase_a2)

    utq = [(b, k, j) for b in range(D // RU) for j in range(0, NCH, UTJ) for k in range(2)]

    def mac_groups(g0, g1):
        for s in range(g0, g1):
            for cls in range(2):
                if s < NG:
                    zq[(s, cls)] = mac(s, cls)
                if 1 <= s < NG + 1:
                    inv(s - 1, cls)
                if utq:
                    ut_piece(*utq.pop(0))
                if cls == 1 and s % 4 == 2:
                    kt_drain(1)
                q = 2 * (s - 2) + cls - 2
                if 0 <= q < 4 * NS:
                    fin16(q // 4, 4 * (q % 4), 4 * (q % 4) + 4, None)
                if cls == 0 and (s - g0) % 2 == 0:
                    ffn_next()

    def phase_b():
        in_mac[0] = True
        ends = [gs for gs, _ in FWAIT[1:]] + [NG + 4]
        for (gs, cc), ge in zip(FWAIT, ends):
            for cp in w_cp[cc]:
                cp.wait()
            ffp_max[0] = sum(FCH[:cc + 1]) // 2
            tk["xs"] = _bf(xs_s[...])
            if gs == 0:
                for _ in range(8):
                    ut_piece(*utq.pop(0))
                for t in range(5):
                    rows = pl.ds(128 * t, 128 if t < 4 else 64)
                    deff[rows, :] = (dkc[rows, :] + k0c[rows, :]) * 2.0
            mac_groups(gs, ge)
        while ffp[1] < ffp_max[0]:
            ffn_next()
        ya_s[...] = tk["y"]

    region(phase_b)

    o_cp = [pltpu.make_async_copy(ob.at[:, pl.ds(128 * t, 128)], out_hbm.at[:, pl.ds(128 * t, 128)], sem_o.at[t])
            for t in range(16)]
    tk["xs"] = _bf(xs_s[...])
    rs = rs_s[...]
    tk["y"] = ya_s[...]
    for cc in range(len(FWAIT), len(FCH)):
        for cp in w_cp[cc]:
            cp.wait()
    hit = hit_s[0]
    for t in range(16):
        @pl.when(((hit >> t) & 1) == 0)
        def _():
            o_cp[t].start(priority=1)
    while ffp[0] < sum(FCH) // 2:
        ffn_gu()
        if ffp[1] < ffp[0] - 1:
            ffn_dn()
    while ffp[1] < ffp[0]:
        ffn_dn()
    upd = (_rb(_rb(tk["y"]) * jnp.concatenate([rs] * 5, axis=1)[:, :D]) * 0.5).astype(BF16)
    upt_s[...] = jnp.concatenate([upd, jnp.zeros((16, 64), BF16)], axis=1).T
    hit = hit_s[0]
    for t in range(16):
        @pl.when(((hit >> t) & 1) == 1)
        def _():
            du = _dot(upt_s[pl.ds(0, D), :], _bf(oh_s[:, pl.ds(128 * t, 128)]))
            for i in range(NS):
                fin16(i, t, t + 1, du[16 * i:16 * i + 16])
            o_cp[t].start(priority=1)
    for cp in o_cp:
        cp.wait()


@jax.jit
def pallas_recurrent_scan__ssm_conv_s4__moe_arch_mod__prompt_kernel(
        A_u, A_A_re, A_A_im, A_B_re, A_B_im, A_C_re, A_C_im, A_log_dt, A_Dskip,
        B_x, B_w_r, B_w_gate, B_w_up, B_w_down):
    scratch = [
        pltpu.SMEM((1,), I32),
        pltpu.VMEM((D, L), BF16),
        pltpu.VMEM((6, D, N), BF16),
        pltpu.VMEM((D,), BF16),
        pltpu.VMEM((D,), BF16),
        pltpu.VMEM((D,), BF16),
        pltpu.VMEM((64, 640), U32),
        pltpu.VMEM((128, 512), U32),
        pltpu.VMEM((336, 512), U32),
        pltpu.VMEM((8, 256), I32),
        pltpu.VMEM((64, 640), U32),
        pltpu.VMEM((D, 128), F32),
        pltpu.VMEM((D, 128), F32),
        pltpu.VMEM((D, 128), F32),
        pltpu.VMEM((D // 2, 896), U32),
        pltpu.VMEM((D // 2, L), U32),
        pltpu.VMEM((D // 2, L), U32),
        pltpu.VMEM((RU, 5120), F32),
        pltpu.VMEM((RU, 5120), F32),
        pltpu.VMEM((RU, 5120), F32),
        pltpu.VMEM((D, L // 2), U32),
        pltpu.VMEM((D, L), BF16),
        pltpu.VMEM((16, 128), F32),
        pltpu.VMEM((8, L), U32),
        pltpu.VMEM((8, D), U32),
        pltpu.SMEM((1,), I32),
        pltpu.VMEM((D, 128), F32),
        pltpu.VMEM((16, D), F32),
        pltpu.VMEM((640, 16), BF16),
        pltpu.SemaphoreType.DMA((17,)),
        pltpu.SemaphoreType.DMA((3, len(FCH))),
        pltpu.SemaphoreType.DMA((16,)),
    ]
    scratch += [pltpu.VMEM((RB, 4096), F32)] * NB
    scratch += [pltpu.VMEM((D // 2, 128 * n), U32) for n in FCH for _ in range(3)]
    out = pl.pallas_call(
        _kernel,
        out_shape=jax.ShapeDtypeStruct((D, L), BF16),
        in_specs=[pl.BlockSpec(memory_space=pl.ANY)] * 14,
        out_specs=pl.BlockSpec(memory_space=pl.ANY),
        scratch_shapes=scratch,
        compiler_params=pltpu.CompilerParams(vmem_limit_bytes=100 * 2**20, disable_semaphore_checks=True,
                                             disable_bounds_checks=True),
        name="s4_mod",
    )(jnp.transpose(A_u[0]), A_A_re, A_A_im, A_B_re, A_B_im, A_C_re, A_C_im, A_log_dt, A_Dskip,
      B_w_r, B_w_gate, B_w_up, jnp.transpose(B_w_down), jnp.asarray(_SEL))
    return jnp.transpose(out)[None]
```

```python
import functools
import math

import numpy as np
import jax
import jax.numpy as jnp
from jax import lax
import jax.experimental.pallas as pl
import jax.experimental.pallas.tpu as pltpu

F32 = jnp.float32
BF16 = jnp.bfloat16
U32 = jnp.uint32
I32 = jnp.int32

D = 576
L = 2048
N = 128
NSEL = 8
NCH = 8
NS = D // 16
NG = D // 8
RB = 64
NB = D // RB
SPB = RB // 16
RU = 16
UTJ = 4
R1 = 128
XW = 22
FCH = (10, 10, 8, 8)
FWAIT = ((0, 0), (26, 1), (51, 2))

_TILES = {
    "odd": (1, 3, 5, 7),
    "even": (2, 4, 6, 8),
    "t2": (258, 260, 262, 264),
    "t3": (516, 520, 772, 776),
    "t4": (1032, 1288, 1544, 1800),
}
_KT = [(0, 256, 0), (128, 256, 256), (384, 128, 512), (512, 128, 576),
       (640, 128, 704), (768, 128, 800), (768, 128, 768), (768, 128, 736)]


def _rlag(l):
    u = int(np.float32(l).view(np.uint32))
    u = (u + 0x7FFF + ((u >> 16) & 1)) & 0xFFFF0000
    return int(np.uint32(u).view(np.float32))


def _tile_pts(name):
    base = name.rstrip("v")
    p = np.array([_TILES[base][l // 32] + 8 * (l % 32) for l in range(128)])
    if name == "t3v":
        p[127] = 512
    if name == "t4v":
        p[127] = 1024
    return p


def _sel_table():
    lags = np.concatenate([_tile_pts("odd"), _tile_pts("even")])
    sel = np.full((8, 256), -1, np.int32)
    for k, (c, tile) in enumerate([(1, "t2"), (2, "t3v"), (4, "t4v"), (1, "even")]):
        pts = _tile_pts(tile)
        for rho, r in enumerate(lags):
            idx = np.nonzero(pts == _rlag(256 * c + int(r)))[0]
            if len(idx):
                sel[k, rho] = idx[0]
    return sel


_SEL = _sel_table()


def _bf(x):
    return pltpu.bitcast(x, BF16)


def _u32(x):
    return pltpu.bitcast(x.astype(BF16), U32)


def _rb(x):
    return x.astype(BF16).astype(F32)


def _cmul(a, b):
    return (a[0] * b[0] - a[1] * b[1], a[0] * b[1] + a[1] * b[0])


def _csq(a):
    t = a[0] * a[1]
    return (a[0] * a[0] - a[1] * a[1], t + t)


def _sincos(th):
    kf = th * (2.0 / math.pi) + 12582912.0
    ki = pltpu.bitcast(kf, I32)
    k = (ki - 0x4B400000).astype(F32)
    r = th - k * 1.5703125
    r = r - k * 4.837512969970703125e-4
    r = r - k * 7.54978995489188216e-8
    r2 = r * r
    s = r + r * r2 * (-1.6666654611e-1 + r2 * (8.3321608736e-3 + r2 * -1.9515295891e-4))
    c = 1.0 + r2 * (-0.5 + r2 * (4.166664568298827e-2 + r2 * (-1.388731625493765e-3 + r2 * 2.443315711809948e-5)))
    swap = (ki & 1) == 1
    sn = jnp.where(swap, c, s)
    cs = jnp.where(swap, s, c)
    sbit = (ki & 2) << 30
    cbit = ((ki + 1) & 2) << 30
    sn = pltpu.bitcast(pltpu.bitcast(sn, I32) ^ sbit, F32)
    cs = pltpu.bitcast(pltpu.bitcast(cs, I32) ^ cbit, F32)
    return cs, sn


def _dot(a, b):
    return jnp.dot(a, b, preferred_element_type=F32)


def _dot_nt(a, b):
    return lax.dot_general(a, b, (((1,), (1,)), ((), ())), preferred_element_type=F32)


def _col_bcast(vec_ref):
    v = vec_ref[...].astype(F32).reshape(1, D)
    vp = jnp.concatenate([v, jnp.zeros((1, 64), F32)], axis=1)
    return [jnp.broadcast_to(vp[:, t * 128:(t + 1) * 128], (128, 128)).T for t in range(5)]


def _base8(p, dt):
    are, aim, bre, bim, cre, cim = p
    y1 = (dt * are) * math.log2(math.e)
    ph = {1: _sincos(dt * aim)}
    e = 1
    while e < 512:
        ph[2 * e] = _csq(ph[e])
        e *= 2
    pw = {}
    for e in (1, 2, 4, 8, 16, 256, 512):
        mg = jnp.exp2(y1 * float(e)) if e > 1 else jnp.exp2(y1)
        pw[e] = (mg * ph[e][0], mg * ph[e][1])
    w = _cmul((cre, cim), (dt * bre, dt * bim))
    k0 = jnp.sum(w[0], axis=1, keepdims=True)
    w1 = _cmul(w, pw[1])
    w2 = _cmul(w1, pw[1])
    w3 = _cmul(w2, pw[1])
    w258 = _cmul(w2, pw[256])

    def rot(z):
        return (pltpu.roll(z[0], 4, 0), pltpu.roll(z[1], 4, 0))
    rots = {e: rot(pw[e]) for e in (2, 4, 8, 16, 512)}
    return (pw, rots, w1, w2, rot(w3), rot(w258)), k0


def _grp_xy(bs, grp, lo4):
    pw, rots, w1, w2, w3r, w258r = bs

    def sel(lo, hi):
        return (jnp.where(lo4, lo[0], hi[0]), jnp.where(lo4, lo[1], hi[1]))
    if grp == 0:
        dup = {e: sel(pw[e], rots[e]) for e in (2, 4, 16, 512)}
        x0, x2, a8 = sel(w1, w3r), sel(w2, w258r), rots[8]
    else:
        dup = {e: sel(rots[e], pw[e]) for e in (2, 4, 16, 512)}
        x0, x2, a8 = sel(w3r, w1), sel(w258r, w2), pw[8]
    xv = [None] * 10
    xv[0] = x0
    xv[1] = _cmul(x0, dup[4])
    xv[2] = x2
    xv[3] = _cmul(xv[2], dup[2])
    xv[4] = _cmul(xv[3], dup[2])
    xv[5] = _cmul(xv[4], dup[2])
    xv[6] = _cmul(xv[3], dup[512])
    xv[7] = _cmul(xv[5], dup[512])
    xv[8] = _cmul(xv[7], dup[512])
    xv[9] = _cmul(xv[8], dup[512])
    y = (jnp.where(lo4, 1.0, a8[0]), jnp.where(lo4, 0.0, -a8[1]))
    m = dup[16]
    ys = [y]
    for _ in range(15):
        y = (y[0] * m[0] + y[1] * m[1], y[1] * m[0] - y[0] * m[1])
        ys.append(y)

    def mat(vs):
        return jnp.concatenate([jnp.concatenate([v[0] for v in vs], 0),
                                jnp.concatenate([v[1] for v in vs], 0)], 1).astype(BF16)
    return mat(xv), mat(ys)


def _dft_tables(um, umt, g0b):
    sub = lax.broadcasted_iota(I32, (8, 128), 0)
    lane = lax.broadcasted_iota(I32, (8, 128), 1)
    lo = lane < 64

    def e512(m):
        return _sincos((m & 511).astype(F32) * (-2.0 * math.pi / 512.0))

    def chain(base, step, n):
        out = [base]
        for _ in range(n - 1):
            out.append(_cmul(out[-1], step))
        return out

    def row(z, r):
        return tuple(jnp.broadcast_to(c[r:r + 1], (8, 128)) for c in z)

    def put(ref, r0, c0, vs):
        for i in range(0, len(vs), 2):
            ref[pl.ds(r0 + 4 * i, 8), pl.ds(c0, 128)] = _u32(jnp.concatenate([vs[i], vs[i + 1]], axis=0))
    f1 = 4 * lane + 1
    k4 = 4 * (lane & 63)
    alt_r = jnp.where((sub & 1) == 1, 1.0, -1.0)
    alt_l = jnp.where((lane & 1) == 1, 1.0, -1.0)
    b1 = e512(f1 * (sub + 1))
    c1 = chain(b1, row(b1, 7), 16)
    put(um, 0, 128, [z[0] for z in c1])
    put(um, 0, 384, [z[1] - z[0] for z in c1])
    put(um, 0, 512, [z[0] + z[1] for z in c1])
    for col, off, q in ((0, 0, jnp.where(lo, 0, 128)), (256, 2, jnp.where(lo, 128, 0))):
        b = e512((k4 + off) * (sub + 1))
        c = chain(e512((k4 + off) * (sub + 1) + q), row(b, 7), 16)
        vs = [z[0] for z in c]
        if off == 0:
            vs = [jnp.where(lane == 64, alt_r, v) for v in vs]
        put(um, 0, col, vs)
    st = e512(32 * (lane + 1))
    c = chain(e512((4 * sub + 1) * (lane + 1)), st, 16)
    put(umt, 0, 128, [z[0] for z in c])
    put(umt, 0, 384, [z[1] - z[0] for z in c])
    put(umt, 0, 512, [z[0] + z[1] for z in c])
    c = chain(e512(4 * sub * (lane + 1)), st, 8)
    re = [z[0] for z in c]
    im = [z[1] for z in c]
    re[0] = jnp.where(sub == 0, alt_l, re[0])
    im[0] = jnp.where(sub == 0, 1.0, im[0])
    put(umt, 0, 0, re + im)
    c = chain(e512((4 * sub + 2) * (lane + 1)), st, 8)
    put(umt, 0, 256, [z[1] for z in c] + [z[0] for z in c])
    for cls, f in ((0, f1), (1, k4 + jnp.where(lo, 0, 2))):
        b = e512(f * (1 + 8 * sub))
        s1 = row(b, 0)
        s64 = e512(f * 64)
        cur = chain((b[0] * (1.0 / 128), b[1] * (1.0 / 128)), s64, 4)
        for lag in range(1, 9):
            re = [z[0] for z in cur]
            im = [z[1] for z in cur]
            if cls == 1:
                sg = (-1.0) ** lag
                re = [jnp.where(lane == 0, (-sg - 1.0) / 512, v) for v in re]
                im = [jnp.where(lane == 0, (1.0 - sg) / 512, v) for v in im]
            r0 = 64 * ((lag - 1) % 2) + 16 * ((lag - 1) // 2)
            put(g0b, r0, 256 * cls, re)
            put(g0b, r0, 256 * cls + 128, im)
            if lag < 8:
                cur = [_cmul(z, s1) for z in cur]


def _ggen(selb, g0b, gm):
    sel = selb[...]

    def onehot(k, r0, n):
        ri = lax.broadcasted_iota(I32, (n, 256), 0) + r0
        return jnp.where(ri == sel[k:k + 1, :], 1.0, 0.0)
    e = jnp.concatenate([onehot(0, 0, 128), onehot(1, 0, 64), onehot(2, 0, 32),
                         onehot(1, 112, 16), onehot(2, 112, 16), onehot(3, 112, 16)], axis=0).astype(BF16)
    g = _dot(e, _bf(g0b[...]))

    def put(r, v):
        gm[pl.ds((r - 256) // 2, v.shape[0] // 2), :] = _u32(v)

    def zero(r, n):
        gm[pl.ds((r - 256) // 2, n // 2), :] = jnp.zeros((n // 2, 512), U32)
    zero(256, 112)
    put(368, g[256:272])
    put(384, g[0:128])
    put(512, g[128:192])
    zero(576, 48)
    put(624, g[224:240])
    put(640, g[128:192])
    put(704, g[192:224])
    zero(736, 80)
    put(816, g[240:256])
    put(832, g[192:224])
    zero(864, 64)


class _Masks:
    def __init__(self):
        sub = lax.broadcasted_iota(I32, (8, 128), 0)
        lane = lax.broadcasted_iota(I32, (8, 128), 1)
        self.lo4 = sub < 4
        self.gidx = 4 * (lane % 32) + (sub % 4)
        self.lo64 = lane < 64
        self.beven = ((lane // 32) % 2) == 0
        self.last = lane == 127
        self.mz = jnp.where(lane == 0, 0.0, 1.0)
        self.row16 = lax.broadcasted_iota(I32, (16, 128), 0)
        self.lane16 = lax.broadcasted_iota(I32, (16, 128), 1)


def _kernel(x_hbm, are_hbm, aim_hbm, bre_hbm, bim_hbm, cre_hbm, cim_hbm, ldt_hbm, dsk_hbm,
            wr_hbm, wg_hbm, wu_hbm, wd_hbm, sel_hbm, out_hbm,
            zs, xb, prm, ldt, dsk, wr, um, g0b, gm, selb,
            umt, dtc, dkc, k0c, xh, vv, ur0, ur1, ur2, yb, ob, rs_s, oh_s, xs_s, hit_s, deff, ya_s, upt_s,
            sem_in, sem_w, sem_o, *rest):
    ksps = rest[:NB]
    kds = rest[-NB:]
    wbuf = [rest[NB + 3 * c:NB + 3 * c + 3] for c in range(len(FCH))]
    urs = (ur0, ur1, ur2)

    prs = [are_hbm, aim_hbm, bre_hbm, bim_hbm, cre_hbm, cim_hbm]
    order = (1, 0, 2, 3, 4, 5)
    grp0 = [(ldt_hbm, ldt), (sel_hbm, selb)]
    grp1 = [(prs[i].at[pl.ds(0, R1)], prm.at[i, pl.ds(0, R1)]) for i in order]
    grp2 = [(prs[i].at[pl.ds(R1, D - R1)], prm.at[i, pl.ds(R1, D - R1)]) for i in order]
    grp2 += [(dsk_hbm, dsk), (wr_hbm, wr)]
    grp3 = [(x_hbm, xb)]
    in_cp = []
    for grp in (grp0, grp1, grp2, grp3):
        n0 = sum(len(g) for g in in_cp)
        in_cp.append([pltpu.make_async_copy(s, d, sem_in.at[n0 + i]) for i, (s, d) in enumerate(grp)])
        for cp in in_cp[-1]:
            cp.start()
    w_cp = []
    off = 0
    for c, n in enumerate(FCH):
        cs = pl.ds(off * 128, n * 128)
        w_cp.append([pltpu.make_async_copy(h.at[:, cs], wbuf[c][i].bitcast(BF16), sem_w.at[i, c])
                     for i, h in enumerate([wg_hbm, wu_hbm, wd_hbm])])
        for cp in w_cp[-1]:
            cp.start(priority=1)
        off += n

    mk = [_Masks()]
    _dft_tables(um, umt, g0b)

    for cp in in_cp[0]:
        cp.wait()
    zs[0] = lax.broadcasted_iota(I32, (8, 128), 1)[0, 0]
    dtb = _col_bcast(ldt)
    for t in range(5):
        n = 128 if t < 4 else 64
        dtc[pl.ds(t * 128, n), :] = _rb(jnp.exp(dtb[t][:n]))
    for cp in in_cp[1]:
        cp.wait()
    zoff = zs[0] * 8

    def dyn(r):
        return pl.multiple_of(zoff + r, 8)

    in_mac = [False]
    ktq = []
    slotno = [0]
    pend = [None]

    def kt_unit(b, c):
        l0, kk, g0 = _KT[c]
        gw = g0b[...] if c == 0 else gm[pl.ds((g0 - 256) // 2, kk // 2), :]
        raw = _dot(kds[b][:, pl.ds(l0, kk)].astype(BF16), _bf(gw))
        rows = pl.ds(dyn(0), RB) if in_mac[0] else pl.ds(0, RB)
        ksps[b][rows, pl.ds(512 * c, 512)] = raw

    def kt_drain(n):
        for _ in range(n):
            if ktq and ktq[0][0] <= slotno[0]:
                kt_unit(*ktq.pop(0)[1:])

    def extract(st, o4):
        m = mk[0]

        def mix(a, b):
            return jnp.where(m.lo4, a, b), pltpu.roll(jnp.where(m.lo4, b, a), 4, 0)

        def four(gg):
            return jnp.where(m.lo64, jnp.where(m.beven, gg[2], gg[3]), jnp.where(m.beven, gg[4], gg[5]))
        for half in range(2):
            g = [[jnp.take_along_axis(o4[half][grp][8 * v:8 * v + 8], m.gidx, axis=1, mode="promise_in_bounds")
                  for v in range(10)] for grp in range(2)]

            def two(va, vb, m1, m2):
                p, q = mix(jnp.where(m1, g[0][va], g[0][vb]), jnp.where(m1, g[1][va], g[1][vb]))
                return jnp.where(m2, p, q)
            t_odd = two(0, 1, m.lo64, m.beven)
            t_even, t_2 = mix(four(g[0]), four(g[1]))
            t_3 = two(6, 7, m.beven, m.lo64)
            t_4 = two(8, 9, m.lo64, m.beven)
            tl = [t_odd, t_even, t_2, jnp.where(m.last, t_2, t_3), t_3, jnp.where(m.last, t_3, t_4), t_4]
            for t in range(7):
                kds[st // SPB][pl.ds(dyn((st % SPB) * 16 + 8 * half), 8), pl.ds(128 * t, 128)] = tl[t]

    def flush():
        extract(*pend[0])
        if (pend[0][0] + 1) % SPB == 0:
            ktq.extend([(slotno[0] + 4, pend[0][0] // SPB, c) for c in range(NCH)])
        pend[0] = None

    def kgen(s0, s1):
        for st in range(s0, s1):
            o4 = []
            for half in range(2):
                rows = pl.ds(st * 16 + 8 * half, 8)
                ps = [prm[k, pl.ds(st * 16, 16), :].astype(F32)[8 * half:8 * half + 8] for k in range(6)]
                bs, k0 = _base8(ps, dtc[rows, :])
                k0c[rows, :] = jnp.broadcast_to(k0, (8, 128))
                xy = [_grp_xy(bs, grp, mk[0].lo4) for grp in range(2)]
                if half == 0 and pend[0] is not None:
                    flush()
                oo = []
                for grp in range(2):
                    yield
                    slotno[0] += 1
                    oo.append(_dot_nt(*xy[grp]))
                o4.append(oo)
            pend[0] = (st, o4)
        if s1 == NS:
            flush()

    tk = {}
    ysv = {}

    def ln_chunk(j):
        cj = slice(256 * j, 256 * j + 256)
        s1 = s2 = None
        for i in range(NS):
            v16 = xb[pl.ds(i * 16, 16), cj].astype(F32)
            for v in (v16[:8], v16[8:]):
                s1, s2 = (v, v * v) if s1 is None else (s1 + v, s2 + v * v)
        mean = jnp.sum(s1, axis=0, keepdims=True) * (1.0 / D)
        var = jnp.sum(s2, axis=0, keepdims=True) * (1.0 / D) - mean * mean
        var = jnp.maximum(var, 0.0)
        sd = _rb(jnp.sqrt(_rb(_rb(var) + 1e-5)))
        mb = jnp.broadcast_to(_rb(mean), (16, 256))
        hi = jnp.broadcast_to(0.5 / sd, (16, 256))
        if j == 0:
            wrow = wr[...].astype(F32).reshape(1, D)
            tk["w"] = [(jnp.broadcast_to(wrow[:, k0:min(k0 + 128, D)], (16, min(128, D - k0)))
                        + jnp.zeros((16, min(128, D - k0)), F32)).astype(BF16) for k0 in range(0, D, 128)]
        r = None
        for i in range(NS):
            rw = pl.ds(i * 8, 8)
            hv = _rb(xb[pl.ds(i * 16, 16), cj].astype(F32) - mb) * hi
            h0, h1 = hv[:, :128], hv[:, 128:]
            xh[rw, pl.ds(256 * j, 128)] = _u32(h0)
            xh[rw, pl.ds(256 * j + 128, 128)] = _u32(h1)
            vv[rw, pl.ds(256 * j, 128)] = _u32(h0 + h1)
            vv[rw, pl.ds(256 * j + 128, 128)] = _u32(h0 - h1)
            if i % 8 == 7 or i == NS - 1:
                k0, k1 = (i // 8) * 128, (i + 1) * 16
                yield
                p = _dot(tk["w"][i // 8], _bf(xh[pl.ds(k0 // 2, (k1 - k0) // 2), cj]))
                r = p if r is None else r + p
        for t in range(2):
            r_t = r[:, 128 * t:128 * t + 128]
            tk["rc"] = r_t if (j == 0 and t == 0) else jnp.where(mk[0].row16 == 2 * j + t, r_t, tk["rc"])

    def topk():
        m = mk[0]
        bits = pltpu.bitcast(_rb(tk["rc"] * 2.0), I32)
        mono = (jnp.where(bits < 0, bits ^ 0x7FFF0000, bits) >> 16) + 32768
        key = pltpu.bitcast(0x30000000 + (mono << 11) + (2047 - (m.row16 * 128 + m.lane16)), F32)
        kcol = jnp.zeros((16, 128), I32)
        for j in range(NSEL):
            mx = jnp.max(jnp.max(key, axis=0, keepdims=True), axis=1, keepdims=True)
            mxb = jnp.broadcast_to(mx, (16, 128))
            key = jnp.where(key == mxb, 0.0, key)
            kcol = jnp.where(m.row16 == j, pltpu.bitcast(mxb, I32), kcol)
        kcol = kcol - 0x30000000
        idxcol = jnp.where(m.row16 < NSEL, 2047 - (kcol & 2047), -1)
        hb = ((kcol >> 11) - 32768) << 16
        rsel = pltpu.bitcast(jnp.where(hb < 0, hb ^ 0x7FFF0000, hb), F32)
        rsel = jnp.where(m.row16 < NSEL, rsel, 0.0)
        rs_s[...] = _rb(jax.nn.sigmoid(rsel))
        oh = jnp.concatenate(
            [jnp.where(idxcol == m.lane16 + 128 * t, 1.0, 0.0) for t in range(16)], axis=1).astype(BF16)
        oh_s[...] = pltpu.bitcast(oh, U32)
        hits = jnp.where(m.row16[:8] < NSEL, jnp.left_shift(1, jnp.maximum(idxcol[:8], 0) >> 7), 0)
        for sh in (4, 2, 1):
            hits = hits | pltpu.roll(hits, sh, 0)
        hit_s[0] = hits[0, 0]
        tcol = jnp.maximum(idxcol, 0) >> 7
        tk["tj"] = [jnp.clip(tcol[j, 0], 0, 15) for j in range(NSEL)]
        tk["ol"] = jnp.where((idxcol & 127) == m.lane16, 1.0, 0.0)

    def xsel(j):
        off = pl.multiple_of(tk["tj"][j] * 128, 128)
        lhs = jnp.where(mk[0].row16 == j, tk["ol"], 0.0).astype(BF16)
        v = _dot_nt(lhs, _bf(xh[:, pl.ds(off, 128)]))
        tk["xa"] = v if j == 0 else tk["xa"] + v
        if j == NSEL - 1:
            xs_s[...] = _u32(tk["xa"] * 2.0)

    ffp = [0, 0]
    ffp_max = [0]

    def wpiece(i, p):
        c = 0
        while 2 * p >= sum(FCH[:c + 1]):
            c += 1
        return _bf(wbuf[c][i][:, pl.ds(256 * p - 128 * sum(FCH[:c]), 256)])

    def ffn_gu():
        p = ffp[0]
        ffp[0] += 1
        gu = _dot(tk["xs"], jnp.concatenate([wpiece(0, p), wpiece(1, p)], axis=1))
        g = _rb(gu[:, :256])
        u = _rb(gu[:, 256:])
        sg = _rb(0.5 * jnp.tanh(0.5 * g) + 0.5)
        tk["h", p] = (_rb(g * sg) * u).astype(BF16)

    def ffn_dn():
        p = ffp[1]
        ffp[1] += 1
        y = _dot_nt(tk.pop(("h", p)), wpiece(2, p))
        tk["y"] = y if p == 0 else tk["y"] + y

    def ffn_next():
        if ffp[1] < ffp[0] - 1 or (ffp[1] < ffp[0] and ffp[0] >= ffp_max[0]):
            ffn_dn()
        elif ffp[0] < ffp_max[0]:
            ffn_gu()

    def fin16(i, c0, c1, du):
        r16 = pl.ds(16 * i, 16)
        cs = pl.ds(128 * c0, 128 * (c1 - c0))
        h = _bf(xh[pl.ds(8 * i, 8), cs]).astype(F32)

        def ycol(c):
            if du is None:
                return jnp.concatenate([ysv.pop((2 * i + hh, c)) for hh in range(2)], axis=0)
            o = 8 * ((c // 2) % 2)
            col = pl.ds(256 * (c // 4) + 128 * (c % 2), 128)
            return jnp.concatenate([_bf(yb[pl.ds(16 * i + 8 * hh, 8), col]).astype(F32)[o:o + 8]
                                    for hh in range(2)], axis=0)
        y = jnp.concatenate([ycol(c) for c in range(c0, c1)], axis=1)
        dv = deff[r16, :]
        s = y + h * jnp.concatenate([dv] * (c1 - c0), axis=1)
        zh = h if du is None else h + du
        g = zh * jnp.tanh(zh) + zh
        ob[r16, cs] = (xb[r16, cs].astype(F32) + s * g).astype(BF16)

    def ut_piece(b, k, j0):
        rw = pl.ds(b * (RU // 2), RU // 2)
        rows = pl.ds(dyn(0), RU)
        ur = urs[b % 3]
        js = range(j0, j0 + UTJ)

        def lhs(ref, o):
            return _bf(jnp.concatenate([ref[rw, pl.ds(256 * j + o, 128)] for j in js], axis=0))

        def put(val, col):
            for i, j in enumerate(js):
                ur[rows, pl.ds(640 * j + col, 128)] = val[i * RU:(i + 1) * RU]
        if k == 0:
            v = _dot(lhs(vv, 0), _bf(um[:, 0:256]))
            b2 = _dot(lhs(vv, 128), _bf(um[:, 256:384]))
            a0 = v[:, :128]

            def sel(p, q):
                return jnp.concatenate([jnp.where(mk[0].lo64, p[8 * i:8 * i + 8], q[8 * i:8 * i + 8])
                                        for i in range(a0.shape[0] // 8)], axis=0)
            put(sel(a0, b2), 0)
            put(v[:, 128:], 128)
            put(pltpu.roll(sel(b2, a0), 64, 1), 256)
        else:
            put(_dot(lhs(xh, 128), _bf(um[:, 384:512])), 384)
            put(_dot(lhs(xh, 0), _bf(um[:, 512:640])), 512)

    def mac(g, cls):
        ur = urs[(8 * g // RU) % 3]
        m = mk[0]

        @functools.lru_cache(None)
        def us(j):
            def ld(c):
                return ur[pl.ds((8 * g) % RU, 8), pl.ds(640 * j + c, 128)]
            if cls == 0:
                a, b = ld(0), ld(256)
                return (a, b, a + b)
            t1, t2, t3 = ld(128), ld(384), ld(512)
            return (t1 + t2, t3 - t1, t2 + t3)

        @functools.lru_cache(None)
        def kraw(j):
            o = 512 * j + 256 * (1 - cls)
            ksp, kr = ksps[8 * g // RB], pl.ds((8 * g) % RB, 8)
            return ksp[kr, pl.ds(o, 128)], ksp[kr, pl.ds(o + 128, 128)]

        @functools.lru_cache(None)
        def ks(j):
            sr, si = kraw(j)
            if j > 0:
                pr, pi_ = kraw(j - 1)
                sr, si = (sr + pr, si + pi_) if cls == 0 else (sr - pr, si - pi_)
            return (sr * m.mz if cls == 0 else sr, si - sr, sr + si)

        def cat(p, q):
            return jnp.concatenate([p, q], axis=0)
        outs = []
        prev = None
        for mo in range(NCH):
            acc = None
            for j in range(mo + 1):
                a, b, s = us(j)
                c_, e_, g_ = ks(mo - j)
                t = (c_ * s, a * e_, b * g_)
                acc = t if acc is None else tuple(x + y for x, y in zip(acc, t))
            z = (acc[0] - acc[2], acc[0] + acc[1])
            if mo % 2 == 1:
                za, zb = prev, z
                if cls == 1:
                    outs.append((cat(za[0] + za[1], zb[0] + zb[1]), cat(za[1], zb[1]), cat(za[0], zb[0])))
                else:
                    zr = _u32(cat(za[0], zb[0]))
                    zis = pltpu.roll(_u32(cat(za[1], zb[1])), 64, 1)
                    outs.append((jnp.where(m.lo64, zr, zis), jnp.where(m.lo64, zis, zr)))
            prev = z
        return outs

    zq, wq = {}, {}

    def inv(g, cls):
        zo = zq.pop((g, cls))

        def st(t):
            v = jnp.concatenate([zo[p][t] for p in range(4)], axis=0)
            return _bf(v) if cls == 0 else v.astype(BF16)
        if cls == 0:
            wq[g] = [_dot(st(t), _bf(umt[:, c:c + 128])) for t, c in ((0, 0), (1, 256))]
        else:
            q1, q2, q3 = [_dot(st(t), _bf(umt[:, c:c + 128])) for t, c in ((0, 128), (1, 384), (2, 512))]
            w0, w2 = wq.pop(g)
            p_ = q1 + w2
            y0 = p_ + (q2 + w0)
            y1 = (q3 + w0) - p_
            for p in range(4):
                yb[pl.ds(8 * g, 8), pl.ds(256 * p, 128)] = _u32(y0[16 * p:16 * p + 16])
                yb[pl.ds(8 * g, 8), pl.ds(256 * p + 128, 128)] = _u32(y1[16 * p:16 * p + 16])
                for e in range(2):
                    ysv[(g, 4 * p + 2 * e)] = y0[16 * p + 8 * e:16 * p + 8 * e + 8]
                    ysv[(g, 4 * p + 2 * e + 1)] = y1[16 * p + 8 * e:16 * p + 8 * e + 8]

    def region(fn):
        @pl.when(zs[0] == 0)
        def _():
            mk[0] = _Masks()
            fn()

    for i, _ in enumerate(kgen(0, R1 // 16)):
        if i == 3:
            _ggen(selb, g0b, gm)
    for cp in in_cp[2]:
        cp.wait()
    slotno[0] += 100
    for _ in kgen(R1 // 16, XW):
        pass
    dkb = _col_bcast(dsk)
    for t in range(5):
        n = 128 if t < 4 else 64
        dkc[pl.ds(t * 128, n), :] = dkb[t][:n]
    in_cp[3][0].wait()

    def phase_a2():
        slotno[0] += 100
        kg = kgen(XW, NS)
        next(kg)
        nslot = 0
        for j in range(NCH):
            for _ in ln_chunk(j):
                kt_drain(1)
                nslot += 1
                if nslot % 5 == 0:
                    next(kg)
        topk()
        xq = list(range(NSEL))
        for i, _ in enumerate(kg):
            kt_drain(i % 2)
            if i >= 20 and xq and i % 4 == 0:
                xsel(xq.pop(0))
        while xq:
            xsel(xq.pop(0))
        slotno[0] += 1000
        kt_drain(len(ktq) - NCH)

    region(phase_a2)

    utq = [(b, k, j) for b in range(D // RU) for j in range(0, NCH, UTJ) for k in range(2)]

    def mac_groups(g0, g1):
        for s in range(g0, g1):
            for cls in range(2):
                if s < NG:
                    zq[(s, cls)] = mac(s, cls)
                if 1 <= s < NG + 1:
                    inv(s - 1, cls)
                if utq:
                    ut_piece(*utq.pop(0))
                if cls == 1 and s % 4 == 3:
                    kt_drain(1)
                q = 2 * (s - 3) + cls - 2
                if 0 <= q < 4 * NS:
                    fin16(q // 4, 4 * (q % 4), 4 * (q % 4) + 4, None)
                if cls == 0 and (s - g0) % 2 == 0:
                    ffn_next()

    def phase_b():
        in_mac[0] = True
        ends = [gs for gs, _ in FWAIT[1:]] + [NG + 5]
        for (gs, cc), ge in zip(FWAIT, ends):
            for cp in w_cp[cc]:
                cp.wait()
            ffp_max[0] = sum(FCH[:cc + 1]) // 2
            tk["xs"] = _bf(xs_s[...])
            if gs == 0:
                for _ in range(8):
                    ut_piece(*utq.pop(0))
                for t in range(5):
                    rows = pl.ds(128 * t, 128 if t < 4 else 64)
                    deff[rows, :] = (dkc[rows, :] + k0c[rows, :]) * 2.0
            mac_groups(gs, ge)
        while ffp[1] < ffp_max[0]:
            ffn_next()
        ya_s[...] = tk["y"]

    region(phase_b)

    o_cp = [pltpu.make_async_copy(ob.at[:, pl.ds(128 * t, 128)], out_hbm.at[:, pl.ds(128 * t, 128)], sem_o.at[t])
            for t in range(16)]
    tk["xs"] = _bf(xs_s[...])
    rs = rs_s[...]
    tk["y"] = ya_s[...]
    for cc in range(len(FWAIT), len(FCH)):
        for cp in w_cp[cc]:
            cp.wait()
    hit = hit_s[0]
    for t in range(16):
        @pl.when(((hit >> t) & 1) == 0)
        def _():
            o_cp[t].start(priority=1)
    while ffp[0] < sum(FCH) // 2:
        ffn_gu()
        if ffp[1] < ffp[0] - 1:
            ffn_dn()
    while ffp[1] < ffp[0]:
        ffn_dn()
    upd = (_rb(_rb(tk["y"]) * jnp.concatenate([rs] * 5, axis=1)[:, :D]) * 0.5).astype(BF16)
    upt_s[...] = jnp.concatenate([upd, jnp.zeros((16, 64), BF16)], axis=1).T
    hit = hit_s[0]
    for t in range(16):
        @pl.when(((hit >> t) & 1) == 1)
        def _():
            du = _dot(upt_s[pl.ds(0, D), :], _bf(oh_s[:, pl.ds(128 * t, 128)]))
            for i in range(NS):
                fin16(i, t, t + 1, du[16 * i:16 * i + 16])
            o_cp[t].start(priority=1)
    for cp in o_cp:
        cp.wait()


@jax.jit
def pallas_recurrent_scan__ssm_conv_s4__moe_arch_mod__prompt_kernel(
        A_u, A_A_re, A_A_im, A_B_re, A_B_im, A_C_re, A_C_im, A_log_dt, A_Dskip,
        B_x, B_w_r, B_w_gate, B_w_up, B_w_down):
    scratch = [
        pltpu.SMEM((1,), I32),
        pltpu.VMEM((D, L), BF16),
        pltpu.VMEM((6, D, N), BF16),
        pltpu.VMEM((D,), BF16),
        pltpu.VMEM((D,), BF16),
        pltpu.VMEM((D,), BF16),
        pltpu.VMEM((64, 640), U32),
        pltpu.VMEM((128, 512), U32),
        pltpu.VMEM((336, 512), U32),
        pltpu.VMEM((8, 256), I32),
        pltpu.VMEM((64, 640), U32),
        pltpu.VMEM((D, 128), F32),
        pltpu.VMEM((D, 128), F32),
        pltpu.VMEM((D, 128), F32),
        pltpu.VMEM((D // 2, L), U32),
        pltpu.VMEM((D // 2, L), U32),
        pltpu.VMEM((RU, 5120), F32),
        pltpu.VMEM((RU, 5120), F32),
        pltpu.VMEM((RU, 5120), F32),
        pltpu.VMEM((D, L // 2), U32),
        pltpu.VMEM((D, L), BF16),
        pltpu.VMEM((16, 128), F32),
        pltpu.VMEM((8, L), U32),
        pltpu.VMEM((8, D), U32),
        pltpu.SMEM((1,), I32),
        pltpu.VMEM((D, 128), F32),
        pltpu.VMEM((16, D), F32),
        pltpu.VMEM((640, 16), BF16),
        pltpu.SemaphoreType.DMA((17,)),
        pltpu.SemaphoreType.DMA((3, len(FCH))),
        pltpu.SemaphoreType.DMA((16,)),
    ]
    scratch += [pltpu.VMEM((RB, 4096), F32)] * NB
    scratch += [pltpu.VMEM((D // 2, 128 * n), U32) for n in FCH for _ in range(3)]
    scratch += [pltpu.VMEM((RB, 896), F32)] * NB
    out = pl.pallas_call(
        _kernel,
        out_shape=jax.ShapeDtypeStruct((D, L), BF16),
        in_specs=[pl.BlockSpec(memory_space=pl.ANY)] * 14,
        out_specs=pl.BlockSpec(memory_space=pl.ANY),
        scratch_shapes=scratch,
        compiler_params=pltpu.CompilerParams(vmem_limit_bytes=100 * 2**20, disable_semaphore_checks=True,
                                             disable_bounds_checks=True),
        name="s4_mod",
    )(jnp.transpose(A_u[0]), A_A_re, A_A_im, A_B_re, A_B_im, A_C_re, A_C_im, A_log_dt, A_Dskip,
      B_w_r, B_w_gate, B_w_up, jnp.transpose(B_w_down), jnp.asarray(_SEL))
    return jnp.transpose(out)[None]
```

```python
import functools
import math

import numpy as np
import jax
import jax.numpy as jnp
from jax import lax
import jax.experimental.pallas as pl
import jax.experimental.pallas.tpu as pltpu

F32 = jnp.float32
BF16 = jnp.bfloat16
U32 = jnp.uint32
I32 = jnp.int32

D = 576
L = 2048
N = 128
NSEL = 8
NCH = 8
NS = D // 16
NG = D // 8
RB = 64
NB = D // RB
SPB = RB // 16
RU = 16
UTJ = 4
R1 = 128
XW = 22
FCH = (10, 10, 8, 8)
FWAIT = ((0, 0), (25, 1), (51, 2))

_TILES = {
    "odd": (1, 3, 5, 7),
    "even": (2, 4, 6, 8),
    "t2": (258, 260, 262, 264),
    "t3": (516, 520, 772, 776),
    "t4": (1032, 1288, 1544, 1800),
}
_KT = [(0, 256, 0), (128, 256, 256), (384, 128, 512), (512, 128, 576),
       (640, 128, 704), (768, 128, 800), (768, 128, 768), (768, 128, 736)]


def _rlag(l):
    u = int(np.float32(l).view(np.uint32))
    u = (u + 0x7FFF + ((u >> 16) & 1)) & 0xFFFF0000
    return int(np.uint32(u).view(np.float32))


def _tile_pts(name):
    base = name.rstrip("v")
    p = np.array([_TILES[base][l // 32] + 8 * (l % 32) for l in range(128)])
    if name == "t3v":
        p[127] = 512
    if name == "t4v":
        p[127] = 1024
    return p


def _sel_table():
    lags = np.concatenate([_tile_pts("odd"), _tile_pts("even")])
    sel = np.full((8, 256), -1, np.int32)
    for k, (c, tile) in enumerate([(1, "t2"), (2, "t3v"), (4, "t4v"), (1, "even")]):
        pts = _tile_pts(tile)
        for rho, r in enumerate(lags):
            idx = np.nonzero(pts == _rlag(256 * c + int(r)))[0]
            if len(idx):
                sel[k, rho] = idx[0]
    return sel


_SEL = _sel_table()


def _bf(x):
    return pltpu.bitcast(x, BF16)


def _u32(x):
    return pltpu.bitcast(x.astype(BF16), U32)


def _rb(x):
    return x.astype(BF16).astype(F32)


def _cmul(a, b):
    return (a[0] * b[0] - a[1] * b[1], a[0] * b[1] + a[1] * b[0])


def _csq(a):
    t = a[0] * a[1]
    return (a[0] * a[0] - a[1] * a[1], t + t)


def _sincos(th):
    kf = th * (2.0 / math.pi) + 12582912.0
    ki = pltpu.bitcast(kf, I32)
    k = (ki - 0x4B400000).astype(F32)
    r = th - k * 1.5703125
    r = r - k * 4.837512969970703125e-4
    r = r - k * 7.54978995489188216e-8
    r2 = r * r
    s = r + r * r2 * (-1.6666654611e-1 + r2 * (8.3321608736e-3 + r2 * -1.9515295891e-4))
    c = 1.0 + r2 * (-0.5 + r2 * (4.166664568298827e-2 + r2 * (-1.388731625493765e-3 + r2 * 2.443315711809948e-5)))
    swap = (ki & 1) == 1
    sn = jnp.where(swap, c, s)
    cs = jnp.where(swap, s, c)
    sbit = (ki & 2) << 30
    cbit = ((ki + 1) & 2) << 30
    sn = pltpu.bitcast(pltpu.bitcast(sn, I32) ^ sbit, F32)
    cs = pltpu.bitcast(pltpu.bitcast(cs, I32) ^ cbit, F32)
    return cs, sn


def _dot(a, b):
    return jnp.dot(a, b, preferred_element_type=F32)


def _dot_nt(a, b):
    return lax.dot_general(a, b, (((1,), (1,)), ((), ())), preferred_element_type=F32)


def _col_bcast(vec_ref):
    v = vec_ref[...].astype(F32).reshape(1, D)
    vp = jnp.concatenate([v, jnp.zeros((1, 64), F32)], axis=1)
    return [jnp.broadcast_to(vp[:, t * 128:(t + 1) * 128], (128, 128)).T for t in range(5)]


def _base8(p, dt):
    are, aim, bre, bim, cre, cim = p
    y1 = (dt * are) * math.log2(math.e)
    ph = {1: _sincos(dt * aim)}
    e = 1
    while e < 512:
        ph[2 * e] = _csq(ph[e])
        e *= 2
    pw = {}
    for e in (1, 2, 4, 8, 16, 256, 512):
        mg = jnp.exp2(y1 * float(e)) if e > 1 else jnp.exp2(y1)
        pw[e] = (mg * ph[e][0], mg * ph[e][1])
    w = _cmul((cre, cim), (dt * bre, dt * bim))
    k0 = jnp.sum(w[0], axis=1, keepdims=True)
    w1 = _cmul(w, pw[1])
    w2 = _cmul(w1, pw[1])
    w3 = _cmul(w2, pw[1])
    w258 = _cmul(w2, pw[256])

    def rot(z):
        return (pltpu.roll(z[0], 4, 0), pltpu.roll(z[1], 4, 0))
    rots = {e: rot(pw[e]) for e in (2, 4, 8, 16, 512)}
    return (pw, rots, w1, w2, rot(w3), rot(w258)), k0


def _grp_xy(bs, grp, lo4):
    pw, rots, w1, w2, w3r, w258r = bs

    def sel(lo, hi):
        return (jnp.where(lo4, lo[0], hi[0]), jnp.where(lo4, lo[1], hi[1]))
    if grp == 0:
        dup = {e: sel(pw[e], rots[e]) for e in (2, 4, 16, 512)}
        x0, x2, a8 = sel(w1, w3r), sel(w2, w258r), rots[8]
    else:
        dup = {e: sel(rots[e], pw[e]) for e in (2, 4, 16, 512)}
        x0, x2, a8 = sel(w3r, w1), sel(w258r, w2), pw[8]
    xv = [None] * 10
    xv[0] = x0
    xv[1] = _cmul(x0, dup[4])
    xv[2] = x2
    xv[3] = _cmul(xv[2], dup[2])
    xv[4] = _cmul(xv[3], dup[2])
    xv[5] = _cmul(xv[4], dup[2])
    xv[6] = _cmul(xv[3], dup[512])
    xv[7] = _cmul(xv[5], dup[512])
    xv[8] = _cmul(xv[7], dup[512])
    xv[9] = _cmul(xv[8], dup[512])
    y = (jnp.where(lo4, 1.0, a8[0]), jnp.where(lo4, 0.0, -a8[1]))
    m = dup[16]
    ys = [y]
    for _ in range(15):
        y = (y[0] * m[0] + y[1] * m[1], y[1] * m[0] - y[0] * m[1])
        ys.append(y)

    def mat(vs):
        return jnp.concatenate([jnp.concatenate([v[0] for v in vs], 0),
                                jnp.concatenate([v[1] for v in vs], 0)], 1).astype(BF16)
    return mat(xv), mat(ys)


def _dft_tables(um, umt, g0b):
    sub = lax.broadcasted_iota(I32, (8, 128), 0)
    lane = lax.broadcasted_iota(I32, (8, 128), 1)
    lo = lane < 64

    def e512(m):
        return _sincos((m & 511).astype(F32) * (-2.0 * math.pi / 512.0))

    def chain(base, step, n):
        out = [base]
        for _ in range(n - 1):
            out.append(_cmul(out[-1], step))
        return out

    def row(z, r):
        return tuple(jnp.broadcast_to(c[r:r + 1], (8, 128)) for c in z)

    def put(ref, r0, c0, vs):
        for i in range(0, len(vs), 2):
            ref[pl.ds(r0 + 4 * i, 8), pl.ds(c0, 128)] = _u32(jnp.concatenate([vs[i], vs[i + 1]], axis=0))
    f1 = 4 * lane + 1
    k4 = 4 * (lane & 63)
    alt_r = jnp.where((sub & 1) == 1, 1.0, -1.0)
    alt_l = jnp.where((lane & 1) == 1, 1.0, -1.0)
    b1 = e512(f1 * (sub + 1))
    c1 = chain(b1, row(b1, 7), 16)
    put(um, 0, 128, [z[0] for z in c1])
    put(um, 0, 384, [z[1] - z[0] for z in c1])
    put(um, 0, 512, [z[0] + z[1] for z in c1])
    for col, off, q in ((0, 0, jnp.where(lo, 0, 128)), (256, 2, jnp.where(lo, 128, 0))):
        b = e512((k4 + off) * (sub + 1))
        c = chain(e512((k4 + off) * (sub + 1) + q), row(b, 7), 16)
        vs = [z[0] for z in c]
        if off == 0:
            vs = [jnp.where(lane == 64, alt_r, v) for v in vs]
        put(um, 0, col, vs)
    st = e512(32 * (lane + 1))
    c = chain(e512((4 * sub + 1) * (lane + 1)), st, 16)
    put(umt, 0, 128, [z[0] for z in c])
    put(umt, 0, 384, [z[1] - z[0] for z in c])
    put(umt, 0, 512, [z[0] + z[1] for z in c])
    c = chain(e512(4 * sub * (lane + 1)), st, 8)
    re = [z[0] for z in c]
    im = [z[1] for z in c]
    re[0] = jnp.where(sub == 0, alt_l, re[0])
    im[0] = jnp.where(sub == 0, 1.0, im[0])
    put(umt, 0, 0, re + im)
    c = chain(e512((4 * sub + 2) * (lane + 1)), st, 8)
    put(umt, 0, 256, [z[1] for z in c] + [z[0] for z in c])
    for cls, f in ((0, f1), (1, k4 + jnp.where(lo, 0, 2))):
        b = e512(f * (1 + 8 * sub))
        s1 = row(b, 0)
        s64 = e512(f * 64)
        cur = chain((b[0] * (1.0 / 128), b[1] * (1.0 / 128)), s64, 4)
        for lag in range(1, 9):
            re = [z[0] for z in cur]
            im = [z[1] for z in cur]
            if cls == 1:
                sg = (-1.0) ** lag
                re = [jnp.where(lane == 0, (-sg - 1.0) / 512, v) for v in re]
                im = [jnp.where(lane == 0, (1.0 - sg) / 512, v) for v in im]
            r0 = 64 * ((lag - 1) % 2) + 16 * ((lag - 1) // 2)
            put(g0b, r0, 256 * cls, re)
            put(g0b, r0, 256 * cls + 128, im)
            if lag < 8:
                cur = [_cmul(z, s1) for z in cur]


def _ggen(selb, g0b, gm):
    sel = selb[...]

    def onehot(k, r0, n):
        ri = lax.broadcasted_iota(I32, (n, 256), 0) + r0
        return jnp.where(ri == sel[k:k + 1, :], 1.0, 0.0)
    e = jnp.concatenate([onehot(0, 0, 128), onehot(1, 0, 64), onehot(2, 0, 32),
                         onehot(1, 112, 16), onehot(2, 112, 16), onehot(3, 112, 16)], axis=0).astype(BF16)
    g = _dot(e, _bf(g0b[...]))

    def put(r, v):
        gm[pl.ds((r - 256) // 2, v.shape[0] // 2), :] = _u32(v)

    def zero(r, n):
        gm[pl.ds((r - 256) // 2, n // 2), :] = jnp.zeros((n // 2, 512), U32)
    zero(256, 112)
    put(368, g[256:272])
    put(384, g[0:128])
    put(512, g[128:192])
    zero(576, 48)
    put(624, g[224:240])
    put(640, g[128:192])
    put(704, g[192:224])
    zero(736, 80)
    put(816, g[240:256])
    put(832, g[192:224])
    zero(864, 64)


class _Masks:
    def __init__(self):
        sub = lax.broadcasted_iota(I32, (8, 128), 0)
        lane = lax.broadcasted_iota(I32, (8, 128), 1)
        self.lo4 = sub < 4
        self.gidx = 4 * (lane % 32) + (sub % 4)
        self.lo64 = lane < 64
        self.beven = ((lane // 32) % 2) == 0
        self.last = lane == 127
        self.mz = jnp.where(lane == 0, 0.0, 1.0)
        self.row16 = lax.broadcasted_iota(I32, (16, 128), 0)
        self.lane16 = lax.broadcasted_iota(I32, (16, 128), 1)


def _kernel(x_hbm, are_hbm, aim_hbm, bre_hbm, bim_hbm, cre_hbm, cim_hbm, ldt_hbm, dsk_hbm,
            wr_hbm, wg_hbm, wu_hbm, wd_hbm, sel_hbm, out_hbm,
            zs, xb, prm, ldt, dsk, wr, um, g0b, gm, selb,
            umt, dtc, dkc, k0c, xh, vv, ur0, ur1, ur2, yb, ob, rs_s, oh_s, xs_s, hit_s, deff, ya_s, upt_s,
            sem_in, sem_w, sem_o, *rest):
    ksps = rest[:NB]
    kds = rest[-NB:]
    wbuf = [rest[NB + 3 * c:NB + 3 * c + 3] for c in range(len(FCH))]
    urs = (ur0, ur1, ur2)

    prs = [are_hbm, aim_hbm, bre_hbm, bim_hbm, cre_hbm, cim_hbm]
    order = (1, 0, 2, 3, 4, 5)
    grp0 = [(ldt_hbm, ldt), (sel_hbm, selb)]
    grp1 = [(prs[i].at[pl.ds(0, R1)], prm.at[i, pl.ds(0, R1)]) for i in order]
    grp2 = [(prs[i].at[pl.ds(R1, D - R1)], prm.at[i, pl.ds(R1, D - R1)]) for i in order]
    grp2 += [(dsk_hbm, dsk), (wr_hbm, wr)]
    grp3 = [(x_hbm, xb)]
    in_cp = []
    for grp in (grp0, grp1, grp2, grp3):
        n0 = sum(len(g) for g in in_cp)
        in_cp.append([pltpu.make_async_copy(s, d, sem_in.at[n0 + i]) for i, (s, d) in enumerate(grp)])
        for cp in in_cp[-1]:
            cp.start()
    w_cp = []
    off = 0
    for c, n in enumerate(FCH):
        cs = pl.ds(off * 128, n * 128)
        w_cp.append([pltpu.make_async_copy(h.at[:, cs], wbuf[c][i], sem_w.at[i, c])
                     for i, h in enumerate([wg_hbm, wu_hbm, wd_hbm])])
        for cp in w_cp[-1]:
            cp.start(priority=1)
        off += n

    mk = [_Masks()]
    _dft_tables(um, umt, g0b)

    for cp in in_cp[0]:
        cp.wait()
    zs[0] = lax.broadcasted_iota(I32, (8, 128), 1)[0, 0]
    dtb = _col_bcast(ldt)
    for t in range(5):
        n = 128 if t < 4 else 64
        dtc[pl.ds(t * 128, n), :] = _rb(jnp.exp(dtb[t][:n]))
    for cp in in_cp[1]:
        cp.wait()
    zoff = zs[0] * 8

    def dyn(r):
        return pl.multiple_of(zoff + r, 8)

    in_mac = [False]
    ktq = []
    slotno = [0]
    pend = [None]

    def kt_unit(b, c):
        l0, kk, g0 = _KT[c]
        gw = g0b[...] if c == 0 else gm[pl.ds((g0 - 256) // 2, kk // 2), :]
        raw = _dot(kds[b][:, pl.ds(l0, kk)].astype(BF16), _bf(gw))
        rows = pl.ds(dyn(0), RB) if in_mac[0] else pl.ds(0, RB)
        ksps[b][rows, pl.ds(512 * c, 512)] = raw

    def kt_drain(n):
        for _ in range(n):
            if ktq and ktq[0][0] <= slotno[0]:
                kt_unit(*ktq.pop(0)[1:])

    def extract(st, o4):
        m = mk[0]

        def mix(a, b):
            return jnp.where(m.lo4, a, b), pltpu.roll(jnp.where(m.lo4, b, a), 4, 0)

        def four(gg):
            return jnp.where(m.lo64, jnp.where(m.beven, gg[2], gg[3]), jnp.where(m.beven, gg[4], gg[5]))
        for half in range(2):
            g = [[jnp.take_along_axis(o4[half][grp][8 * v:8 * v + 8], m.gidx, axis=1, mode="promise_in_bounds")
                  for v in range(10)] for grp in range(2)]

            def two(va, vb, m1, m2):
                p, q = mix(jnp.where(m1, g[0][va], g[0][vb]), jnp.where(m1, g[1][va], g[1][vb]))
                return jnp.where(m2, p, q)
            t_odd = two(0, 1, m.lo64, m.beven)
            t_even, t_2 = mix(four(g[0]), four(g[1]))
            t_3 = two(6, 7, m.beven, m.lo64)
            t_4 = two(8, 9, m.lo64, m.beven)
            tl = [t_odd, t_even, t_2, jnp.where(m.last, t_2, t_3), t_3, jnp.where(m.last, t_3, t_4), t_4]
            for t in range(7):
                kds[st // SPB][pl.ds(dyn((st % SPB) * 16 + 8 * half), 8), pl.ds(128 * t, 128)] = tl[t]

    def flush():
        extract(*pend[0])
        if (pend[0][0] + 1) % SPB == 0:
            ktq.extend([(slotno[0] + 4, pend[0][0] // SPB, c) for c in range(NCH)])
        pend[0] = None

    def kgen(s0, s1):
        for st in range(s0, s1):
            o4 = []
            for half in range(2):
                rows = pl.ds(st * 16 + 8 * half, 8)
                ps = [prm[k, pl.ds(st * 16, 16), :].astype(F32)[8 * half:8 * half + 8] for k in range(6)]
                bs, k0 = _base8(ps, dtc[rows, :])
                k0c[rows, :] = jnp.broadcast_to(k0, (8, 128))
                xy = [_grp_xy(bs, grp, mk[0].lo4) for grp in range(2)]
                if half == 0 and pend[0] is not None:
                    flush()
                oo = []
                for grp in range(2):
                    yield
                    slotno[0] += 1
                    oo.append(_dot_nt(*xy[grp]))
                o4.append(oo)
            pend[0] = (st, o4)
        if s1 == NS:
            flush()

    tk = {}
    ysv = {}

    def ln_chunk(j):
        cj = slice(256 * j, 256 * j + 256)
        s1 = s2 = None
        for i in range(NS):
            v16 = xb[pl.ds(i * 16, 16), cj].astype(F32)
            for v in (v16[:8], v16[8:]):
                s1, s2 = (v, v * v) if s1 is None else (s1 + v, s2 + v * v)
        mean = jnp.sum(s1, axis=0, keepdims=True) * (1.0 / D)
        var = jnp.sum(s2, axis=0, keepdims=True) * (1.0 / D) - mean * mean
        var = jnp.maximum(var, 0.0)
        sd = _rb(jnp.sqrt(_rb(_rb(var) + 1e-5)))
        mb = jnp.broadcast_to(_rb(mean), (16, 256))
        hi = jnp.broadcast_to(0.5 / sd, (16, 256))
        if j == 0:
            wrow = wr[...].astype(F32).reshape(1, D)
            tk["w"] = [(jnp.broadcast_to(wrow[:, k0:min(k0 + 128, D)], (16, min(128, D - k0)))
                        + jnp.zeros((16, min(128, D - k0)), F32)).astype(BF16) for k0 in range(0, D, 128)]
        r = None
        for i in range(NS):
            rw = pl.ds(i * 8, 8)
            hv = _rb(xb[pl.ds(i * 16, 16), cj].astype(F32) - mb) * hi
            h0, h1 = hv[:, :128], hv[:, 128:]
            xh[rw, pl.ds(256 * j, 128)] = _u32(h0)
            xh[rw, pl.ds(256 * j + 128, 128)] = _u32(h1)
            vv[rw, pl.ds(256 * j, 128)] = _u32(h0 + h1)
            vv[rw, pl.ds(256 * j + 128, 128)] = _u32(h0 - h1)
            if i % 8 == 7 or i == NS - 1:
                k0, k1 = (i // 8) * 128, (i + 1) * 16
                yield
                p = _dot(tk["w"][i // 8], _bf(xh[pl.ds(k0 // 2, (k1 - k0) // 2), cj]))
                r = p if r is None else r + p
        for t in range(2):
            r_t = r[:, 128 * t:128 * t + 128]
            tk["rc"] = r_t if (j == 0 and t == 0) else jnp.where(mk[0].row16 == 2 * j + t, r_t, tk["rc"])

    def topk():
        m = mk[0]
        bits = pltpu.bitcast(_rb(tk["rc"] * 2.0), I32)
        mono = (jnp.where(bits < 0, bits ^ 0x7FFF0000, bits) >> 16) + 32768
        key = pltpu.bitcast(0x30000000 + (mono << 11) + (2047 - (m.row16 * 128 + m.lane16)), F32)
        kcol = jnp.zeros((16, 128), I32)
        for j in range(NSEL):
            mx = jnp.max(jnp.max(key, axis=0, keepdims=True), axis=1, keepdims=True)
            mxb = jnp.broadcast_to(mx, (16, 128))
            key = jnp.where(key == mxb, 0.0, key)
            kcol = jnp.where(m.row16 == j, pltpu.bitcast(mxb, I32), kcol)
        kcol = kcol - 0x30000000
        idxcol = jnp.where(m.row16 < NSEL, 2047 - (kcol & 2047), -1)
        hb = ((kcol >> 11) - 32768) << 16
        rsel = pltpu.bitcast(jnp.where(hb < 0, hb ^ 0x7FFF0000, hb), F32)
        rsel = jnp.where(m.row16 < NSEL, rsel, 0.0)
        rs_s[...] = _rb(jax.nn.sigmoid(rsel))
        oh = jnp.concatenate(
            [jnp.where(idxcol == m.lane16 + 128 * t, 1.0, 0.0) for t in range(16)], axis=1).astype(BF16)
        oh_s[...] = pltpu.bitcast(oh, U32)
        hits = jnp.where(m.row16[:8] < NSEL, jnp.left_shift(1, jnp.maximum(idxcol[:8], 0) >> 7), 0)
        for sh in (4, 2, 1):
            hits = hits | pltpu.roll(hits, sh, 0)
        hit_s[0] = hits[0, 0]
        tcol = jnp.maximum(idxcol, 0) >> 7
        tk["tj"] = [jnp.clip(tcol[j, 0], 0, 15) for j in range(NSEL)]
        tk["ol"] = jnp.where((idxcol & 127) == m.lane16, 1.0, 0.0)

    def xsel(j):
        off = pl.multiple_of(tk["tj"][j] * 128, 128)
        lhs = jnp.where(mk[0].row16 == j, tk["ol"], 0.0).astype(BF16)
        v = _dot_nt(lhs, _bf(xh[:, pl.ds(off, 128)]))
        tk["xa"] = v if j == 0 else tk["xa"] + v
        if j == NSEL - 1:
            xs_s[...] = _u32(tk["xa"] * 2.0)

    ffp = [0, 0]
    ffp_max = [0]

    def wpiece(i, p):
        c = 0
        while 2 * p >= sum(FCH[:c + 1]):
            c += 1
        return wbuf[c][i][:, pl.ds(256 * p - 128 * sum(FCH[:c]), 256)]

    def ffn_gu():
        p = ffp[0]
        ffp[0] += 1
        gu = _dot(tk["xs"], jnp.concatenate([wpiece(0, p), wpiece(1, p)], axis=1))
        g = _rb(gu[:, :256])
        u = _rb(gu[:, 256:])
        sg = _rb(0.5 * jnp.tanh(0.5 * g) + 0.5)
        tk["h", p] = (_rb(g * sg) * u).astype(BF16)

    def ffn_dn():
        p = ffp[1]
        ffp[1] += 1
        y = _dot_nt(tk.pop(("h", p)), wpiece(2, p))
        tk["y"] = y if p == 0 else tk["y"] + y

    def ffn_next():
        if ffp[1] < ffp[0] - 1 or (ffp[1] < ffp[0] and ffp[0] >= ffp_max[0]):
            ffn_dn()
        elif ffp[0] < ffp_max[0]:
            ffn_gu()

    def fin16(i, c0, c1, du):
        r16 = pl.ds(16 * i, 16)
        cs = pl.ds(128 * c0, 128 * (c1 - c0))
        h = _bf(xh[pl.ds(8 * i, 8), cs]).astype(F32)

        def ycol(c):
            if du is None:
                return jnp.concatenate([ysv.pop((2 * i + hh, c)) for hh in range(2)], axis=0)
            o = 8 * ((c // 2) % 2)
            col = pl.ds(256 * (c // 4) + 128 * (c % 2), 128)
            return jnp.concatenate([_bf(yb[pl.ds(16 * i + 8 * hh, 8), col]).astype(F32)[o:o + 8]
                                    for hh in range(2)], axis=0)
        y = jnp.concatenate([ycol(c) for c in range(c0, c1)], axis=1)
        dv = deff[r16, :]
        s = y + h * jnp.concatenate([dv] * (c1 - c0), axis=1)
        zh = h if du is None else h + du
        g = zh * jnp.tanh(zh) + zh
        ob[r16, cs] = (xb[r16, cs].astype(F32) + s * g).astype(BF16)

    def ut_piece(b, k, j0):
        rw = pl.ds(b * (RU // 2), RU // 2)
        rows = pl.ds(dyn(0), RU)
        ur = urs[b % 3]
        js = range(j0, j0 + UTJ)

        def lhs(ref, o):
            return _bf(jnp.concatenate([ref[rw, pl.ds(256 * j + o, 128)] for j in js], axis=0))

        def put(val, col):
            for i, j in enumerate(js):
                ur[rows, pl.ds(640 * j + col, 128)] = val[i * RU:(i + 1) * RU]
        if k == 0:
            v = _dot(lhs(vv, 0), _bf(um[:, 0:256]))
            b2 = _dot(lhs(vv, 128), _bf(um[:, 256:384]))
            a0 = v[:, :128]

            def sel(p, q):
                return jnp.concatenate([jnp.where(mk[0].lo64, p[8 * i:8 * i + 8], q[8 * i:8 * i + 8])
                                        for i in range(a0.shape[0] // 8)], axis=0)
            put(sel(a0, b2), 0)
            put(v[:, 128:], 128)
            put(pltpu.roll(sel(b2, a0), 64, 1), 256)
        else:
            put(_dot(lhs(xh, 128), _bf(um[:, 384:512])), 384)
            put(_dot(lhs(xh, 0), _bf(um[:, 512:640])), 512)

    def mac(g, cls):
        ur = urs[(8 * g // RU) % 3]
        m = mk[0]

        @functools.lru_cache(None)
        def us(j):
            def ld(c):
                return ur[pl.ds((8 * g) % RU, 8), pl.ds(640 * j + c, 128)]
            if cls == 0:
                a, b = ld(0), ld(256)
                return (a, b, a + b)
            t1, t2, t3 = ld(128), ld(384), ld(512)
            return (t1 + t2, t3 - t1, t2 + t3)

        @functools.lru_cache(None)
        def kraw(j):
            o = 512 * j + 256 * (1 - cls)
            ksp, kr = ksps[8 * g // RB], pl.ds((8 * g) % RB, 8)
            return ksp[kr, pl.ds(o, 128)], ksp[kr, pl.ds(o + 128, 128)]

        @functools.lru_cache(None)
        def ks(j):
            sr, si = kraw(j)
            if j > 0:
                pr, pi_ = kraw(j - 1)
                sr, si = (sr + pr, si + pi_) if cls == 0 else (sr - pr, si - pi_)
            return (sr * m.mz if cls == 0 else sr, si - sr, sr + si)

        def cat(p, q):
            return jnp.concatenate([p, q], axis=0)
        outs = []
        prev = None
        for mo in range(NCH):
            acc = None
            for j in range(mo + 1):
                a, b, s = us(j)
                c_, e_, g_ = ks(mo - j)
                t = (c_ * s, a * e_, b * g_)
                acc = t if acc is None else tuple(x + y for x, y in zip(acc, t))
            z = (acc[0] - acc[2], acc[0] + acc[1])
            if mo % 2 == 1:
                za, zb = prev, z
                if cls == 1:
                    outs.append((cat(za[0] + za[1], zb[0] + zb[1]), cat(za[1], zb[1]), cat(za[0], zb[0])))
                else:
                    zr = _u32(cat(za[0], zb[0]))
                    zis = pltpu.roll(_u32(cat(za[1], zb[1])), 64, 1)
                    outs.append((jnp.where(m.lo64, zr, zis), jnp.where(m.lo64, zis, zr)))
            prev = z
        return outs

    zq, wq = {}, {}

    def inv(g, cls):
        zo = zq.pop((g, cls))

        def st(t):
            v = jnp.concatenate([zo[p][t] for p in range(4)], axis=0)
            return _bf(v) if cls == 0 else v.astype(BF16)
        if cls == 0:
            wq[g] = [_dot(st(t), _bf(umt[:, c:c + 128])) for t, c in ((0, 0), (1, 256))]
        else:
            q1, q2, q3 = [_dot(st(t), _bf(umt[:, c:c + 128])) for t, c in ((0, 128), (1, 384), (2, 512))]
            w0, w2 = wq.pop(g)
            p_ = q1 + w2
            y0 = p_ + (q2 + w0)
            y1 = (q3 + w0) - p_
            for p in range(4):
                yb[pl.ds(8 * g, 8), pl.ds(256 * p, 128)] = _u32(y0[16 * p:16 * p + 16])
                yb[pl.ds(8 * g, 8), pl.ds(256 * p + 128, 128)] = _u32(y1[16 * p:16 * p + 16])
                for e in range(2):
                    ysv[(g, 4 * p + 2 * e)] = y0[16 * p + 8 * e:16 * p + 8 * e + 8]
                    ysv[(g, 4 * p + 2 * e + 1)] = y1[16 * p + 8 * e:16 * p + 8 * e + 8]

    def region(fn):
        @pl.when(zs[0] == 0)
        def _():
            mk[0] = _Masks()
            fn()

    for i, _ in enumerate(kgen(0, R1 // 16)):
        if i == 3:
            _ggen(selb, g0b, gm)
    for cp in in_cp[2]:
        cp.wait()
    slotno[0] += 100
    for _ in kgen(R1 // 16, XW):
        pass
    dkb = _col_bcast(dsk)
    for t in range(5):
        n = 128 if t < 4 else 64
        dkc[pl.ds(t * 128, n), :] = dkb[t][:n]
    in_cp[3][0].wait()

    def phase_a2():
        slotno[0] += 100
        kg = kgen(XW, NS)
        next(kg)
        nslot = 0
        for j in range(NCH):
            for _ in ln_chunk(j):
                kt_drain(1)
                nslot += 1
                if nslot % 5 == 0:
                    next(kg)
        topk()
        xq = list(range(NSEL))
        for i, _ in enumerate(kg):
            kt_drain(i % 2)
            if i >= 20 and xq and i % 4 == 0:
                xsel(xq.pop(0))
        while xq:
            xsel(xq.pop(0))
        slotno[0] += 1000
        kt_drain(len(ktq) - NCH)

    region(phase_a2)

    utq = [(b, k, j) for b in range(D // RU) for j in range(0, NCH, UTJ) for k in range(2)]

    def mac_groups(g0, g1):
        for s in range(g0, g1):
            for cls in range(2):
                if s < NG:
                    zq[(s, cls)] = mac(s, cls)
                if 1 <= s < NG + 1:
                    inv(s - 1, cls)
                if utq:
                    ut_piece(*utq.pop(0))
                if cls == 1 and s % 4 == 3:
                    kt_drain(1)
                q = 2 * (s - 3) + cls - 2
                if 0 <= q < 4 * NS:
                    fin16(q // 4, 4 * (q % 4), 4 * (q % 4) + 4, None)
                if cls == 0 and (s - g0) % 2 == 0:
                    ffn_next()

    def phase_b():
        in_mac[0] = True
        ends = [gs for gs, _ in FWAIT[1:]] + [NG + 5]
        for (gs, cc), ge in zip(FWAIT, ends):
            for cp in w_cp[cc]:
                cp.wait()
            ffp_max[0] = sum(FCH[:cc + 1]) // 2
            tk["xs"] = _bf(xs_s[...])
            if gs == 0:
                for _ in range(8):
                    ut_piece(*utq.pop(0))
                for t in range(5):
                    rows = pl.ds(128 * t, 128 if t < 4 else 64)
                    deff[rows, :] = (dkc[rows, :] + k0c[rows, :]) * 2.0
            mac_groups(gs, ge)
        while ffp[1] < ffp_max[0]:
            ffn_next()
        ya_s[...] = tk["y"]

    region(phase_b)

    o_cp = [pltpu.make_async_copy(ob.at[:, pl.ds(128 * t, 128)], out_hbm.at[:, pl.ds(128 * t, 128)], sem_o.at[t])
            for t in range(16)]
    tk["xs"] = _bf(xs_s[...])
    rs = rs_s[...]
    tk["y"] = ya_s[...]
    for cc in range(len(FWAIT), len(FCH)):
        for cp in w_cp[cc]:
            cp.wait()
    hit = hit_s[0]
    for t in range(16):
        @pl.when(((hit >> t) & 1) == 0)
        def _():
            o_cp[t].start(priority=1)
    while ffp[0] < sum(FCH) // 2:
        ffn_gu()
        if ffp[1] < ffp[0] - 1:
            ffn_dn()
    while ffp[1] < ffp[0]:
        ffn_dn()
    upd = (_rb(_rb(tk["y"]) * jnp.concatenate([rs] * 5, axis=1)[:, :D]) * 0.5).astype(BF16)
    upt_s[...] = jnp.concatenate([upd, jnp.zeros((16, 64), BF16)], axis=1).T
    hit = hit_s[0]
    for t in range(16):
        @pl.when(((hit >> t) & 1) == 1)
        def _():
            du = _dot(upt_s[pl.ds(0, D), :], _bf(oh_s[:, pl.ds(128 * t, 128)]))
            for i in range(NS):
                fin16(i, t, t + 1, du[16 * i:16 * i + 16])
            o_cp[t].start(priority=1)
    for cp in o_cp:
        cp.wait()


@jax.jit
def pallas_recurrent_scan__ssm_conv_s4__moe_arch_mod__prompt_kernel(
        A_u, A_A_re, A_A_im, A_B_re, A_B_im, A_C_re, A_C_im, A_log_dt, A_Dskip,
        B_x, B_w_r, B_w_gate, B_w_up, B_w_down):
    scratch = [
        pltpu.SMEM((1,), I32),
        pltpu.VMEM((D, L), BF16),
        pltpu.VMEM((6, D, N), BF16),
        pltpu.VMEM((D,), BF16),
        pltpu.VMEM((D,), BF16),
        pltpu.VMEM((D,), BF16),
        pltpu.VMEM((64, 640), U32),
        pltpu.VMEM((128, 512), U32),
        pltpu.VMEM((336, 512), U32),
        pltpu.VMEM((8, 256), I32),
        pltpu.VMEM((64, 640), U32),
        pltpu.VMEM((D, 128), F32),
        pltpu.VMEM((D, 128), F32),
        pltpu.VMEM((D, 128), F32),
        pltpu.VMEM((D // 2, L), U32),
        pltpu.VMEM((D // 2, L), U32),
        pltpu.VMEM((RU, 5120), F32),
        pltpu.VMEM((RU, 5120), F32),
        pltpu.VMEM((RU, 5120), F32),
        pltpu.VMEM((D, L // 2), U32),
        pltpu.VMEM((D, L), BF16),
        pltpu.VMEM((16, 128), F32),
        pltpu.VMEM((8, L), U32),
        pltpu.VMEM((8, D), U32),
        pltpu.SMEM((1,), I32),
        pltpu.VMEM((D, 128), F32),
        pltpu.VMEM((16, D), F32),
        pltpu.VMEM((640, 16), BF16),
        pltpu.SemaphoreType.DMA((17,)),
        pltpu.SemaphoreType.DMA((3, len(FCH))),
        pltpu.SemaphoreType.DMA((16,)),
    ]
    scratch += [pltpu.VMEM((RB, 4096), F32)] * NB
    scratch += [pltpu.VMEM((D, 128 * n), BF16) for n in FCH for _ in range(3)]
    scratch += [pltpu.VMEM((RB, 896), F32)] * NB
    out = pl.pallas_call(
        _kernel,
        out_shape=jax.ShapeDtypeStruct((D, L), BF16),
        in_specs=[pl.BlockSpec(memory_space=pl.ANY)] * 14,
        out_specs=pl.BlockSpec(memory_space=pl.ANY),
        scratch_shapes=scratch,
        compiler_params=pltpu.CompilerParams(vmem_limit_bytes=100 * 2**20, disable_semaphore_checks=True,
                                             disable_bounds_checks=True),
        name="s4_mod",
    )(jnp.transpose(A_u[0]), A_A_re, A_A_im, A_B_re, A_B_im, A_C_re, A_C_im, A_log_dt, A_Dskip,
      B_w_r, B_w_gate, B_w_up, jnp.transpose(B_w_down), jnp.asarray(_SEL))
    return jnp.transpose(out)[None]
```

```python
import functools
import math

import numpy as np
import jax
import jax.numpy as jnp
from jax import lax
import jax.experimental.pallas as pl
import jax.experimental.pallas.tpu as pltpu

F32 = jnp.float32
BF16 = jnp.bfloat16
U32 = jnp.uint32
I32 = jnp.int32

D = 576
L = 2048
N = 128
NSEL = 8
NCH = 8
NS = D // 16
NG = D // 8
RB = 64
NB = D // RB
SPB = RB // 16
RU = 16
UTJ = 4
R1 = 128
XW = 22
FCH = (10, 10, 8, 8)
FWAIT = ((0, 0), (25, 1), (51, 2))

_TILES = {
    "odd": (1, 3, 5, 7),
    "even": (2, 4, 6, 8),
    "t2": (258, 260, 262, 264),
    "t3": (516, 520, 772, 776),
    "t4": (1032, 1288, 1544, 1800),
}
_KT = [(0, 256, 0), (128, 256, 256), (384, 128, 512), (512, 128, 576),
       (640, 128, 704), (768, 128, 800), (768, 128, 768), (768, 128, 736)]


def _rlag(l):
    u = int(np.float32(l).view(np.uint32))
    u = (u + 0x7FFF + ((u >> 16) & 1)) & 0xFFFF0000
    return int(np.uint32(u).view(np.float32))


def _tile_pts(name):
    base = name.rstrip("v")
    p = np.array([_TILES[base][l // 32] + 8 * (l % 32) for l in range(128)])
    if name == "t3v":
        p[127] = 512
    if name == "t4v":
        p[127] = 1024
    return p


def _sel_table():
    lags = np.concatenate([_tile_pts("odd"), _tile_pts("even")])
    sel = np.full((8, 256), -1, np.int32)
    for k, (c, tile) in enumerate([(1, "t2"), (2, "t3v"), (4, "t4v"), (1, "even")]):
        pts = _tile_pts(tile)
        for rho, r in enumerate(lags):
            idx = np.nonzero(pts == _rlag(256 * c + int(r)))[0]
            if len(idx):
                sel[k, rho] = idx[0]
    return sel


_SEL = _sel_table()


def _bf(x):
    return pltpu.bitcast(x, BF16)


def _u32(x):
    return pltpu.bitcast(x.astype(BF16), U32)


def _rb(x):
    return x.astype(BF16).astype(F32)


def _cmul(a, b):
    return (a[0] * b[0] - a[1] * b[1], a[0] * b[1] + a[1] * b[0])


def _csq(a):
    t = a[0] * a[1]
    return (a[0] * a[0] - a[1] * a[1], t + t)


def _sincos(th):
    kf = th * (2.0 / math.pi) + 12582912.0
    ki = pltpu.bitcast(kf, I32)
    k = (ki - 0x4B400000).astype(F32)
    r = th - k * 1.5703125
    r = r - k * 4.837512969970703125e-4
    r = r - k * 7.54978995489188216e-8
    r2 = r * r
    s = r + r * r2 * (-1.6666654611e-1 + r2 * (8.3321608736e-3 + r2 * -1.9515295891e-4))
    c = 1.0 + r2 * (-0.5 + r2 * (4.166664568298827e-2 + r2 * (-1.388731625493765e-3 + r2 * 2.443315711809948e-5)))
    swap = (ki & 1) == 1
    sn = jnp.where(swap, c, s)
    cs = jnp.where(swap, s, c)
    sbit = (ki & 2) << 30
    cbit = ((ki + 1) & 2) << 30
    sn = pltpu.bitcast(pltpu.bitcast(sn, I32) ^ sbit, F32)
    cs = pltpu.bitcast(pltpu.bitcast(cs, I32) ^ cbit, F32)
    return cs, sn


def _dot(a, b):
    return jnp.dot(a, b, preferred_element_type=F32)


def _dot_nt(a, b):
    return lax.dot_general(a, b, (((1,), (1,)), ((), ())), preferred_element_type=F32)


def _col_bcast(vec_ref):
    v = vec_ref[...].astype(F32).reshape(1, D)
    vp = jnp.concatenate([v, jnp.zeros((1, 64), F32)], axis=1)
    return [jnp.broadcast_to(vp[:, t * 128:(t + 1) * 128], (128, 128)).T for t in range(5)]


def _base16(p, dt):
    are, aim, bre, bim, cre, cim = p
    y1 = (dt * are) * math.log2(math.e)
    ph = {1: _sincos(dt * aim)}
    e = 1
    while e < 512:
        ph[2 * e] = _csq(ph[e])
        e *= 2
    pw = {}
    for e in (1, 2, 4, 8, 16, 256, 512):
        mg = jnp.exp2(y1 * float(e)) if e > 1 else jnp.exp2(y1)
        pw[e] = (mg * ph[e][0], mg * ph[e][1])
    w = _cmul((cre, cim), (dt * bre, dt * bim))
    k0 = jnp.sum(w[0], axis=1, keepdims=True)
    w1 = _cmul(w, pw[1])
    w2 = _cmul(w1, pw[1])
    w3 = _cmul(w2, pw[1])
    w258 = _cmul(w2, pw[256])

    def rot(z):
        return tuple(jnp.concatenate([pltpu.roll(c[:8], 4, 0), pltpu.roll(c[8:], 4, 0)], axis=0) for c in z)
    rots = {e: rot(pw[e]) for e in (2, 4, 8, 16, 512)}
    return (pw, rots, w1, w2, rot(w3), rot(w258)), k0


def _vandermonde(bs, lo4):
    pw, rots, w1, w2, w3r, w258r = bs

    def sel(a, b):
        return tuple(jnp.concatenate([jnp.where(lo4, a[c], b[c]), jnp.where(lo4, b[c], a[c])], axis=0)
                     for c in range(2))
    dup = {e: sel(pw[e], rots[e]) for e in (2, 4, 16, 512)}
    xv = [None] * 10
    xv[0] = sel(w1, w3r)
    xv[1] = _cmul(xv[0], dup[4])
    xv[2] = sel(w2, w258r)
    xv[3] = _cmul(xv[2], dup[2])
    xv[4] = _cmul(xv[3], dup[2])
    xv[5] = _cmul(xv[4], dup[2])
    xv[6] = _cmul(xv[3], dup[512])
    xv[7] = _cmul(xv[5], dup[512])
    xv[8] = _cmul(xv[7], dup[512])
    xv[9] = _cmul(xv[8], dup[512])
    y = (jnp.concatenate([jnp.where(lo4, 1.0, rots[8][0]), jnp.where(lo4, 1.0, pw[8][0])], axis=0),
         jnp.concatenate([jnp.where(lo4, 0.0, -rots[8][1]), jnp.where(lo4, 0.0, -pw[8][1])], axis=0))
    m = dup[16]
    ys = [y]
    for _ in range(15):
        y = (y[0] * m[0] + y[1] * m[1], y[1] * m[0] - y[0] * m[1])
        ys.append(y)
    xs = [jnp.concatenate(v, axis=1) for v in xv]
    ys = [jnp.concatenate(v, axis=1) for v in ys]

    def mat(vs, r):
        return jnp.concatenate([v[r:r + 8] for v in vs], axis=0).astype(BF16)
    return [[(mat(xs, 16 * grp + 8 * half), mat(ys, 16 * grp + 8 * half)) for grp in range(2)]
            for half in range(2)]


def _dft_tables(um, umt, g0b):
    sub = lax.broadcasted_iota(I32, (8, 128), 0)
    lane = lax.broadcasted_iota(I32, (8, 128), 1)
    lo = lane < 64

    def e512(m):
        return _sincos((m & 511).astype(F32) * (-2.0 * math.pi / 512.0))

    def chain(base, step, n):
        out = [base]
        for _ in range(n - 1):
            out.append(_cmul(out[-1], step))
        return out

    def row(z, r):
        return tuple(jnp.broadcast_to(c[r:r + 1], (8, 128)) for c in z)

    def put(ref, r0, c0, vs):
        for i in range(0, len(vs), 2):
            ref[pl.ds(r0 + 4 * i, 8), pl.ds(c0, 128)] = _u32(jnp.concatenate([vs[i], vs[i + 1]], axis=0))
    f1 = 4 * lane + 1
    k4 = 4 * (lane & 63)
    alt_r = jnp.where((sub & 1) == 1, 1.0, -1.0)
    alt_l = jnp.where((lane & 1) == 1, 1.0, -1.0)
    b1 = e512(f1 * (sub + 1))
    c1 = chain(b1, row(b1, 7), 16)
    put(um, 0, 128, [z[0] for z in c1])
    put(um, 0, 384, [z[1] - z[0] for z in c1])
    put(um, 0, 512, [z[0] + z[1] for z in c1])
    for col, off, q in ((0, 0, jnp.where(lo, 0, 128)), (256, 2, jnp.where(lo, 128, 0))):
        b = e512((k4 + off) * (sub + 1))
        c = chain(e512((k4 + off) * (sub + 1) + q), row(b, 7), 16)
        vs = [z[0] for z in c]
        if off == 0:
            vs = [jnp.where(lane == 64, alt_r, v) for v in vs]
        put(um, 0, col, vs)
    st = e512(32 * (lane + 1))
    c = chain(e512((4 * sub + 1) * (lane + 1)), st, 16)
    put(umt, 0, 128, [z[0] for z in c])
    put(umt, 0, 384, [z[1] - z[0] for z in c])
    put(umt, 0, 512, [z[0] + z[1] for z in c])
    c = chain(e512(4 * sub * (lane + 1)), st, 8)
    re = [z[0] for z in c]
    im = [z[1] for z in c]
    re[0] = jnp.where(sub == 0, alt_l, re[0])
    im[0] = jnp.where(sub == 0, 1.0, im[0])
    put(umt, 0, 0, re + im)
    c = chain(e512((4 * sub + 2) * (lane + 1)), st, 8)
    put(umt, 0, 256, [z[1] for z in c] + [z[0] for z in c])
    for cls, f in ((0, f1), (1, k4 + jnp.where(lo, 0, 2))):
        b = e512(f * (1 + 8 * sub))
        s1 = row(b, 0)
        s64 = e512(f * 64)
        cur = chain((b[0] * (1.0 / 128), b[1] * (1.0 / 128)), s64, 4)
        for lag in range(1, 9):
            re = [z[0] for z in cur]
            im = [z[1] for z in cur]
            if cls == 1:
                sg = (-1.0) ** lag
                re = [jnp.where(lane == 0, (-sg - 1.0) / 512, v) for v in re]
                im = [jnp.where(lane == 0, (1.0 - sg) / 512, v) for v in im]
            r0 = 64 * ((lag - 1) % 2) + 16 * ((lag - 1) // 2)
            put(g0b, r0, 256 * cls, re)
            put(g0b, r0, 256 * cls + 128, im)
            if lag < 8:
                cur = [_cmul(z, s1) for z in cur]


def _ggen(selb, g0b, gm):
    sel = selb[...]

    def onehot(k, r0, n):
        ri = lax.broadcasted_iota(I32, (n, 256), 0) + r0
        return jnp.where(ri == sel[k:k + 1, :], 1.0, 0.0)
    e = jnp.concatenate([onehot(0, 0, 128), onehot(1, 0, 64), onehot(2, 0, 32),
                         onehot(1, 112, 16), onehot(2, 112, 16), onehot(3, 112, 16)], axis=0).astype(BF16)
    g = _dot(e, _bf(g0b[...]))

    def put(r, v):
        gm[pl.ds((r - 256) // 2, v.shape[0] // 2), :] = _u32(v)

    def zero(r, n):
        gm[pl.ds((r - 256) // 2, n // 2), :] = jnp.zeros((n // 2, 512), U32)
    zero(256, 112)
    put(368, g[256:272])
    put(384, g[0:128])
    put(512, g[128:192])
    zero(576, 48)
    put(624, g[224:240])
    put(640, g[128:192])
    put(704, g[192:224])
    zero(736, 80)
    put(816, g[240:256])
    put(832, g[192:224])
    zero(864, 64)


class _Masks:
    def __init__(self):
        sub = lax.broadcasted_iota(I32, (8, 128), 0)
        lane = lax.broadcasted_iota(I32, (8, 128), 1)
        self.lo4 = sub < 4
        self.gidx = jnp.concatenate([4 * (lane % 32) + (sub % 4)] * 10, axis=0)
        self.lo64u = jnp.concatenate([lane] * (UTJ * RU // 8), axis=0) < 64
        self.lo64 = lane < 64
        self.beven = ((lane // 32) % 2) == 0
        self.last = lane == 127
        self.mz = jnp.where(lane == 0, 0.0, 1.0)
        self.row16 = lax.broadcasted_iota(I32, (16, 128), 0)
        self.lo4x2 = (self.row16 & 7) < 4
        self.lane16 = lax.broadcasted_iota(I32, (16, 128), 1)


def _kernel(x_hbm, are_hbm, aim_hbm, bre_hbm, bim_hbm, cre_hbm, cim_hbm, ldt_hbm, dsk_hbm,
            wr_hbm, wg_hbm, wu_hbm, wd_hbm, sel_hbm, out_hbm,
            zs, xb, prm, ldt, dsk, wr, um, g0b, gm, selb,
            umt, dtc, dkc, k0c, xh, vv, ur0, ur1, ur2, yb, ob, rs_s, oh_s, xs_s, hit_s, deff, ya_s, upt_s,
            sem_in, sem_w, sem_o, *rest):
    ksps = rest[:NB]
    kds = rest[-NB:]
    wbuf = [rest[NB + 3 * c:NB + 3 * c + 3] for c in range(len(FCH))]
    urs = (ur0, ur1, ur2)

    prs = [are_hbm, aim_hbm, bre_hbm, bim_hbm, cre_hbm, cim_hbm]
    order = (1, 0, 2, 3, 4, 5)
    grp0 = [(ldt_hbm, ldt), (sel_hbm, selb)]
    grp1 = [(prs[i].at[pl.ds(0, R1)], prm.at[i, pl.ds(0, R1)]) for i in order]
    grp2 = [(prs[i].at[pl.ds(R1, D - R1)], prm.at[i, pl.ds(R1, D - R1)]) for i in order]
    grp2 += [(dsk_hbm, dsk), (wr_hbm, wr)]
    grp3 = [(x_hbm, xb)]
    in_cp = []
    for grp in (grp0, grp1, grp2, grp3):
        n0 = sum(len(g) for g in in_cp)
        in_cp.append([pltpu.make_async_copy(s, d, sem_in.at[n0 + i]) for i, (s, d) in enumerate(grp)])
        for cp in in_cp[-1]:
            cp.start()
    w_cp = []
    off = 0
    for c, n in enumerate(FCH):
        cs = pl.ds(off * 128, n * 128)
        w_cp.append([pltpu.make_async_copy(h.at[:, cs], wbuf[c][i], sem_w.at[i, c])
                     for i, h in enumerate([wg_hbm, wu_hbm, wd_hbm])])
        for cp in w_cp[-1]:
            cp.start(priority=1)
        off += n

    mk = [_Masks()]
    _dft_tables(um, umt, g0b)

    for cp in in_cp[0]:
        cp.wait()
    zs[0] = lax.broadcasted_iota(I32, (8, 128), 1)[0, 0]
    dtb = _col_bcast(ldt)
    for t in range(5):
        n = 128 if t < 4 else 64
        dtc[pl.ds(t * 128, n), :] = _rb(jnp.exp(dtb[t][:n]))
    for cp in in_cp[1]:
        cp.wait()
    zoff = zs[0] * 8

    def dyn(r):
        return pl.multiple_of(zoff + r, 8)

    in_mac = [False]
    ktq = []
    slotno = [0]
    pend = [None]

    def kt_unit(b, c):
        l0, kk, g0 = _KT[c]
        gw = g0b[...] if c == 0 else gm[pl.ds((g0 - 256) // 2, kk // 2), :]
        raw = _dot(kds[b][:, pl.ds(l0, kk)].astype(BF16), _bf(gw))
        rows = pl.ds(dyn(0), RB) if in_mac[0] else pl.ds(0, RB)
        ksps[b][rows, pl.ds(512 * c, 512)] = raw

    def kt_drain(n):
        for _ in range(n):
            if ktq and ktq[0][0] <= slotno[0]:
                kt_unit(*ktq.pop(0)[1:])

    def extract(st, o4):
        m = mk[0]

        def mix(a, b):
            return jnp.where(m.lo4, a, b), pltpu.roll(jnp.where(m.lo4, b, a), 4, 0)

        def four(gg):
            return jnp.where(m.lo64, jnp.where(m.beven, gg[2], gg[3]), jnp.where(m.beven, gg[4], gg[5]))
        for half in range(2):
            g = [jnp.take_along_axis(o4[half][grp], m.gidx, axis=1, mode="promise_in_bounds") for grp in range(2)]
            g = [[gg[8 * v:8 * v + 8] for v in range(10)] for gg in g]

            def two(va, vb, m1, m2):
                p, q = mix(jnp.where(m1, g[0][va], g[0][vb]), jnp.where(m1, g[1][va], g[1][vb]))
                return jnp.where(m2, p, q)
            t_odd = two(0, 1, m.lo64, m.beven)
            t_even, t_2 = mix(four(g[0]), four(g[1]))
            t_3 = two(6, 7, m.beven, m.lo64)
            t_4 = two(8, 9, m.lo64, m.beven)
            tl = [t_odd, t_even, t_2, jnp.where(m.last, t_2, t_3), t_3, jnp.where(m.last, t_3, t_4), t_4]
            for t in range(7):
                kds[st // SPB][pl.ds(dyn((st % SPB) * 16 + 8 * half), 8), pl.ds(128 * t, 128)] = tl[t]

    def flush():
        extract(*pend[0])
        if (pend[0][0] + 1) % SPB == 0:
            ktq.extend([(slotno[0] + 4, pend[0][0] // SPB, c) for c in range(NCH)])
        pend[0] = None

    def kgen(s0, s1):
        for st in range(s0, s1):
            rows = pl.ds(st * 16, 16)
            bs, k0 = _base16([prm[k, rows, :].astype(F32) for k in range(6)], dtc[rows, :])
            k0c[rows, :] = jnp.broadcast_to(k0, (16, 128))
            xy = _vandermonde(bs, mk[0].lo4x2)
            if pend[0] is not None:
                flush()
            o4 = []
            for half in range(2):
                oo = []
                for grp in range(2):
                    yield
                    slotno[0] += 1
                    oo.append(_dot_nt(*xy[half][grp]))
                o4.append(oo)
            pend[0] = (st, o4)
        if s1 == NS:
            flush()

    tk = {}
    ysv = {}

    def ln_chunk(j):
        cj = slice(256 * j, 256 * j + 256)
        s1 = s2 = None
        for i in range(NS):
            v16 = xb[pl.ds(i * 16, 16), cj].astype(F32)
            for v in (v16[:8], v16[8:]):
                s1, s2 = (v, v * v) if s1 is None else (s1 + v, s2 + v * v)
        mean = jnp.sum(s1, axis=0, keepdims=True) * (1.0 / D)
        var = jnp.sum(s2, axis=0, keepdims=True) * (1.0 / D) - mean * mean
        var = jnp.maximum(var, 0.0)
        sd = _rb(jnp.sqrt(_rb(_rb(var) + 1e-5)))
        mb = _rb(mean)
        hi = 0.5 / sd
        if j == 0:
            wrow = wr[...].astype(F32).reshape(1, D)
            tk["w"] = [(jnp.broadcast_to(wrow[:, k0:min(k0 + 128, D)], (16, min(128, D - k0)))
                        + jnp.zeros((16, min(128, D - k0)), F32)).astype(BF16) for k0 in range(0, D, 128)]
        r = None
        for i, k0 in enumerate(range(0, D, 128)):
            n = min(128, D - k0)
            rw = pl.ds(k0 // 2, n // 2)
            hv = _rb(xb[pl.ds(k0, n), cj].astype(F32) - mb) * hi
            h0, h1 = hv[:, :128], hv[:, 128:]
            xh[rw, pl.ds(256 * j, 128)] = _u32(h0)
            xh[rw, pl.ds(256 * j + 128, 128)] = _u32(h1)
            vv[rw, pl.ds(256 * j, 128)] = _u32(h0 + h1)
            vv[rw, pl.ds(256 * j + 128, 128)] = _u32(h0 - h1)
            yield
            p = _dot(tk["w"][i], _bf(xh[rw, cj]))
            r = p if r is None else r + p
        for t in range(2):
            r_t = r[:, 128 * t:128 * t + 128]
            tk["rc"] = r_t if (j == 0 and t == 0) else jnp.where(mk[0].row16 == 2 * j + t, r_t, tk["rc"])

    def topk():
        m = mk[0]
        bits = pltpu.bitcast(_rb(tk["rc"] * 2.0), I32)
        mono = (jnp.where(bits < 0, bits ^ 0x7FFF0000, bits) >> 16) + 32768
        key = pltpu.bitcast(0x30000000 + (mono << 11) + (2047 - (m.row16 * 128 + m.lane16)), F32)
        kcol = jnp.zeros((16, 128), I32)
        for j in range(NSEL):
            mx = jnp.max(jnp.max(key, axis=0, keepdims=True), axis=1, keepdims=True)
            mxb = jnp.broadcast_to(mx, (16, 128))
            key = jnp.where(key == mxb, 0.0, key)
            kcol = jnp.where(m.row16 == j, pltpu.bitcast(mxb, I32), kcol)
        kcol = kcol - 0x30000000
        idxcol = jnp.where(m.row16 < NSEL, 2047 - (kcol & 2047), -1)
        hb = ((kcol >> 11) - 32768) << 16
        rsel = pltpu.bitcast(jnp.where(hb < 0, hb ^ 0x7FFF0000, hb), F32)
        rsel = jnp.where(m.row16 < NSEL, rsel, 0.0)
        rs_s[...] = _rb(jax.nn.sigmoid(rsel))
        oh = jnp.concatenate(
            [jnp.where(idxcol == m.lane16 + 128 * t, 1.0, 0.0) for t in range(16)], axis=1).astype(BF16)
        oh_s[...] = pltpu.bitcast(oh, U32)
        hits = jnp.where(m.row16[:8] < NSEL, jnp.left_shift(1, jnp.maximum(idxcol[:8], 0) >> 7), 0)
        for sh in (4, 2, 1):
            hits = hits | pltpu.roll(hits, sh, 0)
        hit_s[0] = hits[0, 0]
        tcol = jnp.maximum(idxcol, 0) >> 7
        tk["tj"] = [jnp.clip(tcol[j, 0], 0, 15) for j in range(NSEL)]
        tk["ol"] = jnp.where((idxcol & 127) == m.lane16, 1.0, 0.0)

    def xsel(j):
        off = pl.multiple_of(tk["tj"][j] * 128, 128)
        lhs = jnp.where(mk[0].row16 == j, tk["ol"], 0.0).astype(BF16)
        v = _dot_nt(lhs, _bf(xh[:, pl.ds(off, 128)]))
        tk["xa"] = v if j == 0 else tk["xa"] + v
        if j == NSEL - 1:
            xs_s[...] = _u32(tk["xa"] * 2.0)

    ffp = [0, 0]
    ffp_max = [0]

    def wpiece(i, p):
        c = 0
        while 2 * p >= sum(FCH[:c + 1]):
            c += 1
        return wbuf[c][i][:, pl.ds(256 * p - 128 * sum(FCH[:c]), 256)]

    def ffn_gu():
        p = ffp[0]
        ffp[0] += 1
        gu = _dot(tk["xs"], jnp.concatenate([wpiece(0, p), wpiece(1, p)], axis=1))
        g = _rb(gu[:, :256])
        u = _rb(gu[:, 256:])
        sg = _rb(0.5 * jnp.tanh(0.5 * g) + 0.5)
        tk["h", p] = (_rb(g * sg) * u).astype(BF16)

    def ffn_dn():
        p = ffp[1]
        ffp[1] += 1
        y = _dot_nt(tk.pop(("h", p)), wpiece(2, p))
        tk["y"] = y if p == 0 else tk["y"] + y

    def ffn_next():
        if ffp[1] < ffp[0] - 1 or (ffp[1] < ffp[0] and ffp[0] >= ffp_max[0]):
            ffn_dn()
        elif ffp[0] < ffp_max[0]:
            ffn_gu()

    def combine(x, h, y, dv, zh):
        return (x.astype(F32) + (y + h * dv) * (zh * jnp.tanh(zh) + zh)).astype(BF16)

    def fin16(i, c0, c1):
        r16 = pl.ds(16 * i, 16)
        cs = pl.ds(128 * c0, 128 * (c1 - c0))
        h = _bf(xh[pl.ds(8 * i, 8), cs]).astype(F32)
        y = jnp.concatenate([jnp.concatenate([ysv.pop((2 * i + hh, c)) for hh in range(2)], axis=0)
                             for c in range(c0, c1)], axis=1)
        ob[r16, cs] = combine(xb[r16, cs], h, y, jnp.concatenate([deff[r16, :]] * (c1 - c0), axis=1), h)

    def fin_tile(c, du):
        cs = pl.ds(128 * c, 128)
        h = _bf(xh[:, cs]).astype(F32)
        o = 8 * ((c // 2) % 2)
        y = _bf(yb[:, pl.ds(256 * (c // 4) + 128 * (c % 2), 128)]).astype(F32)
        y = y.reshape(NG, 16, 128)[:, o:o + 8, :].reshape(D, 128)
        ob[:, cs] = combine(xb[:, cs], h, y, deff[...], h + du)

    def ut_piece(b, k, j0):
        rw = pl.ds(b * (RU // 2), RU // 2)
        rows = pl.ds(dyn(0), RU)
        ur = urs[b % 3]
        js = range(j0, j0 + UTJ)

        def lhs(ref, o):
            return _bf(jnp.concatenate([ref[rw, pl.ds(256 * j + o, 128)] for j in js], axis=0))

        def put(val, col):
            for i, j in enumerate(js):
                ur[rows, pl.ds(640 * j + col, 128)] = val[i * RU:(i + 1) * RU]
        if k == 0:
            v = _dot(lhs(vv, 0), _bf(um[:, 0:256]))
            b2 = _dot(lhs(vv, 128), _bf(um[:, 256:384]))
            a0 = v[:, :128]
            put(jnp.where(mk[0].lo64u, a0, b2), 0)
            put(v[:, 128:], 128)
            put(pltpu.roll(jnp.where(mk[0].lo64u, b2, a0), 64, 1), 256)
        else:
            put(_dot(lhs(xh, 128), _bf(um[:, 384:512])), 384)
            put(_dot(lhs(xh, 0), _bf(um[:, 512:640])), 512)

    def mac(g, cls):
        ur = urs[(8 * g // RU) % 3]
        m = mk[0]

        def lcat(*vs):
            return jnp.concatenate(vs, axis=1)

        @functools.lru_cache(None)
        def us(j):
            def ld(c):
                return ur[pl.ds((8 * g) % RU, 8), pl.ds(640 * j + c, 128)]
            if cls == 0:
                a, b = ld(0), ld(256)
                return lcat(a + b, a, b)
            t1, t2, t3 = ld(128), ld(384), ld(512)
            return lcat(t2 + t3, t1 + t2, t3 - t1)

        @functools.lru_cache(None)
        def kraw(j):
            return ksps[8 * g // RB][pl.ds((8 * g) % RB, 8), pl.ds(512 * j + 256 * (1 - cls), 256)]

        @functools.lru_cache(None)
        def ks(j):
            sk = kraw(j)
            if j > 0:
                sk = sk + kraw(j - 1) if cls == 0 else sk - kraw(j - 1)
            sr, si = sk[:, :128], sk[:, 128:]
            return lcat(sr * m.mz if cls == 0 else sr, si - sr, sr + si)

        def cat(p, q):
            return jnp.concatenate([p, q], axis=0)
        outs = []
        prev = None
        for mo in range(NCH):
            acc = None
            for j in range(mo + 1):
                t = ks(mo - j) * us(j)
                acc = t if acc is None else acc + t
            z = (acc[:, :128] - acc[:, 256:], acc[:, :128] + acc[:, 128:256])
            if mo % 2 == 1:
                za, zb = prev, z
                if cls == 1:
                    outs.append((cat(za[0] + za[1], zb[0] + zb[1]), cat(za[1], zb[1]), cat(za[0], zb[0])))
                else:
                    zr = _u32(cat(za[0], zb[0]))
                    zis = pltpu.roll(_u32(cat(za[1], zb[1])), 64, 1)
                    outs.append((jnp.where(m.lo64, zr, zis), jnp.where(m.lo64, zis, zr)))
            prev = z
        return outs

    zq, wq = {}, {}

    def inv(g, cls):
        zo = zq.pop((g, cls))

        def st(t):
            v = jnp.concatenate([zo[p][t] for p in range(4)], axis=0)
            return _bf(v) if cls == 0 else v.astype(BF16)
        if cls == 0:
            wq[g] = [_dot(st(t), _bf(umt[:, c:c + 128])) for t, c in ((0, 0), (1, 256))]
        else:
            q1, q2, q3 = [_dot(st(t), _bf(umt[:, c:c + 128])) for t, c in ((0, 128), (1, 384), (2, 512))]
            w0, w2 = wq.pop(g)
            p_ = q1 + w2
            y0 = p_ + (q2 + w0)
            y1 = (q3 + w0) - p_
            for p in range(4):
                yb[pl.ds(8 * g, 8), pl.ds(256 * p, 128)] = _u32(y0[16 * p:16 * p + 16])
                yb[pl.ds(8 * g, 8), pl.ds(256 * p + 128, 128)] = _u32(y1[16 * p:16 * p + 16])
                for e in range(2):
                    ysv[(g, 4 * p + 2 * e)] = y0[16 * p + 8 * e:16 * p + 8 * e + 8]
                    ysv[(g, 4 * p + 2 * e + 1)] = y1[16 * p + 8 * e:16 * p + 8 * e + 8]

    def region(fn):
        @pl.when(zs[0] == 0)
        def _():
            mk[0] = _Masks()
            fn()

    for i, _ in enumerate(kgen(0, R1 // 16)):
        if i == 3:
            _ggen(selb, g0b, gm)
    for cp in in_cp[2]:
        cp.wait()
    slotno[0] += 100
    for _ in kgen(R1 // 16, XW):
        pass
    dkb = _col_bcast(dsk)
    for t in range(5):
        n = 128 if t < 4 else 64
        dkc[pl.ds(t * 128, n), :] = dkb[t][:n]
    in_cp[3][0].wait()

    def phase_a2():
        slotno[0] += 100
        kg = kgen(XW, NS)
        next(kg)
        nslot = 0
        for j in range(NCH):
            for _ in ln_chunk(j):
                kt_drain(1)
                nslot += 1
                if nslot % 5 == 0:
                    next(kg)
        topk()
        xq = list(range(NSEL))
        for i, _ in enumerate(kg):
            kt_drain(i % 2)
            if i >= 21 and xq and (i - 21) % 4 == 0:
                xsel(xq.pop(0))
        while xq:
            xsel(xq.pop(0))
        slotno[0] += 1000
        kt_drain(len(ktq) - NCH)

    region(phase_a2)

    utq = [(b, k, j) for b in range(D // RU) for j in range(0, NCH, UTJ) for k in range(2)]

    def mac_groups(g0, g1):
        for s in range(g0, g1):
            for cls in range(2):
                if s < NG:
                    zq[(s, cls)] = mac(s, cls)
                if 1 <= s < NG + 1:
                    inv(s - 1, cls)
                if utq:
                    ut_piece(*utq.pop(0))
                if cls == 1 and s % 4 == 0 and s >= 4:
                    kt_drain(1)
                q = 2 * (s - 3) + cls - 2
                if 0 <= q < 4 * NS:
                    fin16(q // 4, 4 * (q % 4), 4 * (q % 4) + 4)
                if cls == 0 and (s - g0) % 2 == 0:
                    ffn_next()

    def phase_b():
        in_mac[0] = True
        ends = [gs for gs, _ in FWAIT[1:]] + [NG + 5]
        for (gs, cc), ge in zip(FWAIT, ends):
            for cp in w_cp[cc]:
                cp.wait()
            ffp_max[0] = sum(FCH[:cc + 1]) // 2
            tk["xs"] = _bf(xs_s[...])
            if gs == 0:
                for _ in range(8):
                    ut_piece(*utq.pop(0))
                for t in range(5):
                    rows = pl.ds(128 * t, 128 if t < 4 else 64)
                    deff[rows, :] = (dkc[rows, :] + k0c[rows, :]) * 2.0
            mac_groups(gs, ge)
        while ffp[1] < ffp_max[0]:
            ffn_next()
        ya_s[...] = tk["y"]

    region(phase_b)

    o_cp = [pltpu.make_async_copy(ob.at[:, pl.ds(128 * t, 128)], out_hbm.at[:, pl.ds(128 * t, 128)], sem_o.at[t])
            for t in range(16)]
    tk["xs"] = _bf(xs_s[...])
    rs = rs_s[...]
    tk["y"] = ya_s[...]
    for cc in range(len(FWAIT), len(FCH)):
        for cp in w_cp[cc]:
            cp.wait()
    hit = hit_s[0]
    for t in range(16):
        @pl.when(((hit >> t) & 1) == 0)
        def _():
            o_cp[t].start(priority=1)
    while ffp[0] < sum(FCH) // 2:
        ffn_gu()
        if ffp[1] < ffp[0] - 1:
            ffn_dn()
    while ffp[1] < ffp[0]:
        ffn_dn()
    upd = (_rb(_rb(tk["y"]) * jnp.concatenate([rs] * 5, axis=1)[:, :D]) * 0.5).astype(BF16)
    upt_s[...] = jnp.concatenate([upd, jnp.zeros((16, 64), BF16)], axis=1).T
    hit = hit_s[0]
    for t in range(16):
        @pl.when(((hit >> t) & 1) == 1)
        def _():
            fin_tile(t, _dot(upt_s[pl.ds(0, D), :], _bf(oh_s[:, pl.ds(128 * t, 128)])))
            o_cp[t].start(priority=1)
    for cp in o_cp:
        cp.wait()


@jax.jit
def pallas_recurrent_scan__ssm_conv_s4__moe_arch_mod__prompt_kernel(
        A_u, A_A_re, A_A_im, A_B_re, A_B_im, A_C_re, A_C_im, A_log_dt, A_Dskip,
        B_x, B_w_r, B_w_gate, B_w_up, B_w_down):
    scratch = [
        pltpu.SMEM((1,), I32),
        pltpu.VMEM((D, L), BF16),
        pltpu.VMEM((6, D, N), BF16),
        pltpu.VMEM((D,), BF16),
        pltpu.VMEM((D,), BF16),
        pltpu.VMEM((D,), BF16),
        pltpu.VMEM((64, 640), U32),
        pltpu.VMEM((128, 512), U32),
        pltpu.VMEM((336, 512), U32),
        pltpu.VMEM((8, 256), I32),
        pltpu.VMEM((64, 640), U32),
        pltpu.VMEM((D, 128), F32),
        pltpu.VMEM((D, 128), F32),
        pltpu.VMEM((D, 128), F32),
        pltpu.VMEM((D // 2, L), U32),
        pltpu.VMEM((D // 2, L), U32),
        pltpu.VMEM((RU, 5120), F32),
        pltpu.VMEM((RU, 5120), F32),
        pltpu.VMEM((RU, 5120), F32),
        pltpu.VMEM((D, L // 2), U32),
        pltpu.VMEM((D, L), BF16),
        pltpu.VMEM((16, 128), F32),
        pltpu.VMEM((8, L), U32),
        pltpu.VMEM((8, D), U32),
        pltpu.SMEM((1,), I32),
        pltpu.VMEM((D, 128), F32),
        pltpu.VMEM((16, D), F32),
        pltpu.VMEM((640, 16), BF16),
        pltpu.SemaphoreType.DMA((17,)),
        pltpu.SemaphoreType.DMA((3, len(FCH))),
        pltpu.SemaphoreType.DMA((16,)),
    ]
    scratch += [pltpu.VMEM((RB, 4096), F32)] * NB
    scratch += [pltpu.VMEM((D, 128 * n), BF16) for n in FCH for _ in range(3)]
    scratch += [pltpu.VMEM((RB, 896), F32)] * NB
    out = pl.pallas_call(
        _kernel,
        out_shape=jax.ShapeDtypeStruct((D, L), BF16),
        in_specs=[pl.BlockSpec(memory_space=pl.ANY)] * 14,
        out_specs=pl.BlockSpec(memory_space=pl.ANY),
        scratch_shapes=scratch,
        compiler_params=pltpu.CompilerParams(vmem_limit_bytes=100 * 2**20, disable_semaphore_checks=True,
                                             disable_bounds_checks=True),
        name="s4_mod",
    )(jnp.transpose(A_u[0]), A_A_re, A_A_im, A_B_re, A_B_im, A_C_re, A_C_im, A_log_dt, A_Dskip,
      B_w_r, B_w_gate, B_w_up, jnp.transpose(B_w_down), jnp.asarray(_SEL))
    return jnp.transpose(out)[None]
```
